```python
import jax
import jax.numpy as jnp

def _softmax(x, axis=-1):
    return jax.nn.softmax(x, axis=axis)

def _gelu(x):
    return jax.nn.gelu(x, approximate=True)

def _silu(x):
    return jax.nn.silu(x)

def _sigmoid(x):
    return jax.nn.sigmoid(x)

def _layernorm(x, axis=-1, eps=1e-05):
    m = jnp.mean(x, axis=axis, keepdims=True)
    v = jnp.var(x, axis=axis, keepdims=True)
    return (x - m) / jnp.sqrt(v + eps)

def _scatter_add(tgt, idx, src, axis=0):
    return tgt.at[idx].add(src)

def _segment_sum(src, seg, n):
    return jax.ops.segment_sum(src, seg, n)

class _Rng:

    def __init__(self, key):
        self._k = key

    def _next(self):
        self._k, sub = jax.random.split(self._k)
        return sub

    def normal(self, shape):
        return jax.random.normal(self._next(), shape, dtype=jnp.bfloat16)

    def randint(self, lo, hi, shape):
        return jax.random.randint(self._next(), shape, lo, hi, dtype=jnp.int32)

    def uniform(self, shape, lo=0.0, hi=1.0):
        return jax.random.uniform(self._next(), shape, jnp.bfloat16, lo, hi)

    def permutation(self, n):
        return jax.random.permutation(self._next(), n)
kernel_name = 'adaLN_cond__sliding_local_dilated__glu_gated_swiglu__prompt'

def setup_inputs():
    _rng = _Rng(jax.random.key(int.from_bytes(__import__("os").urandom(4), "little")))
    _w = lambda a: (lambda t: t.astype(jnp.bfloat16) if jnp.issubdtype(t.dtype, jnp.floating) else t)(jnp.asarray(a))

    def _A_setup():
        B, S, D = (1, 2048, 1024)
        return {'x': _w((lambda *s: _rng.normal(s) * 0.05)(B, S, D)), 'wqkv': _w((lambda *s: _rng.normal(s) * 0.05)(D, 3 * D)), 'wo': _w((lambda *s: _rng.normal(s) * 0.05)(D, D))}
    _A_in = _A_setup()

    def _B_setup():
        B, S, D, F = (1, 2048, 1024, 3584)
        return {'x': _w((lambda *s: _rng.normal(s) * 0.05)(B, S, D)), 'w1': _w((lambda *s: _rng.normal(s) * 0.05)(D, F) * (2.0 / D) ** 0.5), 'w3': _w((lambda *s: _rng.normal(s) * 0.05)(D, F) * (2.0 / D) ** 0.5), 'w2': _w((lambda *s: _rng.normal(s) * 0.05)(F, D) * (2.0 / F) ** 0.5)}
    _B_in = _B_setup()
    return {'A_x': _A_in['x'], 'A_wqkv': _A_in['wqkv'], 'A_wo': _A_in['wo'], 'B_x': _B_in['x'], 'B_w1': _B_in['w1'], 'B_w3': _B_in['w3'], 'B_w2': _B_in['w2'], 'c': _w((lambda *s: _rng.normal(s) * 0.05)(1, 1024)), 'w_mod': _w((lambda *s: _rng.normal(s) * 0.05)(1024, 6 * 1024) * 1024 ** (-0.5))}

def reference(A_x, A_wqkv, A_wo, B_x, B_w1, B_w3, B_w2, c, w_mod):

    def _A_ref(x, wqkv, wo):
        B, S, D = x.shape
        H = 32
        Dh = D // H
        W, dil = (8, 2)
        qkv = (lambda x, *d: x.transpose(*d))((x @ wqkv).reshape(B, S, 3, H, Dh), 2, 0, 3, 1, 4)
        q, k, v = (qkv[0], qkv[1], qkv[2])
        scale = Dh ** (-0.5)
        pos = jnp.arange(S)
        off = jnp.arange(W) * dil
        idx = pos[:, None] - off[None, :]
        mask = idx >= 0
        idx_c = jnp.where(mask, idx, 0).reshape(-1)
        kg = k[:, :, idx_c, :].reshape(B, H, S, W, Dh)
        vg = v[:, :, idx_c, :].reshape(B, H, S, W, Dh)
        logits = jnp.einsum('bhsd,bhswd->bhsw', q, kg) * scale
        logits = jnp.where(mask[None, None, :, :], logits, -1000000000.0)
        attn = _softmax(logits, axis=-1)
        o = jnp.einsum('bhsw,bhswd->bhsd', attn, vg)
        return (lambda x, *d: x.transpose(*d))(o, 0, 2, 1, 3).reshape(B, S, D) @ wo

    def _B_ref(x, w1, w3, w2):
        gate = jnp.einsum('bsd,df->bsf', x, w1)
        up = jnp.einsum('bsd,df->bsf', x, w3)
        h = _silu(gate) * up
        out = jnp.einsum('bsf,fd->bsd', h, w2)
        return out
    x = A_x
    mod = (_silu(c) @ w_mod).reshape(c.shape[0], 6, 1, -1)
    sa, ca, ga, sb, cb, gb = (mod[:, 0].copy(), mod[:, 1].copy(), mod[:, 2].copy(), mod[:, 3].copy(), mod[:, 4].copy(), mod[:, 5].copy())
    h = _layernorm(x, axis=-1) * (1 + ca) + sa
    x = x + ga * _A_ref(h, A_wqkv, A_wo)
    h = _layernorm(x, axis=-1) * (1 + cb) + sb
    x = x + gb * _B_ref(h, B_w1, B_w3, B_w2)
    return x
```

```python
import functools

import jax
import jax.numpy as jnp
import jax.experimental.pallas as pl
import jax.experimental.pallas.tpu as pltpu

S, D, F = 2048, 1024, 3584
H, DH, W, DIL = 32, 32, 8, 2
NG = D // 128
TM = 256
SUB = 128
RB = 16
FC = 512
HALO = 16
EPS = 1e-5
SCALE = DH ** -0.5
LOG2E = 1.4426950408889634
NEG = -1000000000.0 / SCALE

f32 = jnp.float32
bf16 = jnp.bfloat16


def _swap_stage(a, k, b):
    lane = jax.lax.broadcasted_iota(jnp.int32, a[0].shape, 1)
    m0 = (lane & (1 << b)) == 0
    out = list(a)
    for c in range(8):
        if c & (1 << k):
            continue
        lo, hi = a[c], a[c | (1 << k)]
        out[c] = jnp.where(m0, lo, pltpu.roll(hi, 1 << b, 1))
        out[c | (1 << k)] = jnp.where(m0, pltpu.roll(lo, 128 - (1 << b), 1), hi)
    return out


def _permute_qkv_rows(w_ref, r0, nrows):
    for sec in range(3):
        a = [pltpu.bitcast(w_ref[pl.ds(r0, nrows), pl.ds(sec * D + c * 128, 128)], jnp.uint32)
             for c in range(8)]
        for k in range(3):
            a = _swap_stage(a, k, k)
        for c in range(8):
            w_ref[pl.ds(r0, nrows), pl.ds(sec * D + c * 128, 128)] = pltpu.bitcast(a[c], bf16)


def _layernorm(x):
    m = jnp.mean(x, axis=-1, keepdims=True)
    xc = x - m
    v = jnp.mean(xc * xc, axis=-1, keepdims=True)
    return xc * jax.lax.rsqrt(v + EPS)


def _group_sum(z, m3, m4):
    z = z + jnp.where(m3, pltpu.roll(z, 120, 1), pltpu.roll(z, 8, 1))
    z = z + jnp.where(m4, pltpu.roll(z, 112, 1), pltpu.roll(z, 16, 1))
    return z


def _attention_block(q_s, k_s, v_s, r0, row_base):
    lane = jax.lax.broadcasted_iota(jnp.int32, (RB, 128), 1)
    m3 = (lane & 8) == 0
    m4 = (lane & 16) == 0
    q = [q_s[g, pl.ds(r0, RB), :] for g in range(NG)]
    logits = []
    for w in range(W):
        z = None
        for g in range(NG):
            p = q[g] * k_s[g, pl.ds(HALO + r0 - DIL * w, RB), :]
            z = p if z is None else z + p
        z = _group_sum(z, m3, m4)
        if w > 0 and r0 < HALO:
            row = jax.lax.broadcasted_iota(jnp.int32, (RB, 128), 0) + (row_base + r0)
            z = jnp.where(row >= DIL * w, z, NEG)
        logits.append(z)
    m = logits[0]
    for w in range(1, W):
        m = jnp.maximum(m, logits[w])
    e = [jnp.exp2((logits[w] - m) * (SCALE * LOG2E)) for w in range(W)]
    den = e[0]
    for w in range(1, W):
        den = den + e[w]
    inv = pl.reciprocal(den, approx=False)
    outs = []
    for g in range(NG):
        o = None
        for w in range(W):
            p = e[w] * v_s[g, pl.ds(HALO + r0 - DIL * w, RB), :]
            o = p if o is None else o + p
        outs.append((o * inv).astype(bf16))
    return jnp.concatenate(outs, axis=1)


def _kernel(x_ref, c_ref, wqkv_hbm, wo_hbm, w1_hbm, w3_hbm, w2_hbm, wmod_hbm, o_ref,
            wqkv_v, wo_raw, wo_f, wo_v, w1_v, w3_v, w2_v, wmod_v, mod_v, q_s, k_s, v_s, sems):
    step = pl.program_id(0)

    @pl.when(step == 0)
    def _prologue():
        copies = [
            pltpu.make_async_copy(wmod_hbm, wmod_v, sems.at[0]),
            pltpu.make_async_copy(wqkv_hbm, wqkv_v, sems.at[1]),
            pltpu.make_async_copy(wo_hbm, wo_raw, sems.at[2]),
            pltpu.make_async_copy(w1_hbm, w1_v, sems.at[3]),
            pltpu.make_async_copy(w3_hbm, w3_v, sems.at[4]),
            pltpu.make_async_copy(w2_hbm, w2_v, sems.at[5]),
        ]
        for cp in copies:
            cp.start()
        for cp in copies:
            cp.wait()
        c = c_ref[...].astype(f32)
        sc = (c * jax.nn.sigmoid(c)).astype(bf16)
        sc = jnp.broadcast_to(sc, (16, D))
        mod_v[...] = jnp.dot(sc, wmod_v[...], preferred_element_type=f32)[0:8]

        def perm_body(i, carry):
            _permute_qkv_rows(wqkv_v, pl.multiple_of(i * 64, 64), 64)
            return carry
        jax.lax.fori_loop(0, D // 64, perm_body, 0)

        for g in range(NG):
            wo_f[g] = wo_raw[:, g * 128:(g + 1) * 128].astype(f32)

        def wo_body(dlo, carry):
            for g in range(NG):
                rows = [wo_f[g, pl.ds(mid * 8 + dlo, 8, stride=128), :] for mid in range(16)]
                blk = jnp.concatenate(rows, axis=0).astype(bf16)
                wo_v[pl.ds(pl.multiple_of(dlo * 128, 128), 128), g * 128:(g + 1) * 128] = blk
            return carry
        jax.lax.fori_loop(0, 8, wo_body, 0)

        k_s[:, 0:HALO, :] = jnp.zeros((NG, HALO, 128), f32)
        v_s[:, 0:HALO, :] = jnp.zeros((NG, HALO, 128), f32)

    sa = mod_v[0:1, 0 * D:1 * D]
    ca = mod_v[0:1, 1 * D:2 * D]
    ga = mod_v[0:1, 2 * D:3 * D]
    sb = mod_v[0:1, 3 * D:4 * D]
    cb = mod_v[0:1, 4 * D:5 * D]
    gb = mod_v[0:1, 5 * D:6 * D]
    row_base = step * TM
    nsub = TM // SUB

    xs = [x_ref[pl.ds(s * SUB, SUB), :].astype(f32) for s in range(nsub)]
    for s in range(nsub):
        h = (_layernorm(xs[s]) * (1.0 + ca) + sa).astype(bf16)
        for sec, (dst, off) in enumerate(((q_s, 0), (k_s, HALO), (v_s, HALO))):
            res = jnp.dot(h, wqkv_v[:, sec * D:(sec + 1) * D], preferred_element_type=f32)
            for g in range(NG):
                dst[g, pl.ds(off + s * SUB, SUB), :] = res[:, g * 128:(g + 1) * 128]

    x1s, h2s = [], []
    for s in range(nsub):
        o = jnp.concatenate(
            [_attention_block(q_s, k_s, v_s, s * SUB + b * RB, row_base) for b in range(SUB // RB)],
            axis=0)
        att = jnp.dot(o, wo_v[...], preferred_element_type=f32)
        x1 = xs[s] + ga * att
        x1s.append(x1)
        h2s.append((_layernorm(x1) * (1.0 + cb) + sb).astype(bf16))

    k_s[:, 0:HALO, :] = k_s[:, TM:TM + HALO, :]
    v_s[:, 0:HALO, :] = v_s[:, TM:TM + HALO, :]

    for s in range(nsub):
        h2 = h2s[s]
        acc = None
        for j in range(F // FC):
            g = jnp.dot(h2, w1_v[:, j * FC:(j + 1) * FC], preferred_element_type=f32)
            u = jnp.dot(h2, w3_v[:, j * FC:(j + 1) * FC], preferred_element_type=f32)
            hg = 0.5 * g
            a = ((hg + hg * jnp.tanh(hg)) * u).astype(bf16)
            y = jnp.dot(a, w2_v[j * FC:(j + 1) * FC, :], preferred_element_type=f32)
            acc = y if acc is None else acc + y
        o_ref[pl.ds(s * SUB, SUB), :] = (x1s[s] + gb * acc).astype(o_ref.dtype)


@jax.jit
def pallas_adaLN_cond__sliding_local_dilated__glu_gated_swiglu__prompt_kernel(
    A_x: jax.Array,
    A_wqkv: jax.Array,
    A_wo: jax.Array,
    B_x: jax.Array,
    B_w1: jax.Array,
    B_w3: jax.Array,
    B_w2: jax.Array,
    c: jax.Array,
    w_mod: jax.Array,
):
    del B_x
    x = A_x.reshape(S, D)
    hbm = pl.BlockSpec(memory_space=pl.ANY)
    out = pl.pallas_call(
        _kernel,
        grid=(S // TM,),
        in_specs=[
            pl.BlockSpec((TM, D), lambda i: (i, 0)),
            pl.BlockSpec((1, D), lambda i: (0, 0)),
            hbm, hbm, hbm, hbm, hbm, hbm,
        ],
        out_specs=pl.BlockSpec((TM, D), lambda i: (i, 0)),
        out_shape=jax.ShapeDtypeStruct((S, D), A_x.dtype),
        scratch_shapes=[
            pltpu.VMEM((D, 3 * D), bf16),
            pltpu.VMEM((D, D), bf16),
            pltpu.VMEM((NG, D, 128), f32),
            pltpu.VMEM((D, D), bf16),
            pltpu.VMEM((D, F), bf16),
            pltpu.VMEM((D, F), bf16),
            pltpu.VMEM((F, D), bf16),
            pltpu.VMEM((D, 6 * D), bf16),
            pltpu.VMEM((8, 6 * D), f32),
            pltpu.VMEM((NG, TM, 128), f32),
            pltpu.VMEM((NG, HALO + TM, 128), f32),
            pltpu.VMEM((NG, HALO + TM, 128), f32),
            pltpu.SemaphoreType.DMA((6,)),
        ],
        compiler_params=pltpu.CompilerParams(
            dimension_semantics=("arbitrary",),
            vmem_limit_bytes=100 * 1024 * 1024,
        ),
        name="adaln_attn_ffn",
    )(x, c, A_wqkv, A_wo, B_w1, B_w3, B_w2, w_mod)
    return out.reshape(1, S, D)
```

```python
import jax
import jax.numpy as jnp
import jax.experimental.pallas as pl
import jax.experimental.pallas.tpu as pltpu

S, D, F = 2048, 1024, 3584
H, DH, W, DIL = 32, 32, 8, 2
NG = D // 128
TM = 256
NT = S // TM
N1 = NT - 1
SUB = 128
FC = 512
KC = 128
NKC = D // KC
HALO = 16
EPS = 1e-5
SCALE = DH ** -0.5
LOG2E = 1.4426950408889634
QSCALE = SCALE * LOG2E
NEG = -1000000000.0 * LOG2E

f32 = jnp.float32
bf16 = jnp.bfloat16
u32 = jnp.uint32

SEM_C = 0
SEM_X = 1
SEM_WQ = 6
SEM_WS = SEM_WQ + NKC
SEM_WC = SEM_WS + NKC
SEM_WM = SEM_WC + NKC
SEM_WO = SEM_WM + 4
SEM_FF = SEM_WO + 2
NSEM = SEM_FF + 3


def _when(cond, name):
    def deco(body):
        def scoped():
            with jax.named_scope(name):
                body()
        return pl.when(cond)(scoped)
    return deco


def _pack(x):
    return pltpu.bitcast(x, u32)


def _unpack(x):
    return pltpu.bitcast(x, bf16)


def _swap_stage(a, k, b, axis):
    n = 128 if axis == 1 else 8
    idx = jax.lax.broadcasted_iota(jnp.int32, a[0].shape, axis)
    m0 = (idx & (1 << b)) == 0
    out = list(a)
    for c in range(8):
        if c & (1 << k):
            continue
        lo, hi = a[c], a[c | (1 << k)]
        out[c] = jnp.where(m0, lo, pltpu.roll(hi, 1 << b, axis))
        out[c | (1 << k)] = jnp.where(m0, pltpu.roll(lo, n - (1 << b), axis), hi)
    return out


def _permute_qkv_section(w_ref, r0, sec):
    a = [_pack(w_ref[pl.ds(r0, KC), pl.ds(sec * D + c * 128, 128)]) for c in range(8)]
    for k in range(3):
        a = _swap_stage(a, k, k + 1, 1)
    return jnp.concatenate(a, axis=1)


def _ln_stats(x):
    m = jnp.mean(x, axis=-1, keepdims=True)
    xc = x - m
    v = jnp.mean(xc * xc, axis=-1, keepdims=True)
    r = jax.lax.rsqrt(v + EPS)
    return r, m * r


def _modulated_ln(x, scale1, shift):
    r, mr = _ln_stats(x)
    return ((x * r - mr) * scale1 + shift).astype(bf16)


def _attention_rows(q_s, k_s, v_s, q0, row0):
    lane = jax.lax.broadcasted_iota(jnp.int32, (8, 128), 1)
    m0 = (lane & 1) == 0
    m4 = (lane & 16) == 0
    q = [q_s[g, pl.ds(q0, 8), :] * QSCALE for g in range(NG)]
    logits = []
    for w in range(W):
        z = None
        for g in range(NG):
            p = q[g] * k_s[g, pl.ds(q0 + (HALO - DIL * w), 8), :]
            z = p if z is None else z + p
        z = z + jnp.where(m0, pltpu.roll(z, 127, 1), pltpu.roll(z, 1, 1))
        z = z + jnp.where(m4, pltpu.roll(z, 112, 1), pltpu.roll(z, 16, 1))
        if w > 0 and row0 is not None:
            row = jax.lax.broadcasted_iota(jnp.int32, (8, 128), 0) + row0
            z = jnp.where(row >= DIL * w, z, NEG)
        logits.append(z)
    m = logits[0]
    for w in range(1, W):
        m = jnp.maximum(m, logits[w])
    e = [jnp.exp2(logits[w] - m) for w in range(W)]
    den = e[0]
    for w in range(1, W):
        den = den + e[w]
    inv = pl.reciprocal(den, approx=False)
    outs = []
    for g in range(NG):
        o = None
        for w in range(W):
            p = e[w] * v_s[g, pl.ds(q0 + (HALO - DIL * w), 8), :]
            o = p if o is None else o + p
        outs.append(o * inv)
    return jnp.concatenate(outs, axis=1)


def _attention(q_s, k_s, v_s, o_s, q0, o0, nrows, row0=None):
    for b in range(nrows // 16):
        halves = [
            _attention_rows(q_s, k_s, v_s, q0 + b * 16 + t * 8,
                            None if (row0 is None or b > 0) else row0 + t * 8)
            for t in range(2)]
        o_s[pl.ds(o0 + b * 8, 8), :] = _pack(jnp.concatenate(halves, axis=0).astype(bf16))


def _mod_group(wmod_v, st_v, col):
    p = wmod_v[:, pl.ds(col, 128)].astype(f32) * st_v[...]
    acc = p.reshape(D // 32, 32, 128).sum(axis=0)
    return acc.sum(axis=0, keepdims=True)


def _kernel(x_hbm, c_hbm, wqkv_hbm, wo_hbm, w1_hbm, w3_hbm, w2_hbm, wmod_hbm, o_ref,
            x_v, c_v, wqkv_raw, wqkv_p, wo_raw, wo_p, w1_v, w3_v, w2_v, wmod_v, mod_v, st_v,
            xn_s, wcur_s, h1_s, h_s, q0_s, k0_s, v0_s, q_s, k_s, v_s, o_s, sems):
    step = pl.program_id(0)

    def cp_x(i):
        n = TM if i < 4 else 4 * TM
        return pltpu.make_async_copy(x_hbm.at[pl.ds(i * TM, n)], x_v.at[pl.ds(i * TM, n)],
                                     sems.at[SEM_X + i])

    def cp_wq(k):
        rows = pl.ds(k * KC, KC)
        return pltpu.make_async_copy(wqkv_hbm.at[rows], wqkv_raw.at[rows], sems.at[SEM_WQ + k])

    def cp_wmod(col, n, sem):
        cols = pl.ds(col, n)
        return pltpu.make_async_copy(wmod_hbm.at[:, cols], wmod_v.at[:, cols], sems.at[sem])

    cp_ws = lambda k: cp_wmod(k * KC, KC, SEM_WS + k)
    cp_wc = lambda k: cp_wmod(D + k * KC, KC, SEM_WC + k)
    cp_wm = lambda p: cp_wmod((2 + p) * D, D, SEM_WM + p)

    def cp_wo(i):
        cols = pl.ds(0, 256) if i == 0 else pl.ds(256, D - 256)
        return pltpu.make_async_copy(wo_hbm.at[:, cols], wo_raw.at[:, cols], sems.at[SEM_WO + i])

    cp_c = lambda: pltpu.make_async_copy(c_hbm, c_v, sems.at[SEM_C])
    cp_w1 = lambda: pltpu.make_async_copy(w1_hbm, w1_v, sems.at[SEM_FF])
    cp_w3 = lambda: pltpu.make_async_copy(w3_hbm, w3_v, sems.at[SEM_FF + 1])
    cp_w2 = lambda: pltpu.make_async_copy(w2_hbm, w2_v, sems.at[SEM_FF + 2])

    def ln1_next(r0):
        sa = mod_v[0:1, 0 * D:1 * D]
        ca1 = 1.0 + mod_v[0:1, 1 * D:2 * D]
        for s in range(TM // SUB):
            x = x_v[pl.ds(r0 + s * SUB, SUB), :].astype(f32)
            h_s[pl.ds(s * SUB // 2, SUB // 2), :] = _pack(_modulated_ln(x, ca1, sa))

    tile0_dst = ((q0_s, 0), (k0_s, HALO), (v0_s, HALO))
    rest_dst = ((q_s, 0), (k_s, HALO), (v_s, HALO))

    @_when(step == 0, 'first')
    def _first():
        order = [cp_c(), cp_wq(0), cp_x(0), cp_ws(0), cp_wc(0), cp_x(1)]
        for k in range(1, NKC):
            order += [cp_wq(k), cp_ws(k), cp_wc(k)]
        order += [cp_x(2), cp_x(3), cp_wo(0), cp_wm(0), cp_x(4), cp_wo(1), cp_wm(1), cp_wm(2),
                  cp_wm(3), cp_w1(), cp_w3(), cp_w2()]
        for cp in order:
            cp.start()

        for dst, off in rest_dst:
            dst[:, pl.ds(off, TM), :] = jnp.zeros((NG, TM, 128), f32)
        cp_c().wait()
        c = c_v[...].astype(f32)
        sc = c * jax.nn.sigmoid(c)
        st_v[...] = jnp.transpose(jnp.broadcast_to(sc, (128, D)))

        def normalize(t):
            for s in range(TM // SUB):
                x = x_v[pl.ds(t * TM + s * SUB, SUB), :].astype(f32)
                r, mr = _ln_stats(x)
                xn = x * r - mr
                for g in range(NG):
                    xn_s[g, pl.ds(t * TM + s * SUB, SUB), :] = xn[:, g * 128:(g + 1) * 128]

        def mod_chunk(k):
            col = k * KC if isinstance(k, int) else pl.multiple_of(k * KC, KC)
            sa = _mod_group(wmod_v, st_v, col)
            ca = _mod_group(wmod_v, st_v, D + col)
            mod_v[:, pl.ds(col, KC)] = jnp.broadcast_to(sa, (8, KC))
            mod_v[:, pl.ds(D + col, KC)] = jnp.broadcast_to(ca, (8, KC))
            return sa, 1.0 + ca

        def h_chunk(k, t, sa, ca1):
            return (xn_s[k, pl.ds(t * TM, TM), :] * ca1 + sa).astype(bf16)

        def mm(h, w, sec, dsts, first):
            res = jnp.dot(h, _unpack(w), preferred_element_type=f32)
            dst, off = dsts[sec]
            for g in range(NG):
                blk = res[:, g * 128:(g + 1) * 128]
                if first:
                    dst[g, pl.ds(off, TM), :] = blk
                else:
                    dst[g, pl.ds(off, TM), :] += blk

        def keep(k, sec, wp):
            r0 = k * (KC // 2) if isinstance(k, int) else pl.multiple_of(k * (KC // 2), KC // 2)
            wcur_s[:, sec * D:(sec + 1) * D] = wp
            wqkv_p[pl.ds(r0, KC // 2), sec * D:(sec + 1) * D] = wp

        cp_wq(0).wait()
        for sec in range(3):
            keep(0, sec, _permute_qkv_section(wqkv_raw, 0, sec))
        cp_x(0).wait()
        normalize(0)
        cp_ws(0).wait()
        cp_wc(0).wait()
        sa, ca1 = mod_chunk(0)
        h0 = h_chunk(0, 0, sa, ca1)
        for sec in range(3):
            mm(h0, wcur_s[:, sec * D:(sec + 1) * D], sec, tile0_dst, True)
        cp_x(1).wait()
        normalize(1)
        h1_s[...] = _pack(h_chunk(0, 1, mod_v[0:1, 0:KC], 1.0 + mod_v[0:1, D:D + KC]))

        def chunk_body(k0, carry):
            k = k0 + 1
            cp_wq(k).wait()
            cp_ws(k).wait()
            cp_wc(k).wait()
            h1 = _unpack(h1_s[...])
            for sec in range(3):
                mm(h1, wcur_s[:, sec * D:(sec + 1) * D], sec, rest_dst, False)
            sa, ca1 = mod_chunk(k)
            h0 = h_chunk(k, 0, sa, ca1)
            h1_s[...] = _pack(h_chunk(k, 1, sa, ca1))
            for sec in range(3):
                wp = _permute_qkv_section(wqkv_raw, pl.multiple_of(k * KC, KC), sec)
                mm(h0, wp, sec, tile0_dst, False)
                keep(k, sec, wp)
            return carry
        jax.lax.fori_loop(0, NKC - 1, chunk_body, 0)

        cp_x(2).wait()
        h1 = _unpack(h1_s[...])
        for sec in range(3):
            mm(h1, wcur_s[:, sec * D:(sec + 1) * D], sec, rest_dst, False)
        ln1_next(2 * TM)
        k0_s[:, 0:HALO, :] = jnp.zeros((NG, HALO, 128), f32)
        v0_s[:, 0:HALO, :] = jnp.broadcast_to(v0_s[:, HALO:HALO + 1, :], (NG, HALO, 128))
        k_s[:, 0:HALO, :] = k0_s[:, TM:TM + HALO, :]
        v_s[:, 0:HALO, :] = v0_s[:, TM:TM + HALO, :]

    @_when(step == 1, 'wait1')
    def _():
        cp_x(3).wait()
        cp_wo(0).wait()
        cp_wm(0).wait()

    @_when(step == 2, 'wait2')
    def _():
        cp_x(4).wait()

    @_when(step == 4, 'wait4')
    def _():
        cp_wo(1).wait()
        cp_wm(1).wait()

    @_when(step == 5, 'wait5')
    def _():
        cp_wm(2).wait()

    @_when(step == 6, 'wait6')
    def _():
        cp_wm(3).wait()

    @_when(jnp.logical_and(step >= 1, step < N1), 'phase1')
    def _phase1():
        part = jnp.maximum(step - 3, 0)
        base = pl.multiple_of(step * TM, TM)
        h = _unpack(h_s[...])
        for sec, (dst, off) in enumerate(rest_dst):
            res = jnp.dot(h, _unpack(wqkv_p[:, sec * D:(sec + 1) * D]), preferred_element_type=f32)
            for g in range(NG):
                dst[g, pl.ds(base + off, TM), :] = res[:, g * 128:(g + 1) * 128]
        ln1_next(pl.multiple_of(jnp.minimum(step + 2, NT - 1) * TM, TM))
        r0 = pl.multiple_of(part * 64, 64)
        _attention(q0_s, k0_s, v0_s, o_s, r0, pl.multiple_of(part * 32, 32), 64, row0=r0)
        for gg in range(2):
            col = pl.ds(pl.multiple_of(part * 256 + gg * 128, 128), 128)
            for mid in range(8):
                a = [_pack(wo_raw[pl.ds(c * 128 + mid * 16, 16), col]) for c in range(8)]
                for k in range(3):
                    a = _swap_stage(a, k, k, 0)
                for s in range(8):
                    wo_p[pl.ds(s * 64 + mid * 8, 8), col] = a[s]
        for j in range(NG):
            col = pl.multiple_of((2 + part) * D + j * 128, 128)
            mod_v[:, pl.ds(col, 128)] = jnp.broadcast_to(_mod_group(wmod_v, st_v, col), (8, 128))

    @_when(step == N1, 'wait7')
    def _():
        cp_w1().wait()
        cp_w3().wait()
        cp_w2().wait()

    @_when(step >= N1, 'phase2')
    def _phase2():
        j2 = step - N1
        ga = mod_v[0:1, 2 * D:3 * D]
        sb = mod_v[0:1, 3 * D:4 * D]
        cb1 = 1.0 + mod_v[0:1, 4 * D:5 * D]
        gb = mod_v[0:1, 5 * D:6 * D]
        row0 = pl.multiple_of(j2 * TM, TM)
        nsub = TM // SUB
        os_ = [_unpack(o_s[pl.ds(s * SUB // 2, SUB // 2), :]) for s in range(nsub)]
        x1s, h2s = [], []
        for s in range(nsub):
            att = jnp.dot(os_[s], _unpack(wo_p[...]), preferred_element_type=f32)
            x1 = x_v[pl.ds(row0 + s * SUB, SUB), :].astype(f32) + ga * att
            x1s.append(x1)
            h2s.append(_modulated_ln(x1, cb1, sb))

        nq = pl.multiple_of(jnp.minimum(j2, NT - 2) * TM, TM)
        _attention(q_s, k_s, v_s, o_s, nq, 0, TM)

        def gate_up(h2, j):
            g = jnp.dot(h2, w1_v[:, j * FC:(j + 1) * FC], preferred_element_type=f32)
            u = jnp.dot(h2, w3_v[:, j * FC:(j + 1) * FC], preferred_element_type=f32)
            hg = 0.5 * g
            return ((hg + hg * jnp.tanh(hg)) * u).astype(bf16)

        def down(a, j):
            return jnp.dot(a, w2_v[j * FC:(j + 1) * FC, :], preferred_element_type=f32)

        a0 = jnp.concatenate([gate_up(h2s[s], 0) for s in range(nsub)], axis=0)
        h2 = jnp.concatenate(h2s, axis=0)
        acc = down(a0, 0)
        for j in range(1, F // FC):
            acc = acc + down(gate_up(h2, j), j)
        o_ref[...] = (jnp.concatenate(x1s, axis=0) + gb * acc).astype(o_ref.dtype)


@jax.jit
def pallas_adaLN_cond__sliding_local_dilated__glu_gated_swiglu__prompt_kernel(
    A_x: jax.Array,
    A_wqkv: jax.Array,
    A_wo: jax.Array,
    B_x: jax.Array,
    B_w1: jax.Array,
    B_w3: jax.Array,
    B_w2: jax.Array,
    c: jax.Array,
    w_mod: jax.Array,
):
    del B_x
    x = A_x.reshape(S, D)
    hbm = pl.BlockSpec(memory_space=pl.ANY)
    out = pl.pallas_call(
        _kernel,
        grid=(N1 + NT,),
        in_specs=[hbm] * 8,
        out_specs=pl.BlockSpec((TM, D), lambda i: (jnp.maximum(i - N1, 0), 0)),
        out_shape=jax.ShapeDtypeStruct((S, D), A_x.dtype),
        scratch_shapes=[
            pltpu.VMEM((S, D), bf16),
            pltpu.VMEM((1, D), bf16),
            pltpu.VMEM((D, 3 * D), bf16),
            pltpu.VMEM((D // 2, 3 * D), u32),
            pltpu.VMEM((D, D), bf16),
            pltpu.VMEM((D // 2, D), u32),
            pltpu.VMEM((D, F), bf16),
            pltpu.VMEM((D, F), bf16),
            pltpu.VMEM((F, D), bf16),
            pltpu.VMEM((D, 6 * D), bf16),
            pltpu.VMEM((8, 6 * D), f32),
            pltpu.VMEM((D, 128), f32),
            pltpu.VMEM((NG, 2 * TM, 128), f32),
            pltpu.VMEM((KC // 2, 3 * D), u32),
            pltpu.VMEM((TM // 2, KC), u32),
            pltpu.VMEM((TM // 2, D), u32),
            pltpu.VMEM((NG, TM, 128), f32),
            pltpu.VMEM((NG, HALO + TM, 128), f32),
            pltpu.VMEM((NG, HALO + TM, 128), f32),
            pltpu.VMEM((NG, S - TM, 128), f32),
            pltpu.VMEM((NG, HALO + S - TM, 128), f32),
            pltpu.VMEM((NG, HALO + S - TM, 128), f32),
            pltpu.VMEM((TM // 2, D), u32),
            pltpu.SemaphoreType.DMA((NSEM,)),
        ],
        compiler_params=pltpu.CompilerParams(
            dimension_semantics=("arbitrary",),
            vmem_limit_bytes=110 * 1024 * 1024,
        ),
        name="adaln_attn_ffn",
    )(x, c, A_wqkv, A_wo, B_w1, B_w3, B_w2, w_mod)
    return out.reshape(1, S, D)
```

```python
import jax
import jax.numpy as jnp
import jax.experimental.pallas as pl
import jax.experimental.pallas.tpu as pltpu

S, D, F = 2048, 1024, 3584
H, DH, W, DIL = 32, 32, 8, 2
NG = D // 128
TM = 256
NT = S // TM
N1 = NT - 1
SUB = 128
FC = 512
KC = 128
NKC = D // KC
HALO = 16
LNR = 16
EPS = 1e-5
SCALE = DH ** -0.5
LOG2E = 1.4426950408889634
QSCALE = SCALE * LOG2E
NEG = -1000000000.0 * LOG2E

f32 = jnp.float32
bf16 = jnp.bfloat16
u32 = jnp.uint32

SEM_C = 0
SEM_X = 1
SEM_WQ = 6
SEM_WS = SEM_WQ + NKC
SEM_WC = SEM_WS + NKC
SEM_WM = SEM_WC + NKC
SEM_WO = SEM_WM + 4
SEM_FF = SEM_WO + 2
NSEM = SEM_FF + 3


def _when(cond, name):
    def deco(body):
        def scoped():
            with jax.named_scope(name):
                body()
        return pl.when(cond)(scoped)
    return deco


def _pack(x):
    return pltpu.bitcast(x, u32)


def _unpack(x):
    return pltpu.bitcast(x, bf16)


class _Chain:
    def __init__(self, always):
        self.always = always
        self.tok = None

    def after(self, x):
        if self.tok is None:
            return x
        t = self.tok if self.tok.dtype == x.dtype else pltpu.bitcast(self.tok, x.dtype)
        return jnp.where(self.always, x, t)

    def after_rows(self, x):
        x00 = self.after(x[0:8, 0:128])
        return jnp.concatenate([jnp.concatenate([x00, x[0:8, 128:]], axis=1), x[8:]], axis=0)


def _swap_stage(a, k, b, axis):
    n = 128 if axis == 1 else 8
    idx = jax.lax.broadcasted_iota(jnp.int32, a[0].shape, axis)
    m0 = (idx & (1 << b)) == 0
    out = list(a)
    for c in range(8):
        if c & (1 << k):
            continue
        lo, hi = a[c], a[c | (1 << k)]
        out[c] = jnp.where(m0, lo, pltpu.roll(hi, 1 << b, axis))
        out[c | (1 << k)] = jnp.where(m0, pltpu.roll(lo, n - (1 << b), axis), hi)
    return out


def _permute_qkv_section(w_ref, r0, sec):
    a = [_pack(w_ref[pl.ds(r0, KC), pl.ds(sec * D + c * 128, 128)]) for c in range(8)]
    for k in range(3):
        a = _swap_stage(a, k, k + 1, 1)
    return jnp.concatenate(a, axis=1)


def _ln_stats(x):
    m = jnp.mean(x, axis=-1, keepdims=True)
    xc = x - m
    v = jnp.mean(xc * xc, axis=-1, keepdims=True)
    r = jax.lax.rsqrt(v + EPS)
    return r, m * r


def _modulated_ln(x, scale1, shift):
    r, mr = _ln_stats(x)
    return ((x * r - mr) * scale1 + shift).astype(bf16)


def _attention_rows(q_s, k_s, v_s, q0, row0):
    lane = jax.lax.broadcasted_iota(jnp.int32, (8, 128), 1)
    m0 = (lane & 1) == 0
    m4 = (lane & 16) == 0
    q = [q_s[g, pl.ds(q0, 8), :] * QSCALE for g in range(NG)]
    logits = []
    for w in range(W):
        z = None
        for g in range(NG):
            p = q[g] * k_s[g, pl.ds(q0 + (HALO - DIL * w), 8), :]
            z = p if z is None else z + p
        z = z + jnp.where(m0, pltpu.roll(z, 127, 1), pltpu.roll(z, 1, 1))
        z = z + jnp.where(m4, pltpu.roll(z, 112, 1), pltpu.roll(z, 16, 1))
        if w > 0 and row0 is not None:
            row = jax.lax.broadcasted_iota(jnp.int32, (8, 128), 0) + row0
            z = jnp.where(row >= DIL * w, z, NEG)
        logits.append(z)
    m = logits[0]
    for w in range(1, W):
        m = jnp.maximum(m, logits[w])
    e = [jnp.exp2(logits[w] - m) for w in range(W)]
    den = e[0]
    for w in range(1, W):
        den = den + e[w]
    inv = pl.reciprocal(den, approx=False)
    outs = []
    for g in range(NG):
        o = None
        for w in range(W):
            p = e[w] * v_s[g, pl.ds(q0 + (HALO - DIL * w), 8), :]
            o = p if o is None else o + p
        outs.append(o * inv)
    return jnp.concatenate(outs, axis=1)


def _attention(q_s, k_s, v_s, o_s, q0, o0, nrows, row0=None):
    for b in range(nrows // 16):
        halves = [
            _attention_rows(q_s, k_s, v_s, q0 + b * 16 + t * 8,
                            None if (row0 is None or b > 0) else row0 + t * 8)
            for t in range(2)]
        o_s[pl.ds(o0 + b * 8, 8), :] = _pack(jnp.concatenate(halves, axis=0).astype(bf16))


def _mod_cols(wmod_v, st_v, cols, n, chain=None):
    acc = [None] * len(cols)
    for r in range(0, D, 8):
        s = st_v[r:r + 8, :]
        if r == 0 and chain is not None:
            s = chain.after(s)
        if n > 128:
            s = jnp.concatenate([s] * (n // 128), axis=1)
        for i, col in enumerate(cols):
            p = wmod_v[r:r + 8, pl.ds(col, n)].astype(f32) * s
            acc[i] = p if acc[i] is None else acc[i] + p
    if chain is not None:
        chain.tok = acc[0][:, 0:128]
    return [a.sum(axis=0, keepdims=True) for a in acc]


def _kernel(x_hbm, c_hbm, wqkv_hbm, wo_hbm, w1_hbm, w3_hbm, w2_hbm, wmod_hbm, o_ref,
            x_v, c_v, wqkv_raw, wqkv_p, wo_raw, wo_p, w1_v, w3_v, w2_v, wmod_v, mod_v, st_v,
            xn_s, wcur_s, h1_s, h_s, q0_s, k0_s, v0_s, q_s, k_s, v_s, o_s, flag_s, sems):
    step = pl.program_id(0)

    def new_chain():
        return _Chain(jax.lax.broadcasted_iota(jnp.int32, (8, 128), 1) < flag_s[0])

    def cp_x(i):
        n = TM if i < 4 else 4 * TM
        return pltpu.make_async_copy(x_hbm.at[pl.ds(i * TM, n)], x_v.at[pl.ds(i * TM, n)],
                                     sems.at[SEM_X + i])

    def cp_wq(k):
        rows = pl.ds(k * KC, KC)
        return pltpu.make_async_copy(wqkv_hbm.at[rows], wqkv_raw.at[rows], sems.at[SEM_WQ + k])

    def cp_wmod(col, n, sem):
        cols = pl.ds(col, n)
        return pltpu.make_async_copy(wmod_hbm.at[:, cols], wmod_v.at[:, cols], sems.at[sem])

    cp_ws = lambda k: cp_wmod(k * KC, KC, SEM_WS + k)
    cp_wc = lambda k: cp_wmod(D + k * KC, KC, SEM_WC + k)
    cp_wm = lambda p: cp_wmod((2 + p) * D, D, SEM_WM + p)

    def cp_wo(i):
        cols = pl.ds(0, 256) if i == 0 else pl.ds(256, D - 256)
        return pltpu.make_async_copy(wo_hbm.at[:, cols], wo_raw.at[:, cols], sems.at[SEM_WO + i])

    cp_c = lambda: pltpu.make_async_copy(c_hbm, c_v, sems.at[SEM_C])
    cp_w1 = lambda: pltpu.make_async_copy(w1_hbm, w1_v, sems.at[SEM_FF])
    cp_w3 = lambda: pltpu.make_async_copy(w3_hbm, w3_v, sems.at[SEM_FF + 1])
    cp_w2 = lambda: pltpu.make_async_copy(w2_hbm, w2_v, sems.at[SEM_FF + 2])

    def ln1_next(r0, chains, extra=None):
        sa = mod_v[0:1, 0 * D:1 * D]
        ca1 = 1.0 + mod_v[0:1, 1 * D:2 * D]
        for i, r in enumerate(range(0, TM, LNR)):
            chain = chains[i % len(chains)]
            x = chain.after_rows(x_v[pl.ds(r0 + r, LNR), :].astype(f32))
            h = _modulated_ln(x, ca1, sa)
            chain.tok = _pack(h[:, 0:128])
            h_s[pl.ds(r, LNR), :] = h
            if extra is not None:
                extra(i)

    tile0_dst = ((q0_s, 0), (k0_s, HALO), (v0_s, HALO))
    rest_dst = ((q_s, 0), (k_s, HALO), (v_s, HALO))

    @_when(step == 0, 'first')
    def _first():
        order = [cp_c(), cp_wq(0), cp_x(0), cp_ws(0), cp_wc(0), cp_x(1)]
        for k in range(1, NKC):
            order += [cp_wq(k), cp_ws(k), cp_wc(k)]
        order += [cp_x(2), cp_x(3), cp_wo(0), cp_wm(0), cp_x(4), cp_wo(1), cp_wm(1), cp_wm(2),
                  cp_wm(3), cp_w1(), cp_w3(), cp_w2()]
        for cp in order:
            cp.start()
        flag_s[0] = 128

        for dst, off in rest_dst:
            dst[:, pl.ds(off, TM), :] = jnp.zeros((NG, TM, 128), f32)
        cp_c().wait()
        c = c_v[...].astype(f32)
        sc = c * jax.nn.sigmoid(c)
        st_v[...] = jnp.transpose(jnp.broadcast_to(sc, (128, D)))

        def normalize(t):
            for r0 in range(t * TM, (t + 1) * TM, LNR):
                x = x_v[pl.ds(r0, LNR), :].astype(f32)
                r, mr = _ln_stats(x)
                xn = x * r - mr
                for g in range(NG):
                    xn_s[g, pl.ds(r0, LNR), :] = xn[:, g * 128:(g + 1) * 128]

        def mod_chunk(k):
            col = k * KC if isinstance(k, int) else pl.multiple_of(k * KC, KC)
            sa, ca = _mod_cols(wmod_v, st_v, [col, D + col], KC)
            mod_v[:, pl.ds(col, KC)] = jnp.broadcast_to(sa, (8, KC))
            mod_v[:, pl.ds(D + col, KC)] = jnp.broadcast_to(ca, (8, KC))
            return sa, 1.0 + ca

        def h_chunk(k, t, sa, ca1):
            return (xn_s[k, pl.ds(t * TM, TM), :] * ca1 + sa).astype(bf16)

        def mm(h, w, sec, dsts, first):
            res = jnp.dot(h, _unpack(w), preferred_element_type=f32)
            dst, off = dsts[sec]
            for g in range(NG):
                blk = res[:, g * 128:(g + 1) * 128]
                if first:
                    dst[g, pl.ds(off, TM), :] = blk
                else:
                    dst[g, pl.ds(off, TM), :] += blk

        def keep(k, sec, wp):
            r0 = k * (KC // 2) if isinstance(k, int) else pl.multiple_of(k * (KC // 2), KC // 2)
            wcur_s[:, sec * D:(sec + 1) * D] = wp
            wqkv_p[pl.ds(r0, KC // 2), sec * D:(sec + 1) * D] = wp

        scope = jax.named_scope
        with scope('w_wq0'):
            cp_wq(0).wait()
        with scope('perm0'):
            for sec in range(3):
                keep(0, sec, _permute_qkv_section(wqkv_raw, 0, sec))
        with scope('w_x0'):
            cp_x(0).wait()
        with scope('norm0'):
            normalize(0)
        with scope('w_m0'):
            cp_ws(0).wait()
            cp_wc(0).wait()
        with scope('mm0'):
            sa, ca1 = mod_chunk(0)
            h0 = h_chunk(0, 0, sa, ca1)
            for sec in range(3):
                mm(h0, wcur_s[:, sec * D:(sec + 1) * D], sec, tile0_dst, True)
        with scope('w_x1'):
            cp_x(1).wait()
        with scope('norm1'):
            normalize(1)
            h1_s[...] = _pack(h_chunk(0, 1, mod_v[0:1, 0:KC], 1.0 + mod_v[0:1, D:D + KC]))

        def chunk_body(k0, carry):
            k = k0 + 1
            with scope('w_chunk'):
                cp_wq(k).wait()
                cp_ws(k).wait()
                cp_wc(k).wait()
            with scope('chunk'):
                h1 = _unpack(h1_s[...])
                for sec in range(3):
                    mm(h1, wcur_s[:, sec * D:(sec + 1) * D], sec, rest_dst, False)
                sa, ca1 = mod_chunk(k)
                h0 = h_chunk(k, 0, sa, ca1)
                h1_s[...] = _pack(h_chunk(k, 1, sa, ca1))
                for sec in range(3):
                    wp = _permute_qkv_section(wqkv_raw, pl.multiple_of(k * KC, KC), sec)
                    mm(h0, wp, sec, tile0_dst, False)
                    keep(k, sec, wp)
            return carry
        jax.lax.fori_loop(0, NKC - 1, chunk_body, 0)

        with scope('w_x2'):
            cp_x(2).wait()
        h1 = _unpack(h1_s[...])
        for sec in range(3):
            mm(h1, wcur_s[:, sec * D:(sec + 1) * D], sec, rest_dst, False)
        ln1_next(2 * TM, [new_chain() for _ in range(4)])
        k0_s[:, 0:HALO, :] = jnp.zeros((NG, HALO, 128), f32)
        v0_s[:, 0:HALO, :] = jnp.broadcast_to(v0_s[:, HALO:HALO + 1, :], (NG, HALO, 128))
        k_s[:, 0:HALO, :] = k0_s[:, TM:TM + HALO, :]
        v_s[:, 0:HALO, :] = v0_s[:, TM:TM + HALO, :]

    @_when(step == 1, 'wait1')
    def _():
        cp_x(3).wait()
        cp_wo(0).wait()
        cp_wm(0).wait()

    @_when(step == 2, 'wait2')
    def _():
        cp_x(4).wait()

    @_when(step == 4, 'wait4')
    def _():
        cp_wo(1).wait()
        cp_wm(1).wait()

    @_when(step == 5, 'wait5')
    def _():
        cp_wm(2).wait()

    @_when(step == 6, 'wait6')
    def _():
        cp_wm(3).wait()

    @_when(jnp.logical_and(step >= 1, step < N1), 'phase1')
    def _phase1():
        part = jnp.maximum(step - 3, 0)
        base = pl.multiple_of(step * TM, TM)
        h = h_s[...]
        for sec, (dst, off) in enumerate(rest_dst):
            res = jnp.dot(h, _unpack(wqkv_p[:, sec * D:(sec + 1) * D]), preferred_element_type=f32)
            for g in range(NG):
                dst[g, pl.ds(base + off, TM), :] = res[:, g * 128:(g + 1) * 128]
        chain = new_chain()

        def wo_unit(i):
            gg, mid = i // 8, i % 8
            col = pl.ds(pl.multiple_of(part * 256 + gg * 128, 128), 128)
            a = [_pack(wo_raw[pl.ds(c * 128 + mid * 16, 16), col]) for c in range(8)]
            a[0] = chain.after(a[0])
            for k in range(3):
                a = _swap_stage(a, k, k, 0)
            for s in range(8):
                wo_p[pl.ds(s * 64 + mid * 8, 8), col] = a[s]
            chain.tok = a[7]

        ln1_next(pl.multiple_of(jnp.minimum(step + 2, NT - 1) * TM, TM), [chain], wo_unit)
        for c0 in range(0, D, 256):
            col = pl.multiple_of((2 + part) * D + c0, 256)
            val, = _mod_cols(wmod_v, st_v, [col], 256, chain)
            mod_v[:, pl.ds(col, 256)] = jnp.broadcast_to(val, (8, 256))
        r0 = pl.multiple_of(part * 64, 64)
        _attention(q0_s, k0_s, v0_s, o_s, r0, pl.multiple_of(part * 32, 32), 64, row0=r0)

    @_when(step == N1, 'wait7')
    def _():
        cp_w1().wait()
        cp_w3().wait()
        cp_w2().wait()

    @_when(step >= N1, 'phase2')
    def _phase2():
        j2 = step - N1
        ga = mod_v[0:1, 2 * D:3 * D]
        sb = mod_v[0:1, 3 * D:4 * D]
        cb1 = 1.0 + mod_v[0:1, 4 * D:5 * D]
        gb = mod_v[0:1, 5 * D:6 * D]
        row0 = pl.multiple_of(j2 * TM, TM)
        nsub = TM // SUB
        os_ = [_unpack(o_s[pl.ds(s * SUB // 2, SUB // 2), :]) for s in range(nsub)]
        x1s, h2s = [], []
        for s in range(nsub):
            att = jnp.dot(os_[s], _unpack(wo_p[...]), preferred_element_type=f32)
            x1 = x_v[pl.ds(row0 + s * SUB, SUB), :].astype(f32) + ga * att
            x1s.append(x1)
            h2s.append(jnp.concatenate(
                [_modulated_ln(x1[r:r + LNR], cb1, sb) for r in range(0, SUB, LNR)], axis=0))

        nq = pl.multiple_of(jnp.minimum(j2, NT - 2) * TM, TM)
        _attention(q_s, k_s, v_s, o_s, nq, 0, TM)

        def gate_up(h2, j):
            g = jnp.dot(h2, w1_v[:, j * FC:(j + 1) * FC], preferred_element_type=f32)
            u = jnp.dot(h2, w3_v[:, j * FC:(j + 1) * FC], preferred_element_type=f32)
            hg = 0.5 * g
            return ((hg + hg * jnp.tanh(hg)) * u).astype(bf16)

        def down(a, j):
            return jnp.dot(a, w2_v[j * FC:(j + 1) * FC, :], preferred_element_type=f32)

        a0 = jnp.concatenate([gate_up(h2s[s], 0) for s in range(nsub)], axis=0)
        h2 = jnp.concatenate(h2s, axis=0)
        acc = down(a0, 0)
        for j in range(1, F // FC):
            acc = acc + down(gate_up(h2, j), j)
        o_ref[...] = (jnp.concatenate(x1s, axis=0) + gb * acc).astype(o_ref.dtype)


@jax.jit
def pallas_adaLN_cond__sliding_local_dilated__glu_gated_swiglu__prompt_kernel(
    A_x: jax.Array,
    A_wqkv: jax.Array,
    A_wo: jax.Array,
    B_x: jax.Array,
    B_w1: jax.Array,
    B_w3: jax.Array,
    B_w2: jax.Array,
    c: jax.Array,
    w_mod: jax.Array,
):
    del B_x
    x = A_x.reshape(S, D)
    hbm = pl.BlockSpec(memory_space=pl.ANY)
    out = pl.pallas_call(
        _kernel,
        grid=(N1 + NT,),
        in_specs=[hbm] * 8,
        out_specs=pl.BlockSpec((TM, D), lambda i: (jnp.maximum(i - N1, 0), 0)),
        out_shape=jax.ShapeDtypeStruct((S, D), A_x.dtype),
        scratch_shapes=[
            pltpu.VMEM((S, D), bf16),
            pltpu.VMEM((1, D), bf16),
            pltpu.VMEM((D, 3 * D), bf16),
            pltpu.VMEM((D // 2, 3 * D), u32),
            pltpu.VMEM((D, D), bf16),
            pltpu.VMEM((D // 2, D), u32),
            pltpu.VMEM((D, F), bf16),
            pltpu.VMEM((D, F), bf16),
            pltpu.VMEM((F, D), bf16),
            pltpu.VMEM((D, 6 * D), bf16),
            pltpu.VMEM((8, 6 * D), f32),
            pltpu.VMEM((D, 128), f32),
            pltpu.VMEM((NG, 2 * TM, 128), f32),
            pltpu.VMEM((KC // 2, 3 * D), u32),
            pltpu.VMEM((TM // 2, KC), u32),
            pltpu.VMEM((TM, D), bf16),
            pltpu.VMEM((NG, TM, 128), f32),
            pltpu.VMEM((NG, HALO + TM, 128), f32),
            pltpu.VMEM((NG, HALO + TM, 128), f32),
            pltpu.VMEM((NG, S - TM, 128), f32),
            pltpu.VMEM((NG, HALO + S - TM, 128), f32),
            pltpu.VMEM((NG, HALO + S - TM, 128), f32),
            pltpu.VMEM((TM // 2, D), u32),
            pltpu.SMEM((1,), jnp.int32),
            pltpu.SemaphoreType.DMA((NSEM,)),
        ],
        compiler_params=pltpu.CompilerParams(
            dimension_semantics=("arbitrary",),
            vmem_limit_bytes=110 * 1024 * 1024,
        ),
        name="adaln_attn_ffn",
    )(x, c, A_wqkv, A_wo, B_w1, B_w3, B_w2, w_mod)
    return out.reshape(1, S, D)
```

```python
import jax
import jax.numpy as jnp
import jax.experimental.pallas as pl
import jax.experimental.pallas.tpu as pltpu

S, D, F = 2048, 1024, 3584
H, DH, W, DIL = 32, 32, 8, 2
NG = D // 128
TM = 256
NT = S // TM
N1 = NT - 1
SUB = 64
FC = 512
KC = 128
NKC = D // KC
HALO = 16
LNR = 16
EPS = 1e-5
SCALE = DH ** -0.5
LOG2E = 1.4426950408889634
QSCALE = SCALE * LOG2E
NEG = -1000000000.0 * LOG2E

f32 = jnp.float32
bf16 = jnp.bfloat16
u32 = jnp.uint32

SEM_C = 0
SEM_X = 1
SEM_WQ = 6
SEM_WS = SEM_WQ + NKC
SEM_WC = SEM_WS + NKC
SEM_WM = SEM_WC + NKC
SEM_WO = SEM_WM + 4
SEM_FF = SEM_WO + 2
NSEM = SEM_FF + 3


def _when(cond, name):
    def deco(body):
        def scoped():
            with jax.named_scope(name):
                body()
        return pl.when(cond)(scoped)
    return deco


def _pack(x):
    return pltpu.bitcast(x, u32)


def _unpack(x):
    return pltpu.bitcast(x, bf16)


class _Chain:
    def __init__(self, always):
        self.always = always
        self.tok = None

    def after(self, x):
        if self.tok is None:
            return x
        t = self.tok if self.tok.dtype == x.dtype else pltpu.bitcast(self.tok, x.dtype)
        return jnp.where(self.always, x, t)

    def after_rows(self, x):
        x00 = self.after(x[0:8, 0:128])
        return jnp.concatenate([jnp.concatenate([x00, x[0:8, 128:]], axis=1), x[8:]], axis=0)


def _swap_stage(a, k, b, axis):
    n = 128 if axis == 1 else 8
    idx = jax.lax.broadcasted_iota(jnp.int32, a[0].shape, axis)
    m0 = (idx & (1 << b)) == 0
    out = list(a)
    for c in range(8):
        if c & (1 << k):
            continue
        lo, hi = a[c], a[c | (1 << k)]
        out[c] = jnp.where(m0, lo, pltpu.roll(hi, 1 << b, axis))
        out[c | (1 << k)] = jnp.where(m0, pltpu.roll(lo, n - (1 << b), axis), hi)
    return out


def _permute_qkv_section(w_ref, r0, sec):
    a = [_pack(w_ref[pl.ds(r0, KC), pl.ds(sec * D + c * 128, 128)]) for c in range(8)]
    for k in range(3):
        a = _swap_stage(a, k, k + 1, 1)
    return jnp.concatenate(a, axis=1)


def _ln_stats(x):
    m = jnp.mean(x, axis=-1, keepdims=True)
    xc = x - m
    v = jnp.mean(xc * xc, axis=-1, keepdims=True)
    r = jax.lax.rsqrt(v + EPS)
    return r, m * r


def _modulated_ln(x, scale1, shift):
    r, mr = _ln_stats(x)
    return ((x * r - mr) * scale1 + shift).astype(bf16)


def _attention_rows(q_s, k_s, v_s, q0, row0):
    lane = jax.lax.broadcasted_iota(jnp.int32, (8, 128), 1)
    m0 = (lane & 1) == 0
    m4 = (lane & 16) == 0
    q = [q_s[g, pl.ds(q0, 8), :] * QSCALE for g in range(NG)]
    logits = []
    for w in range(W):
        z = None
        for g in range(NG):
            p = q[g] * k_s[g, pl.ds(q0 + (HALO - DIL * w), 8), :]
            z = p if z is None else z + p
        z = z + jnp.where(m0, pltpu.roll(z, 127, 1), pltpu.roll(z, 1, 1))
        z = z + jnp.where(m4, pltpu.roll(z, 112, 1), pltpu.roll(z, 16, 1))
        if w > 0 and row0 is not None:
            row = jax.lax.broadcasted_iota(jnp.int32, (8, 128), 0) + row0
            z = jnp.where(row >= DIL * w, z, NEG)
        logits.append(z)
    m = logits[0]
    for w in range(1, W):
        m = jnp.maximum(m, logits[w])
    e = [jnp.exp2(logits[w] - m) for w in range(W)]
    den = e[0]
    for w in range(1, W):
        den = den + e[w]
    inv = pl.reciprocal(den, approx=False)
    outs = []
    for g in range(NG):
        o = None
        for w in range(W):
            p = e[w] * v_s[g, pl.ds(q0 + (HALO - DIL * w), 8), :]
            o = p if o is None else o + p
        outs.append(o * inv)
    return jnp.concatenate(outs, axis=1)


def _attention(q_s, k_s, v_s, o_s, q0, o0, nrows, row0=None):
    for r in range(0, nrows, 8):
        o = _attention_rows(q_s, k_s, v_s, q0 + r,
                            None if (row0 is None or r >= HALO) else row0 + r)
        o_s[pl.ds(o0 + r, 8), :] = o.astype(bf16)


def _mod_cols(wmod_v, st_v, cols, n, chain=None):
    acc = [None] * len(cols)
    for r in range(0, D, 8):
        s = st_v[r:r + 8, :]
        if r == 0 and chain is not None:
            s = chain.after(s)
        if n > 128:
            s = jnp.concatenate([s] * (n // 128), axis=1)
        for i, col in enumerate(cols):
            p = wmod_v[r:r + 8, pl.ds(col, n)].astype(f32) * s
            acc[i] = p if acc[i] is None else acc[i] + p
    if chain is not None:
        chain.tok = acc[0][:, 0:128]
    return [a.sum(axis=0, keepdims=True) for a in acc]


def _kernel(x_hbm, c_hbm, wqkv_hbm, wo_hbm, w1_hbm, w3_hbm, w2_hbm, wmod_hbm, o_ref,
            x_v, wqkv_raw, wqkv_p, wo_raw, wo_p, w1_v, w3_v, w2_v, wmod_v, mod_v, st_v,
            xn_s, wcur_s, h1_s, h_s, q0_s, k0_s, v0_s, q_s, k_s, v_s, o_s, c_v, flag_s, sems):
    step = pl.program_id(0)

    def new_chain():
        return _Chain(jax.lax.broadcasted_iota(jnp.int32, (8, 128), 1) < flag_s[0])

    def cp_x(i):
        n = TM if i < 4 else 4 * TM
        return pltpu.make_async_copy(x_hbm.at[pl.ds(i * TM, n)], x_v.at[pl.ds(i * TM, n)],
                                     sems.at[SEM_X + i])

    def cp_wq(k):
        rows = pl.ds(k * KC, KC)
        return pltpu.make_async_copy(wqkv_hbm.at[rows], wqkv_raw.at[rows], sems.at[SEM_WQ + k])

    def cp_wmod(col, n, sem):
        cols = pl.ds(col, n)
        return pltpu.make_async_copy(wmod_hbm.at[:, cols], wmod_v.at[:, cols], sems.at[sem])

    cp_ws = lambda k: cp_wmod(k * KC, KC, SEM_WS + k)
    cp_wc = lambda k: cp_wmod(D + k * KC, KC, SEM_WC + k)
    cp_wm = lambda p: cp_wmod((2 + p) * D, D, SEM_WM + p)

    def cp_wo(i):
        cols = pl.ds(0, 256) if i == 0 else pl.ds(256, D - 256)
        return pltpu.make_async_copy(wo_hbm.at[:, cols], wo_raw.at[:, cols], sems.at[SEM_WO + i])

    cp_c = lambda: pltpu.make_async_copy(c_hbm, c_v, sems.at[SEM_C])
    cp_w1 = lambda: pltpu.make_async_copy(w1_hbm, w1_v, sems.at[SEM_FF])
    cp_w3 = lambda: pltpu.make_async_copy(w3_hbm, w3_v, sems.at[SEM_FF + 1])
    cp_w2 = lambda: pltpu.make_async_copy(w2_hbm, w2_v, sems.at[SEM_FF + 2])

    def ln1_next(r0, chains, extra=None):
        sa = mod_v[0:1, 0 * D:1 * D]
        ca1 = 1.0 + mod_v[0:1, 1 * D:2 * D]
        for i, r in enumerate(range(0, TM, LNR)):
            chain = chains[i % len(chains)]
            x = chain.after_rows(x_v[pl.ds(r0 + r, LNR), :].astype(f32))
            h = _modulated_ln(x, ca1, sa)
            chain.tok = _pack(h[:, 0:128])
            h_s[pl.ds(r, LNR), :] = h
            if extra is not None:
                extra(i)

    tile0_dst = ((q0_s, 0), (k0_s, HALO), (v0_s, HALO))
    rest_dst = ((q_s, 0), (k_s, HALO), (v_s, HALO))

    @_when(step == 0, 'first')
    def _first():
        order = [cp_c(), cp_wq(0), cp_x(0), cp_ws(0), cp_wc(0), cp_x(1)]
        for k in range(1, NKC):
            order += [cp_wq(k), cp_ws(k), cp_wc(k)]
        order += [cp_x(2), cp_x(3), cp_wo(0), cp_wm(0), cp_x(4), cp_wo(1), cp_wm(1), cp_wm(2),
                  cp_wm(3), cp_w1(), cp_w3(), cp_w2()]
        for cp in order:
            cp.start()
        flag_s[0] = 128

        for dst, off in rest_dst:
            dst[:, pl.ds(off, TM), :] = jnp.zeros((NG, TM, 128), f32)
        cp_c().wait()
        c = c_v[...].astype(f32)
        sc = c * jax.nn.sigmoid(c)
        st_v[...] = jnp.transpose(jnp.broadcast_to(sc, (128, D)))

        def normalize(t):
            for r0 in range(t * TM, (t + 1) * TM, LNR):
                x = x_v[pl.ds(r0, LNR), :].astype(f32)
                r, mr = _ln_stats(x)
                xn = x * r - mr
                for g in range(NG):
                    xn_s[g, pl.ds(r0, LNR), :] = xn[:, g * 128:(g + 1) * 128]

        def mod_chunk(k):
            col = k * KC if isinstance(k, int) else pl.multiple_of(k * KC, KC)
            sa, ca = _mod_cols(wmod_v, st_v, [col, D + col], KC)
            mod_v[:, pl.ds(col, KC)] = jnp.broadcast_to(sa, (8, KC))
            mod_v[:, pl.ds(D + col, KC)] = jnp.broadcast_to(ca, (8, KC))
            return sa, 1.0 + ca

        def h_chunk(k, t, sa, ca1):
            return (xn_s[k, pl.ds(t * TM, TM), :] * ca1 + sa).astype(bf16)

        def mm(h, w, sec, dsts, first):
            res = jnp.dot(h, _unpack(w), preferred_element_type=f32)
            dst, off = dsts[sec]
            for g in range(NG):
                blk = res[:, g * 128:(g + 1) * 128]
                if first:
                    dst[g, pl.ds(off, TM), :] = blk
                else:
                    dst[g, pl.ds(off, TM), :] += blk

        def keep(k, sec, wp):
            r0 = k * (KC // 2) if isinstance(k, int) else pl.multiple_of(k * (KC // 2), KC // 2)
            wcur_s[:, sec * D:(sec + 1) * D] = wp
            wqkv_p[pl.ds(r0, KC // 2), sec * D:(sec + 1) * D] = wp

        scope = jax.named_scope
        with scope('w_wq0'):
            cp_wq(0).wait()
        with scope('perm0'):
            for sec in range(3):
                keep(0, sec, _permute_qkv_section(wqkv_raw, 0, sec))
        with scope('w_x0'):
            cp_x(0).wait()
        with scope('norm0'):
            normalize(0)
        with scope('w_m0'):
            cp_ws(0).wait()
            cp_wc(0).wait()
        with scope('mm0'):
            sa, ca1 = mod_chunk(0)
            h0 = h_chunk(0, 0, sa, ca1)
            for sec in range(3):
                mm(h0, wcur_s[:, sec * D:(sec + 1) * D], sec, tile0_dst, True)
        with scope('w_x1'):
            cp_x(1).wait()
        with scope('norm1'):
            normalize(1)
            h1_s[...] = _pack(h_chunk(0, 1, mod_v[0:1, 0:KC], 1.0 + mod_v[0:1, D:D + KC]))

        def chunk_body(k0, carry):
            k = k0 + 1
            with scope('w_chunk'):
                cp_wq(k).wait()
                cp_ws(k).wait()
                cp_wc(k).wait()
            with scope('chunk'):
                h1 = _unpack(h1_s[...])
                for sec in range(3):
                    mm(h1, wcur_s[:, sec * D:(sec + 1) * D], sec, rest_dst, False)
                sa, ca1 = mod_chunk(k)
                h0 = h_chunk(k, 0, sa, ca1)
                h1_s[...] = _pack(h_chunk(k, 1, sa, ca1))
                for sec in range(3):
                    wp = _permute_qkv_section(wqkv_raw, pl.multiple_of(k * KC, KC), sec)
                    mm(h0, wp, sec, tile0_dst, False)
                    keep(k, sec, wp)
            return carry
        jax.lax.fori_loop(0, NKC - 1, chunk_body, 0)

        with scope('w_x2'):
            cp_x(2).wait()
        h1 = _unpack(h1_s[...])
        for sec in range(3):
            mm(h1, wcur_s[:, sec * D:(sec + 1) * D], sec, rest_dst, False)
        ln1_next(2 * TM, [new_chain() for _ in range(4)])
        k0_s[:, 0:HALO, :] = jnp.zeros((NG, HALO, 128), f32)
        v0_s[:, 0:HALO, :] = jnp.broadcast_to(v0_s[:, HALO:HALO + 1, :], (NG, HALO, 128))
        k_s[:, 0:HALO, :] = k0_s[:, TM:TM + HALO, :]
        v_s[:, 0:HALO, :] = v0_s[:, TM:TM + HALO, :]

    @_when(step == 1, 'wait1')
    def _():
        cp_x(3).wait()
        cp_wo(0).wait()
        cp_wm(0).wait()

    @_when(step == 2, 'wait2')
    def _():
        cp_x(4).wait()

    @_when(step == 4, 'wait4')
    def _():
        cp_wo(1).wait()
        cp_wm(1).wait()

    @_when(step == 5, 'wait5')
    def _():
        cp_wm(2).wait()

    @_when(step == 6, 'wait6')
    def _():
        cp_wm(3).wait()

    @_when(jnp.logical_and(step >= 1, step < N1), 'phase1')
    def _phase1():
        part = jnp.maximum(step - 3, 0)
        base = pl.multiple_of(step * TM, TM)
        h = h_s[...]
        for sec, (dst, off) in enumerate(rest_dst):
            res = jnp.dot(h, _unpack(wqkv_p[:, sec * D:(sec + 1) * D]), preferred_element_type=f32)
            for g in range(NG):
                dst[g, pl.ds(base + off, TM), :] = res[:, g * 128:(g + 1) * 128]
        chain = new_chain()

        def wo_unit(i):
            gg, mid = i // 8, i % 8
            col = pl.ds(pl.multiple_of(part * 256 + gg * 128, 128), 128)
            a = [_pack(wo_raw[pl.ds(c * 128 + mid * 16, 16), col]) for c in range(8)]
            a[0] = chain.after(a[0])
            for k in range(3):
                a = _swap_stage(a, k, k, 0)
            for s in range(8):
                wo_p[pl.ds(s * 64 + mid * 8, 8), col] = a[s]
            chain.tok = a[7]

        ln1_next(pl.multiple_of(jnp.minimum(step + 2, NT - 1) * TM, TM), [chain], wo_unit)
        for c0 in range(0, D, 256):
            col = pl.multiple_of((2 + part) * D + c0, 256)
            val, = _mod_cols(wmod_v, st_v, [col], 256, chain)
            mod_v[:, pl.ds(col, 256)] = jnp.broadcast_to(val, (8, 256))
        r0 = pl.multiple_of(part * 64, 64)
        _attention(q0_s, k0_s, v0_s, o_s, r0, r0, 64, row0=r0)

    @_when(step == N1, 'wait7')
    def _():
        cp_w1().wait()
        cp_w3().wait()
        cp_w2().wait()

    @_when(step >= N1, 'phase2')
    def _phase2():
        j2 = step - N1
        ga = mod_v[0:1, 2 * D:3 * D]
        sb = mod_v[0:1, 3 * D:4 * D]
        cb1 = 1.0 + mod_v[0:1, 4 * D:5 * D]
        gb = mod_v[0:1, 5 * D:6 * D]
        row0 = pl.multiple_of(j2 * TM, TM)
        nsub = TM // SUB
        os_ = [o_s[pl.ds(s * SUB, SUB), :] for s in range(nsub)]
        x1s, h2s = [], []
        for s in range(nsub):
            att = jnp.dot(os_[s], _unpack(wo_p[...]), preferred_element_type=f32)
            x1 = x_v[pl.ds(row0 + s * SUB, SUB), :].astype(f32) + ga * att
            x1s.append(x1)
            chain = new_chain()
            parts = []
            for r in range(0, SUB, LNR):
                h = _modulated_ln(chain.after_rows(x1[r:r + LNR]), cb1, sb)
                chain.tok = _pack(h[:, 0:128])
                parts.append(h)
            h2s.append(jnp.concatenate(parts, axis=0))

        nq = pl.multiple_of(jnp.minimum(j2, NT - 2) * TM, TM)
        _attention(q_s, k_s, v_s, o_s, nq, 0, TM)

        def gate_up(h2, j):
            g = jnp.dot(h2, w1_v[:, j * FC:(j + 1) * FC], preferred_element_type=f32)
            u = jnp.dot(h2, w3_v[:, j * FC:(j + 1) * FC], preferred_element_type=f32)
            hg = 0.5 * g
            return ((hg + hg * jnp.tanh(hg)) * u).astype(bf16)

        def down(a, j):
            return jnp.dot(a, w2_v[j * FC:(j + 1) * FC, :], preferred_element_type=f32)

        a0 = jnp.concatenate([gate_up(h2s[s], 0) for s in range(nsub)], axis=0)
        h2 = jnp.concatenate(h2s, axis=0)
        acc = down(a0, 0)
        for j in range(1, F // FC):
            acc = acc + down(gate_up(h2, j), j)
        o_ref[...] = (jnp.concatenate(x1s, axis=0) + gb * acc).astype(o_ref.dtype)


@jax.jit
def pallas_adaLN_cond__sliding_local_dilated__glu_gated_swiglu__prompt_kernel(
    A_x: jax.Array,
    A_wqkv: jax.Array,
    A_wo: jax.Array,
    B_x: jax.Array,
    B_w1: jax.Array,
    B_w3: jax.Array,
    B_w2: jax.Array,
    c: jax.Array,
    w_mod: jax.Array,
):
    del B_x
    x = A_x.reshape(S, D)
    hbm = pl.BlockSpec(memory_space=pl.ANY)
    out = pl.pallas_call(
        _kernel,
        grid=(N1 + NT,),
        in_specs=[hbm] * 8,
        out_specs=pl.BlockSpec((TM, D), lambda i: (jnp.maximum(i - N1, 0), 0)),
        out_shape=jax.ShapeDtypeStruct((S, D), A_x.dtype),
        scratch_shapes=[
            pltpu.VMEM((S, D), bf16),
            pltpu.VMEM((D, 3 * D), bf16),
            pltpu.VMEM((D // 2, 3 * D), u32),
            pltpu.VMEM((D, D), bf16),
            pltpu.VMEM((D // 2, D), u32),
            pltpu.VMEM((D, F), bf16),
            pltpu.VMEM((D, F), bf16),
            pltpu.VMEM((F, D), bf16),
            pltpu.VMEM((D, 6 * D), bf16),
            pltpu.VMEM((8, 6 * D), f32),
            pltpu.VMEM((D, 128), f32),
            pltpu.VMEM((NG, 2 * TM, 128), f32),
            pltpu.VMEM((KC // 2, 3 * D), u32),
            pltpu.VMEM((TM // 2, KC), u32),
            pltpu.VMEM((TM, D), bf16),
            pltpu.VMEM((NG, TM, 128), f32),
            pltpu.VMEM((NG, HALO + TM, 128), f32),
            pltpu.VMEM((NG, HALO + TM, 128), f32),
            pltpu.VMEM((NG, S - TM, 128), f32),
            pltpu.VMEM((NG, HALO + S - TM, 128), f32),
            pltpu.VMEM((NG, HALO + S - TM, 128), f32),
            pltpu.VMEM((TM, D), bf16),
            pltpu.VMEM((1, D), bf16),
            pltpu.SMEM((1,), jnp.int32),
            pltpu.SemaphoreType.DMA((NSEM,)),
        ],
        compiler_params=pltpu.CompilerParams(
            dimension_semantics=("arbitrary",),
            vmem_limit_bytes=110 * 1024 * 1024,
        ),
        name="adaln_attn_ffn",
    )(x, c, A_wqkv, A_wo, B_w1, B_w3, B_w2, w_mod)
    return out.reshape(1, S, D)
```

```python
import jax
import jax.numpy as jnp
import jax.experimental.pallas as pl
import jax.experimental.pallas.tpu as pltpu

S, D, F = 2048, 1024, 3584
H, DH, W, DIL = 32, 32, 8, 2
NG = D // 128
TM = 256
NT = S // TM
T0 = 3
N1 = NT - T0 + 1
SUB = 64
HN = 256
FH = F // 2
DH2 = D // 2
KC = 128
NKC = D // KC
RU1 = 112
RU2 = 368
HALO = 16
PARTS = 'LMA'
SMODE = 'be'
EARLY = (0, 0)
PACE = 0
PK = 1
UR = 8
UC = 256
NW = 1
PULL0 = 2
SLINK = True
SW = 256
WB1 = 2
WB2 = 1
LNR = 16
EPS = 1e-5
SCALE = DH ** -0.5
LOG2E = 1.4426950408889634
QSCALE = SCALE * LOG2E
NEG = -1000000000.0 * LOG2E

f32 = jnp.float32
bf16 = jnp.bfloat16
u32 = jnp.uint32

SEM_C = 0
SEM_X = 1
SEM_WQ0 = SEM_X + NT
SEM_CH = SEM_WQ0 + 1
SEM_WM = SEM_CH + NKC
SEM_WO = SEM_WM + 4
SEM_FF = SEM_WO + 2
NSEM = SEM_FF + (N1 - 1)


def _when(cond, name):
    def deco(body):
        def scoped():
            with jax.named_scope(name):
                body()
        return pl.when(cond)(scoped)
    return deco


def _pack(x):
    return pltpu.bitcast(x, u32)


def _unpack(x):
    return pltpu.bitcast(x, bf16)


def _spack(x):
    return x if PK == 1 else _pack(x)


def _sunpack(x):
    return x if PK == 1 else _unpack(x)


def _dot(a, b):
    return jnp.dot(a, b, preferred_element_type=f32)


class _Chain:
    def __init__(self, always):
        self.always = always
        self.tok = None

    def after(self, x):
        if self.tok is None:
            return x
        t = self.tok if self.tok.dtype == x.dtype else pltpu.bitcast(self.tok, x.dtype)
        return jnp.where(self.always, x, t)

    def pace(self, done, n):
        t = done
        if self.tok is not None and n > 0:
            d = self.tok
            for _ in range(n):
                d = jnp.tanh(d)
            t = d + t
        self.tok = t

    def after_rows(self, x):
        x00 = self.after(x[0:8, 0:128])
        top = x00 if x.shape[1] == 128 else jnp.concatenate([x00, x[0:8, 128:]], axis=1)
        return top if x.shape[0] == 8 else jnp.concatenate([top, x[8:]], axis=0)


def _swap_stage(a, k, b, axis):
    n = 128 if axis == 1 else 8
    idx = jax.lax.broadcasted_iota(jnp.int32, a[0].shape, axis)
    m0 = (idx & (1 << b)) == 0
    out = list(a)
    for c in range(8):
        if c & (1 << k):
            continue
        lo, hi = a[c], a[c | (1 << k)]
        out[c] = jnp.where(m0, lo, pltpu.roll(hi, 1 << b, axis))
        out[c | (1 << k)] = jnp.where(m0, pltpu.roll(lo, n - (1 << b), axis), hi)
    return out


def _permute_qkv_section(w_ref, r0, sec):
    c0 = sec * D if isinstance(sec, int) else pl.multiple_of(sec * D, D)
    a = [_pack(w_ref[pl.ds(r0, KC), pl.ds(c0 + c * 128, 128)]) for c in range(8)]
    for k in range(3):
        a = _swap_stage(a, k, k + 1, 1)
    return jnp.concatenate(a, axis=1)


def _ln_stats(x):
    m = jnp.mean(x, axis=-1, keepdims=True)
    xc = x - m
    v = jnp.mean(xc * xc, axis=-1, keepdims=True)
    r = jax.lax.rsqrt(v + EPS)
    return r, m * r


def _modulated_ln(x, scale1, shift):
    r, mr = _ln_stats(x)
    return (x * r - mr) * scale1 + shift


def _attention_rows(q_s, k_s, v_s, q0, row0, wb, chain=None):
    lane = jax.lax.broadcasted_iota(jnp.int32, (8, 128), 1)
    m0 = (lane & 1) == 0
    m4 = (lane & 16) == 0
    qscale = QSCALE if chain is None else chain.after(jnp.full((8, 128), QSCALE, f32))
    q = [q_s[g, pl.ds(q0, 8), :] * qscale for g in range(NG)]
    logits = []
    for w0 in range(0, W, wb):
        zs = []
        for w in range(w0, w0 + wb):
            z = None
            for g in range(NG):
                p = q[g] * k_s[g, pl.ds(q0 + (HALO - DIL * w), 8), :]
                z = p if z is None else z + p
            zs.append(z)
        zs = [z + jnp.where(m0, pltpu.roll(z, 127, 1), pltpu.roll(z, 1, 1)) for z in zs]
        zs = [z + jnp.where(m4, pltpu.roll(z, 112, 1), pltpu.roll(z, 16, 1)) for z in zs]
        for w, z in zip(range(w0, w0 + wb), zs):
            if w > 0 and row0 is not None:
                row = jax.lax.broadcasted_iota(jnp.int32, (8, 128), 0) + row0
                z = jnp.where(row >= DIL * w, z, NEG)
            logits.append(z)
    m = logits[0]
    for w in range(1, W):
        m = jnp.maximum(m, logits[w])
    e = [jnp.exp2(logits[w] - m) for w in range(W)]
    den = e[0]
    for w in range(1, W):
        den = den + e[w]
    inv = pl.reciprocal(den, approx=False)
    outs = []
    for g in range(NG):
        o = None
        for w in range(W):
            p = e[w] * v_s[g, pl.ds(q0 + (HALO - DIL * w), 8), :]
            o = p if o is None else o + p
        outs.append(o * inv)
    if chain is not None:
        chain.tok = outs[-1]
    return jnp.concatenate(outs, axis=1)


def _attention(q_s, k_s, v_s, o_s, q0, o0, nrows, wb, row0=None):
    for r in range(0, nrows, 8):
        o = _attention_rows(q_s, k_s, v_s, q0 + r,
                            None if (row0 is None or r >= HALO) else row0 + r, wb)
        o_s[pl.ds(o0 + r, 8), :] = o.astype(bf16)


def _mod_cols(wmod_v, st_v, cols, n, chain=None):
    acc = [None] * len(cols)
    for r in range(0, D, 8):
        s = st_v[r:r + 8, :]
        if r == 0 and chain is not None:
            s = chain.after(s)
        if n > 128:
            s = jnp.concatenate([s] * (n // 128), axis=1)
        for i, col in enumerate(cols):
            p = wmod_v[r:r + 8, pl.ds(col, n)].astype(f32) * s
            acc[i] = p if acc[i] is None else acc[i] + p
    if chain is not None:
        chain.tok = acc[0][:, 0:128]
    return [a.sum(axis=0, keepdims=True) for a in acc]


def _lhs_operands(a11, a12, a21, a22):
    ops = (a11 + a22, a21 + a22, a11, a22, a11 + a12, a21 - a11, a12 - a22)
    return [v.astype(bf16) for v in ops]


def _rhs_sums(b11, b12, b21, b22):
    return (b11 + b22, b12 - b22, b21 - b11, b11 + b12, b21 + b22)


def _rhs_operands(sums, b11, b22):
    return [sums(0), b11, sums(1), sums(2), b22, sums(3), sums(4)]


def _combine(m):
    return (m[0] + m[3] - m[4] + m[6], m[2] + m[4], m[1] + m[3], m[0] - m[1] + m[2] + m[5])


def _new_chain(flag_s):
    return _Chain(jax.lax.broadcasted_iota(jnp.int32, (8, 128), 1) < flag_s[0])


def _ln1_next(x_v, mod_v, h_s, r0, chains, extra=None):
    sa = mod_v[0:1, 0 * D:1 * D]
    ca1 = 1.0 + mod_v[0:1, 1 * D:2 * D]
    for i, r in enumerate(range(0, TM, LNR)):
        chain = chains[i % len(chains)]
        x = chain.after_rows(x_v[pl.ds(r0 + r, LNR), :].astype(f32))
        h = _modulated_ln(x, ca1, sa)
        chain.tok = h[0:8, 0:128]
        h_s[pl.ds(r, LNR), :] = h.astype(bf16)
        if extra is not None:
            extra(i)


def _phase1(step, x_v, wqkv_p, wo_raw, wo_p, w1_v, w3_v, w2_v, s1_v, s3_v, s2_v, wmod_v, mod_v, st_v,
            h_s, q0_s, k0_s, v0_s, q_s, k_s, v_s, o_s, flag_s):
    step = jnp.clip(step, 1, N1 - 1)
    part = jnp.maximum(step - 2, 0)
    base = pl.multiple_of((step + T0 - 2) * TM, TM)
    h = h_s[...]
    chain = _new_chain(flag_s)

    ln_r0 = pl.multiple_of(jnp.minimum(step + T0, NT - 1) * TM, TM)
    sa = mod_v[0:1, 0 * D:1 * D]
    ca1 = 1.0 + mod_v[0:1, 1 * D:2 * D]

    def ln_unit(i):
        x = chain.after_rows(x_v[pl.ds(ln_r0 + i * LNR, LNR), :].astype(f32))
        hn = _modulated_ln(x, ca1, sa)
        chain.tok = hn[0:8, 0:128]
        h_s[pl.ds(i * LNR, LNR), :] = hn.astype(bf16)

    def wo_unit(i):
        gg, mid = i // 8, i % 8
        col = pl.ds(pl.multiple_of(part * 256 + gg * 128, 128), 128)
        a = [_pack(wo_raw[pl.ds(c * 128 + mid * 16, 16), col]) for c in range(8)]
        a[0] = chain.after(a[0])
        for k in range(3):
            a = _swap_stage(a, k, k, 0)
        for s in range(8):
            wo_p[pl.ds(s * 64 + mid * 8, 8), col] = a[s]
        chain.tok = a[7]

    at_r0 = pl.multiple_of(part * 64, 64)

    def attn_unit(i):
        o = _attention_rows(q0_s, k0_s, v0_s, at_r0 + i * 8,
                            at_r0 + i * 8 if i * 8 < HALO else None, WB1, chain)
        o_s[pl.ds(at_r0 + i * 8, 8), :] = o.astype(bf16)

    mod_col = pl.multiple_of(step * D, D)

    def mod_unit(i):
        col = pl.multiple_of(mod_col + i * 256, 256)
        val, = _mod_cols(wmod_v, st_v, [col], 256, chain)
        mod_v[:, pl.ds(col, 256)] = jnp.broadcast_to(val, (8, 256))

    sum_units = []
    for w_v, s_v, half, ru, ch in ((w1_v, s1_v, DH2, RU1, FH), (w3_v, s3_v, DH2, RU1, FH),
                                   (w2_v, s2_v, FH, RU2, DH2)):
        r_lo = jnp.minimum((step - 1) * (ru // 16), (half - ru) // 16)
        srcs = [w_v.at[pl.ds(pl.multiple_of(i * half + r_lo * 16, 16), ru)] for i in range(2)]
        dst = s_v.at[:, pl.ds(pl.multiple_of(r_lo * (16 // PK), 16 // PK), ru // PK)]
        r_bk = jnp.clip(r_lo + flag_s[0] - 128, 0, (half - ru) // 16)
        back = s_v.at[:, pl.ds(pl.multiple_of(r_bk * (16 // PK), 16 // PK), ru // PK)]
        sum_units += [(srcs, dst, back, ch, r, c0)
                      for r in range(0, ru, UR) for c0 in range(0, ch, UC)]

    def sum_unit(u):
        srcs, dst, back, ch, r, c0 = sum_units[u]
        q = [srcs[i][r:r + UR, j * ch + c0:j * ch + c0 + UC].astype(f32)
             for i in range(2) for j in range(2)]
        q[0] = chain.after_rows(q[0])
        for i, v in enumerate(_rhs_sums(*q)):
            dst[i, r // PK:(r + UR) // PK, c0:c0 + UC] = _spack(v.astype(bf16))
        bk = back[0, r // PK:r // PK + 8, c0:c0 + 128]
        chain.tok = bk.astype(f32) if PK == 1 else bk

    chain.tok = None
    for i in range(16):
        ln_unit(i)
        wo_unit(i)
    for i in range(4):
        mod_unit(i)
    for i in range(8):
        chain.tok = None
        attn_unit(i)

    npiece = 3 * NG // NW
    nsum = len(sum_units)
    done = 0
    chain.tok = None
    for t in range(npiece):
        upto = min(nsum, -(-nsum * max(t + 1 - PULL0, 0) // (npiece - PULL0)))
        if not SLINK:
            chain.tok = None
        for u in range(done, upto):
            sum_unit(u)
        sec, g0 = t * NW // NG, t * NW % NG
        dst, off = (q_s, k_s, v_s)[sec], (0 if sec == 0 else HALO)
        w = wqkv_p[:, t * NW * 128:(t + 1) * NW * 128]
        if upto > done:
            w = chain.after_rows(w)
        done = upto
        res = _dot(h, _unpack(w))
        for g in range(NW):
            dst[g0 + g, pl.ds(base + off, TM), :] = res[:, g * 128:(g + 1) * 128]


def _phase2(step, x_v, wo_p, w1_v, w3_v, w2_v, s1_v, s3_v, s2_v, mod_v, q_s, k_s, v_s, o_s, flag_s,
            o_ref):
    j2 = jnp.clip(step - N1, 0, NT - 1)
    ga = mod_v[0:1, 2 * D:3 * D]
    sb = mod_v[0:1, 3 * D:4 * D]
    cb1 = 1.0 + mod_v[0:1, 4 * D:5 * D]
    gb = mod_v[0:1, 5 * D:6 * D]
    row0 = pl.multiple_of(j2 * TM, TM)
    nsub = TM // SUB
    os_ = [o_s[pl.ds(s * SUB, SUB), :] for s in range(nsub)]
    x1s, h2s = [], []
    for s in range(nsub):
        att = _dot(os_[s], _unpack(wo_p[...]))
        x1 = x_v[pl.ds(row0 + s * SUB, SUB), :].astype(f32) + ga * att
        x1s.append(x1)
        chain = _new_chain(flag_s)
        parts = []
        for r in range(0, SUB, LNR):
            h = _modulated_ln(chain.after_rows(x1[r:r + LNR]), cb1, sb)
            chain.tok = h[0:8, 0:128]
            parts.append(h)
        h2s.append(jnp.concatenate(parts, axis=0))

    nq = pl.multiple_of(jnp.minimum(j2, NT - 2) * TM, TM)
    _attention(q_s, k_s, v_s, o_s, nq, 0, TM, WB2)

    groups = [_lhs_operands(h2s[2 * g][:, :DH2], h2s[2 * g][:, DH2:],
                            h2s[2 * g + 1][:, :DH2], h2s[2 * g + 1][:, DH2:])
              for g in range(nsub // 2)]

    def stack(per_group):
        return [jnp.concatenate([ops[i] for ops in per_group], axis=0) for i in range(7)]

    def up_proj(a, w_v, s_v, j):
        c0 = j * HN
        b = _rhs_operands(lambda i: _sunpack(s_v[i, :, c0:c0 + HN]),
                          w_v[0:DH2, c0:c0 + HN], w_v[DH2:, FH + c0:FH + c0 + HN])
        return _combine([_dot(a[i], b[i]) for i in range(7)])

    def gate_up(a, j):
        act = []
        for g, u in zip(up_proj(a, w1_v, s1_v, j), up_proj(a, w3_v, s3_v, j)):
            hg = 0.5 * g
            act.append((hg + hg * jnp.tanh(hg)) * u)
        return _lhs_operands(*act)

    h_all = stack(groups)
    acc = None
    for j in range(FH // HN):
        a = stack([gate_up(ops, 0) for ops in groups]) if j == 0 else gate_up(h_all, j)
        r0 = j * HN
        b = _rhs_operands(lambda i: _sunpack(s2_v[i, r0 // PK:(r0 + HN) // PK, :]),
                          w2_v[r0:r0 + HN, 0:DH2], w2_v[FH + r0:FH + r0 + HN, DH2:])
        m = [_dot(a[i], b[i]) for i in range(7)]
        acc = m if acc is None else [p + q for p, q in zip(acc, m)]
    c11, c12, c21, c22 = _combine(acc)
    for g in range(nsub // 2):
        rows = slice(g * SUB, (g + 1) * SUB)
        for t, (left, right) in enumerate(((c11, c12), (c21, c22))):
            y = jnp.concatenate([left[rows], right[rows]], axis=1)
            o_ref[pl.ds((2 * g + t) * SUB, SUB), :] = (
                x1s[2 * g + t] + gb * y).astype(o_ref.dtype)


def _kernel(x_hbm, c_hbm, wqkv_hbm, wo_hbm, w1_hbm, w3_hbm, w2_hbm, wmod_hbm, o_ref,
            x_v, wqkv_raw, wqkv_p, wo_raw, wo_p, w1_v, w3_v, w2_v, s1_v, s3_v, s2_v,
            wmod_v, mod_v, st_v, xn_s, wcur_s, hl_s, h_s, q0_s, k0_s, v0_s, q_s, k_s, v_s,
            o_s, c_v, flag_s, sems):
    step = pl.program_id(0)

    def new_chain():
        return _new_chain(flag_s)

    def cp_rows(src, dst, r0, n, sem):
        rows = pl.ds(r0, n)
        return pltpu.make_async_copy(src.at[rows], dst.at[rows], sems.at[sem])

    def cp_cols(src, dst, c0, n, sem):
        cols = pl.ds(c0, n)
        return pltpu.make_async_copy(src.at[:, cols], dst.at[:, cols], sems.at[sem])

    cp_c = lambda: [pltpu.make_async_copy(c_hbm, c_v, sems.at[SEM_C])]
    cp_x = lambda i: [cp_rows(x_hbm, x_v, i * TM, TM, SEM_X + i)]
    cp_wq0 = lambda: [cp_rows(wqkv_hbm, wqkv_raw, 0, KC, SEM_WQ0)]
    cp_wm = lambda p: [cp_cols(wmod_hbm, wmod_v, (2 + p) * D, D, SEM_WM + p)]

    def cp_chunk(k, with_wq=True):
        cps = [cp_rows(wqkv_hbm, wqkv_raw, k * KC, KC, SEM_CH + k)] if with_wq else []
        return cps + [cp_cols(wmod_hbm, wmod_v, k * KC, KC, SEM_CH + k),
                      cp_cols(wmod_hbm, wmod_v, D + k * KC, KC, SEM_CH + k)]

    def cp_wo(i):
        c0, n = (0, 256) if i == 0 else (256, D - 256)
        return [cp_cols(wo_hbm, wo_raw, c0, n, SEM_WO + i)]

    def cp_ff(i):
        cps = []
        for src, dst, half, ru in ((w1_hbm, w1_v, DH2, RU1), (w3_hbm, w3_v, DH2, RU1),
                                   (w2_hbm, w2_v, FH, RU2)):
            n = min(ru, half - i * ru)
            cps += [cp_rows(src, dst, h * half + i * ru, n, SEM_FF + i) for h in range(2)]
        return cps

    def wait(*groups):
        for cps in groups:
            for cp in cps:
                cp.wait()

    def qkv_dst(t, sec):
        off = 0 if sec == 0 else HALO
        if t == 0:
            return (q0_s, k0_s, v0_s)[sec], off
        return (q_s, k_s, v_s)[sec], off + (t - 1) * TM

    @_when(step == 0, 'first')
    def _first():
        order = cp_c() + cp_wq0() + cp_x(0) + cp_chunk(0, False) + cp_x(1) + cp_x(2)
        for k in range(1, NKC):
            order += cp_chunk(k)
        order += cp_x(3) + cp_x(4) + cp_wo(0) + cp_ff(0)
        order += cp_x(5) + cp_wm(0) + cp_ff(1)
        order += cp_x(6) + cp_wo(1) + cp_wm(1) + cp_ff(2)
        order += cp_x(7) + cp_wm(2) + cp_ff(3)
        order += cp_wm(3) + cp_ff(4)
        for cp in order:
            cp.start()
        flag_s[0] = 128

        last = T0 - 1

        def zero_body(g, carry):
            for sec in range(3):
                dst, off = qkv_dst(last, sec)
                dst[g, pl.ds(off, TM), :] = jnp.zeros((TM, 128), f32)
            return carry
        jax.lax.fori_loop(0, NG, zero_body, 0)
        wait(cp_c())
        c = c_v[...].astype(f32)
        sc = c * jax.nn.sigmoid(c)
        st_v[...] = jnp.transpose(jnp.broadcast_to(sc, (128, D)))

        def normalize(row0, nrows, chains=None):
            for i in range(nrows // LNR):
                r0 = row0 + i * LNR
                x = x_v[pl.ds(r0, LNR), :].astype(f32)
                if chains is not None:
                    x = chains[i % len(chains)].after_rows(x)
                r, mr = _ln_stats(x)
                xn = x * r - mr
                if chains is not None:
                    chains[i % len(chains)].tok = xn[0:8, 0:128]
                for g in range(NG):
                    xn_s[g, pl.ds(r0, LNR), :] = xn[:, g * 128:(g + 1) * 128]

        def mod_chunk(k):
            col = k * KC if isinstance(k, int) else pl.multiple_of(k * KC, KC)
            sa, ca = _mod_cols(wmod_v, st_v, [col, D + col], KC)
            mod_v[:, pl.ds(col, KC)] = jnp.broadcast_to(sa, (8, KC))
            mod_v[:, pl.ds(D + col, KC)] = jnp.broadcast_to(ca, (8, KC))
            return sa, 1.0 + ca

        def h_chunk(k, t, n, sa, ca1):
            return (xn_s[k, pl.ds(t * TM, n * TM), :] * ca1 + sa).astype(bf16)

        def mm(h, w, sec, tiles, first):
            res = _dot(h, _unpack(w))
            for i, t in enumerate(tiles):
                dst, off = qkv_dst(t, sec)
                for g in range(NG):
                    blk = res[i * TM:(i + 1) * TM, g * 128:(g + 1) * 128]
                    if first:
                        dst[g, pl.ds(off, TM), :] = blk
                    else:
                        dst[g, pl.ds(off, TM), :] += blk

        def wcur(sec):
            return wcur_s[:, sec * D:(sec + 1) * D]

        def keep(k, sec, wp):
            r0 = k * (KC // 2) if isinstance(k, int) else pl.multiple_of(k * (KC // 2), KC // 2)
            cols = pl.ds(sec * D if isinstance(sec, int) else pl.multiple_of(sec * D, D), D)
            wcur_s[:, cols] = wp
            wqkv_p[pl.ds(r0, KC // 2), cols] = wp

        scope = jax.named_scope
        mod0 = lambda: (mod_v[0:1, 0:KC], 1.0 + mod_v[0:1, D:D + KC])
        with scope('w_wq0'):
            wait(cp_wq0())
        with scope('perm0'):
            def perm_body(sec, carry):
                keep(0, sec, _permute_qkv_section(wqkv_raw, 0, sec))
                return carry
            jax.lax.fori_loop(0, 3, perm_body, 0)
        with scope('w_x0'):
            wait(cp_x(0))
        with scope('norm0'):
            def norm_body(i, carry):
                normalize(pl.multiple_of(i * 64, 64), 64)
                return carry
            jax.lax.fori_loop(0, TM // 64, norm_body, 0)
        with scope('w_m0'):
            wait(cp_chunk(0, False), cp_x(1))
        with scope('mm00'):
            sa, ca1 = mod_chunk(0)
            h0 = h_chunk(0, 0, 1, sa, ca1)
            for sec in range(3):
                mm(h0, wcur(sec), sec, [0], True)
            normalize(TM, TM, [new_chain() for _ in range(4)])
        with scope('w_x2'):
            wait(cp_x(2))
        with scope('mm01'):
            h1 = h_chunk(0, 1, 1, *mod0())
            for sec in range(3):
                mm(h1, wcur(sec), sec, [1], True)
            normalize(2 * TM, TM, [new_chain() for _ in range(4)])
            hl_s[...] = _pack(h_chunk(0, last, 1, *mod0()))

        def chunk_body(k0, carry):
            k = k0 + 1
            with scope('w_chunk'):
                wait(cp_chunk(k))
            with scope('chunk'):
                hl = _unpack(hl_s[...])
                for sec in range(3):
                    mm(hl, wcur(sec), sec, [last], False)
                sa, ca1 = mod_chunk(k)
                hf = h_chunk(k, 0, last, sa, ca1)
                hl_s[...] = _pack(h_chunk(k, last, 1, sa, ca1))
                for sec in range(3):
                    wp = _permute_qkv_section(wqkv_raw, pl.multiple_of(k * KC, KC), sec)
                    mm(hf, wp, sec, list(range(last)), False)
                    keep(k, sec, wp)
            return carry
        jax.lax.fori_loop(0, NKC - 1, chunk_body, 0)

        with scope('w_x3'):
            wait(cp_x(T0))
        hl = _unpack(hl_s[...])
        for sec in range(3):
            mm(hl, wcur(sec), sec, [last], False)
        _ln1_next(x_v, mod_v, h_s, T0 * TM, [new_chain() for _ in range(4)])
        k0_s[:, 0:HALO, :] = jnp.zeros((NG, HALO, 128), f32)
        v0_s[:, 0:HALO, :] = jnp.broadcast_to(v0_s[:, HALO:HALO + 1, :], (NG, HALO, 128))
        k_s[:, 0:HALO, :] = k0_s[:, TM:TM + HALO, :]
        v_s[:, 0:HALO, :] = v0_s[:, TM:TM + HALO, :]

    @_when(step == 1, 'wait1')
    def _():
        wait(cp_x(4), cp_wo(0), cp_ff(0))

    @_when(step == 2, 'wait2')
    def _():
        wait(cp_x(5), cp_wm(0), cp_ff(1))

    @_when(step == 3, 'wait3')
    def _():
        wait(cp_x(6), cp_wo(1), cp_wm(1), cp_ff(2))

    @_when(step == 4, 'wait4')
    def _():
        wait(cp_x(7), cp_wm(2), cp_ff(3))

    @_when(step == 5, 'wait5')
    def _():
        wait(cp_wm(3), cp_ff(4))

    @_when(jnp.logical_and(step >= 1, step < N1), 'phase1')
    def _():
        _phase1(step, x_v, wqkv_p, wo_raw, wo_p, w1_v, w3_v, w2_v, s1_v, s3_v, s2_v, wmod_v, mod_v, st_v,
                h_s, q0_s, k0_s, v0_s, q_s, k_s, v_s, o_s, flag_s)

    @_when(step >= N1, 'phase2')
    def _():
        _phase2(step, x_v, wo_p, w1_v, w3_v, w2_v, s1_v, s3_v, s2_v, mod_v, q_s, k_s, v_s, o_s, flag_s,
                o_ref)


def _scratch_shapes():
    return [
        pltpu.VMEM((S, D), bf16),
        pltpu.VMEM((D, 3 * D), bf16),
        pltpu.VMEM((D // 2, 3 * D), u32),
        pltpu.VMEM((D, D), bf16),
        pltpu.VMEM((D // 2, D), u32),
        pltpu.VMEM((D, F), bf16),
        pltpu.VMEM((D, F), bf16),
        pltpu.VMEM((F, D), bf16),
        pltpu.VMEM((5, DH2 // PK, FH), bf16 if PK == 1 else u32),
        pltpu.VMEM((5, DH2 // PK, FH), bf16 if PK == 1 else u32),
        pltpu.VMEM((5, FH // PK, DH2), bf16 if PK == 1 else u32),
        pltpu.VMEM((D, 6 * D), bf16),
        pltpu.VMEM((8, 6 * D), f32),
        pltpu.VMEM((D, 128), f32),
        pltpu.VMEM((NG, T0 * TM, 128), f32),
        pltpu.VMEM((KC // 2, 3 * D), u32),
        pltpu.VMEM((TM // 2, KC), u32),
        pltpu.VMEM((TM, D), bf16),
        pltpu.VMEM((NG, TM, 128), f32),
        pltpu.VMEM((NG, HALO + TM, 128), f32),
        pltpu.VMEM((NG, HALO + TM, 128), f32),
        pltpu.VMEM((NG, S - TM, 128), f32),
        pltpu.VMEM((NG, HALO + S - TM, 128), f32),
        pltpu.VMEM((NG, HALO + S - TM, 128), f32),
        pltpu.VMEM((TM, D), bf16),
        pltpu.VMEM((1, D), bf16),
        pltpu.SMEM((1,), jnp.int32),
        pltpu.SemaphoreType.DMA((NSEM,)),
    ]


@jax.jit
def pallas_adaLN_cond__sliding_local_dilated__glu_gated_swiglu__prompt_kernel(
    A_x: jax.Array,
    A_wqkv: jax.Array,
    A_wo: jax.Array,
    B_x: jax.Array,
    B_w1: jax.Array,
    B_w3: jax.Array,
    B_w2: jax.Array,
    c: jax.Array,
    w_mod: jax.Array,
):
    del B_x
    x = A_x.reshape(S, D)
    hbm = pl.BlockSpec(memory_space=pl.ANY)
    out = pl.pallas_call(
        _kernel,
        grid=(N1 + NT,),
        in_specs=[hbm] * 8,
        out_specs=pl.BlockSpec((TM, D), lambda i: (jnp.maximum(i - N1, 0), 0)),
        out_shape=jax.ShapeDtypeStruct((S, D), A_x.dtype),
        scratch_shapes=_scratch_shapes(),
        compiler_params=pltpu.CompilerParams(
            dimension_semantics=("arbitrary",),
            vmem_limit_bytes=118 * 1024 * 1024,
        ),
        name="adaln_attn_ffn",
    )(x, c, A_wqkv, A_wo, B_w1, B_w3, B_w2, w_mod)
    return out.reshape(1, S, D)
```

```python
import jax
import jax.numpy as jnp
import jax.experimental.pallas as pl
import jax.experimental.pallas.tpu as pltpu

S, D, F = 2048, 1024, 3584
H, DH, W, DIL = 32, 32, 8, 2
NG = D // 128
TM = 256
NT = S // TM
T0 = 3
N1 = NT - T0 + 1
SUB = 64
HN = 256
FH = F // 2
DH2 = D // 2
KC = 128
NKC = D // KC
RU1 = 112
RU2 = 368
HALO = 16
PARTS = 'LMA'
SMODE = 'be'
EARLY = (0, 0)
PACE = 0
PK = 1
LN2CH = 32
NGRP = 2
NSEP = 1
UR = 8
UC = 256
NW = 1
PULL0 = 2
SLINK = True
SW = 256
WB1 = 2
WB2 = 1
LNR = 16
EPS = 1e-5
SCALE = DH ** -0.5
LOG2E = 1.4426950408889634
QSCALE = SCALE * LOG2E
NEG = -1000000000.0 * LOG2E

f32 = jnp.float32
bf16 = jnp.bfloat16
u32 = jnp.uint32

SEM_C = 0
SEM_X = 1
SEM_WQ0 = SEM_X + NT
SEM_CH = SEM_WQ0 + 1
SEM_WM = SEM_CH + NKC
SEM_WO = SEM_WM + 4
SEM_FF = SEM_WO + 2
SEM_OUT = SEM_FF + (N1 - 1)
NSEM = SEM_OUT + 2


def _when(cond, name):
    def deco(body):
        def scoped():
            with jax.named_scope(name):
                body()
        return pl.when(cond)(scoped)
    return deco


def _pack(x):
    return pltpu.bitcast(x, u32)


def _unpack(x):
    return pltpu.bitcast(x, bf16)


def _spack(x):
    return x if PK == 1 else _pack(x)


def _sunpack(x):
    return x if PK == 1 else _unpack(x)


def _dot(a, b):
    return jnp.dot(a, b, preferred_element_type=f32)


class _Chain:
    def __init__(self, always):
        self.always = always
        self.tok = None

    def after(self, x):
        if self.tok is None:
            return x
        t = self.tok if self.tok.dtype == x.dtype else pltpu.bitcast(self.tok, x.dtype)
        return jnp.where(self.always, x, t)

    def pace(self, done, n):
        t = done
        if self.tok is not None and n > 0:
            d = self.tok
            for _ in range(n):
                d = jnp.tanh(d)
            t = d + t
        self.tok = t

    def after_rows(self, x):
        x00 = self.after(x[0:8, 0:128])
        top = x00 if x.shape[1] == 128 else jnp.concatenate([x00, x[0:8, 128:]], axis=1)
        return top if x.shape[0] == 8 else jnp.concatenate([top, x[8:]], axis=0)


def _swap_stage(a, k, b, axis):
    n = 128 if axis == 1 else 8
    idx = jax.lax.broadcasted_iota(jnp.int32, a[0].shape, axis)
    m0 = (idx & (1 << b)) == 0
    out = list(a)
    for c in range(8):
        if c & (1 << k):
            continue
        lo, hi = a[c], a[c | (1 << k)]
        out[c] = jnp.where(m0, lo, pltpu.roll(hi, 1 << b, axis))
        out[c | (1 << k)] = jnp.where(m0, pltpu.roll(lo, n - (1 << b), axis), hi)
    return out


def _permute_qkv_section(w_ref, r0, sec):
    c0 = sec * D if isinstance(sec, int) else pl.multiple_of(sec * D, D)
    a = [_pack(w_ref[pl.ds(r0, KC), pl.ds(c0 + c * 128, 128)]) for c in range(8)]
    for k in range(3):
        a = _swap_stage(a, k, k + 1, 1)
    return jnp.concatenate(a, axis=1)


def _ln_stats(x):
    m = jnp.mean(x, axis=-1, keepdims=True)
    xc = x - m
    v = jnp.mean(xc * xc, axis=-1, keepdims=True)
    r = jax.lax.rsqrt(v + EPS)
    return r, m * r


def _modulated_ln(x, scale1, shift):
    r, mr = _ln_stats(x)
    return (x * r - mr) * scale1 + shift


def _attention_rows(q_s, k_s, v_s, q0, row0, wb, chain=None):
    lane = jax.lax.broadcasted_iota(jnp.int32, (8, 128), 1)
    m0 = (lane & 1) == 0
    m4 = (lane & 16) == 0
    qscale = QSCALE if chain is None else chain.after(jnp.full((8, 128), QSCALE, f32))
    q = [q_s[g, pl.ds(q0, 8), :] * qscale for g in range(NG)]
    logits = []
    for w0 in range(0, W, wb):
        zs = []
        for w in range(w0, w0 + wb):
            z = None
            for g in range(NG):
                p = q[g] * k_s[g, pl.ds(q0 + (HALO - DIL * w), 8), :]
                z = p if z is None else z + p
            zs.append(z)
        zs = [z + jnp.where(m0, pltpu.roll(z, 127, 1), pltpu.roll(z, 1, 1)) for z in zs]
        zs = [z + jnp.where(m4, pltpu.roll(z, 112, 1), pltpu.roll(z, 16, 1)) for z in zs]
        for w, z in zip(range(w0, w0 + wb), zs):
            if w > 0 and row0 is not None:
                row = jax.lax.broadcasted_iota(jnp.int32, (8, 128), 0) + row0
                z = jnp.where(row >= DIL * w, z, NEG)
            logits.append(z)
    m = logits[0]
    for w in range(1, W):
        m = jnp.maximum(m, logits[w])
    e = [jnp.exp2(logits[w] - m) for w in range(W)]
    den = e[0]
    for w in range(1, W):
        den = den + e[w]
    inv = pl.reciprocal(den, approx=False)
    outs = []
    for g in range(NG):
        o = None
        for w in range(W):
            p = e[w] * v_s[g, pl.ds(q0 + (HALO - DIL * w), 8), :]
            o = p if o is None else o + p
        outs.append(o * inv)
    if chain is not None:
        chain.tok = outs[-1]
    return jnp.concatenate(outs, axis=1)


def _attention(q_s, k_s, v_s, o_s, q0, o0, nrows, wb, row0=None):
    for r in range(0, nrows, 8):
        o = _attention_rows(q_s, k_s, v_s, q0 + r,
                            None if (row0 is None or r >= HALO) else row0 + r, wb)
        o_s[pl.ds(o0 + r, 8), :] = o.astype(bf16)


def _mod_cols(wmod_v, st_v, cols, n, chain=None):
    acc = [None] * len(cols)
    for r in range(0, D, 8):
        s = st_v[r:r + 8, :]
        if r == 0 and chain is not None:
            s = chain.after(s)
        if n > 128:
            s = jnp.concatenate([s] * (n // 128), axis=1)
        for i, col in enumerate(cols):
            p = wmod_v[r:r + 8, pl.ds(col, n)].astype(f32) * s
            acc[i] = p if acc[i] is None else acc[i] + p
    if chain is not None:
        chain.tok = acc[0][:, 0:128]
    return [a.sum(axis=0, keepdims=True) for a in acc]


def _lhs_operands(a11, a12, a21, a22):
    ops = (a11 + a22, a21 + a22, a11, a22, a11 + a12, a21 - a11, a12 - a22)
    return [v.astype(bf16) for v in ops]


def _rhs_sums(b11, b12, b21, b22):
    return (b11 + b22, b12 - b22, b21 - b11, b11 + b12, b21 + b22)


def _rhs_operands(sums, b11, b22):
    return [sums(0), b11, sums(1), sums(2), b22, sums(3), sums(4)]


def _combine(m):
    return (m[0] + m[3] - m[4] + m[6], m[2] + m[4], m[1] + m[3], m[0] - m[1] + m[2] + m[5])


def _new_chain(flag_s):
    return _Chain(jax.lax.broadcasted_iota(jnp.int32, (8, 128), 1) < flag_s[0])


def _ln1_next(x_v, mod_v, h_s, r0, chains, extra=None):
    sa = mod_v[0:1, 0 * D:1 * D]
    ca1 = 1.0 + mod_v[0:1, 1 * D:2 * D]
    for i, r in enumerate(range(0, TM, LNR)):
        chain = chains[i % len(chains)]
        x = chain.after_rows(x_v[pl.ds(r0 + r, LNR), :].astype(f32))
        h = _modulated_ln(x, ca1, sa)
        chain.tok = h[0:8, 0:128]
        h_s[pl.ds(r, LNR), :] = h.astype(bf16)
        if extra is not None:
            extra(i)


def _phase1(step, x_v, wqkv_p, wo_raw, wo_p, w1_v, w3_v, w2_v, s1_v, s3_v, s2_v, wmod_v, mod_v, st_v,
            h_s, q0_s, k0_s, v0_s, q_s, k_s, v_s, o_s, flag_s):
    step = jnp.clip(step, 1, N1 - 1)
    part = jnp.maximum(step - 2, 0)
    base = pl.multiple_of((step + T0 - 2) * TM, TM)
    h = h_s[...]
    chain = _new_chain(flag_s)

    ln_r0 = pl.multiple_of(jnp.minimum(step + T0, NT - 1) * TM, TM)
    sa = mod_v[0:1, 0 * D:1 * D]
    ca1 = 1.0 + mod_v[0:1, 1 * D:2 * D]

    def ln_unit(i):
        x = chain.after_rows(x_v[pl.ds(ln_r0 + i * LNR, LNR), :].astype(f32))
        hn = _modulated_ln(x, ca1, sa)
        chain.tok = hn[0:8, 0:128]
        h_s[pl.ds(i * LNR, LNR), :] = hn.astype(bf16)

    def wo_unit(i):
        gg, mid = i // 8, i % 8
        col = pl.ds(pl.multiple_of(part * 256 + gg * 128, 128), 128)
        a = [_pack(wo_raw[pl.ds(c * 128 + mid * 16, 16), col]) for c in range(8)]
        a[0] = chain.after(a[0])
        for k in range(3):
            a = _swap_stage(a, k, k, 0)
        for s in range(8):
            wo_p[pl.ds(s * 64 + mid * 8, 8), col] = a[s]
        chain.tok = a[7]

    at_r0 = pl.multiple_of(part * 64, 64)

    def attn_unit(i):
        o = _attention_rows(q0_s, k0_s, v0_s, at_r0 + i * 8,
                            at_r0 + i * 8 if i * 8 < HALO else None, WB1, chain)
        o_s[pl.ds(at_r0 + i * 8, 8), :] = o.astype(bf16)

    mod_col = pl.multiple_of(step * D, D)

    def mod_unit(i):
        col = pl.multiple_of(mod_col + i * 256, 256)
        val, = _mod_cols(wmod_v, st_v, [col], 256, chain)
        mod_v[:, pl.ds(col, 256)] = jnp.broadcast_to(val, (8, 256))

    sum_units = []
    for w_v, s_v, half, ru, ch in ((w1_v, s1_v, DH2, RU1, FH), (w3_v, s3_v, DH2, RU1, FH),
                                   (w2_v, s2_v, FH, RU2, DH2)):
        r_lo = jnp.minimum((step - 1) * (ru // 16), (half - ru) // 16)
        srcs = [w_v.at[pl.ds(pl.multiple_of(i * half + r_lo * 16, 16), ru)] for i in range(2)]
        dst = s_v.at[:, pl.ds(pl.multiple_of(r_lo * (16 // PK), 16 // PK), ru // PK)]
        r_bk = jnp.clip(r_lo + flag_s[0] - 128, 0, (half - ru) // 16)
        back = s_v.at[:, pl.ds(pl.multiple_of(r_bk * (16 // PK), 16 // PK), ru // PK)]
        sum_units += [(srcs, dst, back, ch, r, c0)
                      for r in range(0, ru, UR) for c0 in range(0, ch, UC)]

    def sum_unit(u):
        srcs, dst, back, ch, r, c0 = sum_units[u]
        q = [srcs[i][r:r + UR, j * ch + c0:j * ch + c0 + UC].astype(f32)
             for i in range(2) for j in range(2)]
        q[0] = chain.after_rows(q[0])
        for i, v in enumerate(_rhs_sums(*q)):
            dst[i, r // PK:(r + UR) // PK, c0:c0 + UC] = _spack(v.astype(bf16))
        bk = back[0, r // PK:r // PK + 8, c0:c0 + 128]
        chain.tok = bk.astype(f32) if PK == 1 else bk

    chain.tok = None
    for i in range(16):
        ln_unit(i)
        wo_unit(i)
    for i in range(4):
        mod_unit(i)
    for i in range(8):
        chain.tok = None
        attn_unit(i)

    npiece = 3 * NG // NW
    nsum = len(sum_units)
    done = 0
    chain.tok = None
    for t in range(npiece):
        upto = min(nsum, -(-nsum * max(t + 1 - PULL0, 0) // (npiece - PULL0)))
        if not SLINK:
            chain.tok = None
        for u in range(done, upto):
            sum_unit(u)
        sec, g0 = t * NW // NG, t * NW % NG
        dst, off = (q_s, k_s, v_s)[sec], (0 if sec == 0 else HALO)
        w = wqkv_p[:, t * NW * 128:(t + 1) * NW * 128]
        if upto > done:
            w = chain.after_rows(w)
        done = upto
        res = _dot(h, _unpack(w))
        for g in range(NW):
            dst[g0 + g, pl.ds(base + off, TM), :] = res[:, g * 128:(g + 1) * 128]


def _phase2(step, x_v, wo_p, w1_v, w3_v, w2_v, s1_v, s3_v, s2_v, mod_v, q_s, k_s, v_s, o_s, flag_s,
            o_ref):
    j2 = jnp.clip(step - N1, 0, NT - 1)
    ga = mod_v[0:1, 2 * D:3 * D]
    sb = mod_v[0:1, 3 * D:4 * D]
    cb1 = 1.0 + mod_v[0:1, 4 * D:5 * D]
    gb = mod_v[0:1, 5 * D:6 * D]
    row0 = pl.multiple_of(j2 * TM, TM)
    nsub = TM // SUB
    os_ = [o_s[pl.ds(s * SUB, SUB), :] for s in range(nsub)]
    x1s, blocks = [], []
    for s in range(nsub):
        att = _dot(os_[s], _unpack(wo_p[...]))
        x1 = x_v[pl.ds(row0 + s * SUB, SUB), :].astype(f32) + ga * att
        x1s.append(x1)
        chain = _new_chain(flag_s)
        for r in range(0, SUB, 32):
            hs = []
            for rr in (r, r + 16):
                hs.append(_modulated_ln(chain.after_rows(x1[rr:rr + 16]), cb1, sb))
                if LN2CH == 16 or rr > r:
                    chain.tok = hs[-1][0:8, 0:128]
            blocks.append(_lhs_operands(hs[0][:, :DH2], hs[0][:, DH2:],
                                        hs[1][:, :DH2], hs[1][:, DH2:]))

    nq = pl.multiple_of(jnp.minimum(j2, NT - 2) * TM, TM)
    _attention(q_s, k_s, v_s, o_s, nq, 0, TM, WB2)

    def stack(per_group):
        return [jnp.concatenate([ops[i] for ops in per_group], axis=0) for i in range(7)]

    nb = len(blocks) // NGRP
    groups = [stack(blocks[g * nb:(g + 1) * nb]) for g in range(NGRP)]

    def up_proj(a, w_v, s_v, j):
        c0 = j * HN
        b = _rhs_operands(lambda i: _sunpack(s_v[i, :, c0:c0 + HN]),
                          w_v[0:DH2, c0:c0 + HN], w_v[DH2:, FH + c0:FH + c0 + HN])
        return _combine([_dot(a[i], b[i]) for i in range(7)])

    def gate_up(a, j):
        act = []
        for g, u in zip(up_proj(a, w1_v, s1_v, j), up_proj(a, w3_v, s3_v, j)):
            hg = 0.5 * g
            act.append((hg + hg * jnp.tanh(hg)) * u)
        return _lhs_operands(*act)

    h_all = stack(groups)
    sep = [[gate_up(ops, j) for j in range(NSEP)] for ops in groups]
    acc = None
    for j in range(FH // HN):
        a = stack([sp[j] for sp in sep]) if j < NSEP else gate_up(h_all, j)
        r0 = j * HN
        b = _rhs_operands(lambda i: _sunpack(s2_v[i, r0 // PK:(r0 + HN) // PK, :]),
                          w2_v[r0:r0 + HN, 0:DH2], w2_v[FH + r0:FH + r0 + HN, DH2:])
        m = [_dot(a[i], b[i]) for i in range(7)]
        acc = m if acc is None else [p + q for p, q in zip(acc, m)]
    c11, c12, c21, c22 = _combine(acc)
    x1 = jnp.concatenate(x1s, axis=0)
    for blk in range(TM // 32):
        rows = slice(blk * 16, (blk + 1) * 16)
        for t, (left, right) in enumerate(((c11, c12), (c21, c22))):
            y = jnp.concatenate([left[rows], right[rows]], axis=1)
            r = blk * 32 + t * 16
            o_ref[r:r + 16, :] = (x1[r:r + 16] + gb * y).astype(o_ref.dtype)


def _kernel(x_hbm, c_hbm, wqkv_hbm, wo_hbm, w1_hbm, w3_hbm, w2_hbm, wmod_hbm, o_hbm,
            x_v, wqkv_raw, wqkv_p, wo_raw, wo_p, w1_v, w3_v, w2_v, s1_v, s3_v, s2_v,
            wmod_v, mod_v, st_v, xn_s, wcur_s, hl_s, h_s, q0_s, k0_s, v0_s, q_s, k_s, v_s,
            o_s, o_ref, c_v, flag_s, sems):
    step = pl.program_id(0)

    def new_chain():
        return _new_chain(flag_s)

    def cp_rows(src, dst, r0, n, sem):
        rows = pl.ds(r0, n)
        return pltpu.make_async_copy(src.at[rows], dst.at[rows], sems.at[sem])

    def cp_cols(src, dst, c0, n, sem):
        cols = pl.ds(c0, n)
        return pltpu.make_async_copy(src.at[:, cols], dst.at[:, cols], sems.at[sem])

    cp_c = lambda: [pltpu.make_async_copy(c_hbm, c_v, sems.at[SEM_C])]
    cp_x = lambda i: [cp_rows(x_hbm, x_v, i * TM, TM, SEM_X + i)]
    cp_wq0 = lambda: [cp_rows(wqkv_hbm, wqkv_raw, 0, KC, SEM_WQ0)]
    cp_wm = lambda p: [cp_cols(wmod_hbm, wmod_v, (2 + p) * D, D, SEM_WM + p)]

    def cp_chunk(k, with_wq=True):
        cps = [cp_rows(wqkv_hbm, wqkv_raw, k * KC, KC, SEM_CH + k)] if with_wq else []
        return cps + [cp_cols(wmod_hbm, wmod_v, k * KC, KC, SEM_CH + k),
                      cp_cols(wmod_hbm, wmod_v, D + k * KC, KC, SEM_CH + k)]

    def cp_wo(i):
        c0, n = (0, 256) if i == 0 else (256, D - 256)
        return [cp_cols(wo_hbm, wo_raw, c0, n, SEM_WO + i)]

    def cp_ff(i):
        cps = []
        for src, dst, half, ru in ((w1_hbm, w1_v, DH2, RU1), (w3_hbm, w3_v, DH2, RU1),
                                   (w2_hbm, w2_v, FH, RU2)):
            n = min(ru, half - i * ru)
            cps += [cp_rows(src, dst, h * half + i * ru, n, SEM_FF + i) for h in range(2)]
        return cps

    def wait(*groups):
        for cps in groups:
            for cp in cps:
                cp.wait()

    def qkv_dst(t, sec):
        off = 0 if sec == 0 else HALO
        if t == 0:
            return (q0_s, k0_s, v0_s)[sec], off
        return (q_s, k_s, v_s)[sec], off + (t - 1) * TM

    @_when(step == 0, 'first')
    def _first():
        order = cp_c() + cp_wq0() + cp_x(0) + cp_chunk(0, False) + cp_x(1) + cp_x(2)
        for k in range(1, NKC):
            order += cp_chunk(k)
        order += cp_x(3) + cp_x(4) + cp_wo(0) + cp_ff(0)
        order += cp_x(5) + cp_wm(0) + cp_ff(1)
        order += cp_x(6) + cp_wo(1) + cp_wm(1) + cp_ff(2)
        order += cp_x(7) + cp_wm(2) + cp_ff(3)
        order += cp_wm(3) + cp_ff(4)
        for cp in order:
            cp.start()
        flag_s[0] = 128

        last = T0 - 1

        def zero_body(g, carry):
            for sec in range(3):
                dst, off = qkv_dst(last, sec)
                dst[g, pl.ds(off, TM), :] = jnp.zeros((TM, 128), f32)
            return carry
        jax.lax.fori_loop(0, NG, zero_body, 0)
        wait(cp_c())
        c = c_v[...].astype(f32)
        sc = c * jax.nn.sigmoid(c)
        st_v[...] = jnp.transpose(jnp.broadcast_to(sc, (128, D)))

        def normalize(row0, nrows, chains=None):
            for i in range(nrows // LNR):
                r0 = row0 + i * LNR
                x = x_v[pl.ds(r0, LNR), :].astype(f32)
                if chains is not None:
                    x = chains[i % len(chains)].after_rows(x)
                r, mr = _ln_stats(x)
                xn = x * r - mr
                if chains is not None:
                    chains[i % len(chains)].tok = xn[0:8, 0:128]
                for g in range(NG):
                    xn_s[g, pl.ds(r0, LNR), :] = xn[:, g * 128:(g + 1) * 128]

        def mod_chunk(k):
            col = k * KC if isinstance(k, int) else pl.multiple_of(k * KC, KC)
            sa, ca = _mod_cols(wmod_v, st_v, [col, D + col], KC)
            mod_v[:, pl.ds(col, KC)] = jnp.broadcast_to(sa, (8, KC))
            mod_v[:, pl.ds(D + col, KC)] = jnp.broadcast_to(ca, (8, KC))
            return sa, 1.0 + ca

        def h_chunk(k, t, n, sa, ca1):
            return (xn_s[k, pl.ds(t * TM, n * TM), :] * ca1 + sa).astype(bf16)

        def mm(h, w, sec, tiles, first):
            res = _dot(h, _unpack(w))
            for i, t in enumerate(tiles):
                dst, off = qkv_dst(t, sec)
                for g in range(NG):
                    blk = res[i * TM:(i + 1) * TM, g * 128:(g + 1) * 128]
                    if first:
                        dst[g, pl.ds(off, TM), :] = blk
                    else:
                        dst[g, pl.ds(off, TM), :] += blk

        def wcur(sec):
            return wcur_s[:, sec * D:(sec + 1) * D]

        def keep(k, sec, wp):
            r0 = k * (KC // 2) if isinstance(k, int) else pl.multiple_of(k * (KC // 2), KC // 2)
            cols = pl.ds(sec * D if isinstance(sec, int) else pl.multiple_of(sec * D, D), D)
            wcur_s[:, cols] = wp
            wqkv_p[pl.ds(r0, KC // 2), cols] = wp

        scope = jax.named_scope
        mod0 = lambda: (mod_v[0:1, 0:KC], 1.0 + mod_v[0:1, D:D + KC])
        with scope('w_wq0'):
            wait(cp_wq0())
        with scope('perm0'):
            def perm_body(sec, carry):
                keep(0, sec, _permute_qkv_section(wqkv_raw, 0, sec))
                return carry
            jax.lax.fori_loop(0, 3, perm_body, 0)
        with scope('w_x0'):
            wait(cp_x(0))
        with scope('norm0'):
            def norm_body(i, carry):
                normalize(pl.multiple_of(i * 64, 64), 64)
                return carry
            jax.lax.fori_loop(0, TM // 64, norm_body, 0)
        with scope('w_m0'):
            wait(cp_chunk(0, False), cp_x(1))
        with scope('mm00'):
            sa, ca1 = mod_chunk(0)
            h0 = h_chunk(0, 0, 1, sa, ca1)
            for sec in range(3):
                mm(h0, wcur(sec), sec, [0], True)
            normalize(TM, TM, [new_chain() for _ in range(4)])
        with scope('w_x2'):
            wait(cp_x(2))
        with scope('mm01'):
            h1 = h_chunk(0, 1, 1, *mod0())
            for sec in range(3):
                mm(h1, wcur(sec), sec, [1], True)
            normalize(2 * TM, TM, [new_chain() for _ in range(4)])
            hl_s[...] = _pack(h_chunk(0, last, 1, *mod0()))

        def chunk_body(k0, carry):
            k = k0 + 1
            with scope('w_chunk'):
                wait(cp_chunk(k))
            with scope('chunk'):
                hl = _unpack(hl_s[...])
                for sec in range(3):
                    mm(hl, wcur(sec), sec, [last], False)
                sa, ca1 = mod_chunk(k)
                hf = h_chunk(k, 0, last, sa, ca1)
                hl_s[...] = _pack(h_chunk(k, last, 1, sa, ca1))
                for sec in range(3):
                    wp = _permute_qkv_section(wqkv_raw, pl.multiple_of(k * KC, KC), sec)
                    mm(hf, wp, sec, list(range(last)), False)
                    keep(k, sec, wp)
            return carry
        jax.lax.fori_loop(0, NKC - 1, chunk_body, 0)

        with scope('w_x3'):
            wait(cp_x(T0))
        hl = _unpack(hl_s[...])
        for sec in range(3):
            mm(hl, wcur(sec), sec, [last], False)
        _ln1_next(x_v, mod_v, h_s, T0 * TM, [new_chain() for _ in range(4)])
        k0_s[:, 0:HALO, :] = jnp.zeros((NG, HALO, 128), f32)
        v0_s[:, 0:HALO, :] = jnp.broadcast_to(v0_s[:, HALO:HALO + 1, :], (NG, HALO, 128))
        k_s[:, 0:HALO, :] = k0_s[:, TM:TM + HALO, :]
        v_s[:, 0:HALO, :] = v0_s[:, TM:TM + HALO, :]

    @_when(step == 1, 'wait1')
    def _():
        wait(cp_x(4), cp_wo(0), cp_ff(0))

    @_when(step == 2, 'wait2')
    def _():
        wait(cp_x(5), cp_wm(0), cp_ff(1))

    @_when(step == 3, 'wait3')
    def _():
        wait(cp_x(6), cp_wo(1), cp_wm(1), cp_ff(2))

    @_when(step == 4, 'wait4')
    def _():
        wait(cp_x(7), cp_wm(2), cp_ff(3))

    @_when(step == 5, 'wait5')
    def _():
        wait(cp_wm(3), cp_ff(4))

    @_when(jnp.logical_and(step >= 1, step < N1), 'phase1')
    def _():
        _phase1(step, x_v, wqkv_p, wo_raw, wo_p, w1_v, w3_v, w2_v, s1_v, s3_v, s2_v, wmod_v, mod_v, st_v,
                h_s, q0_s, k0_s, v0_s, q_s, k_s, v_s, o_s, flag_s)

    def cp_out(j):
        rows = pl.ds(pl.multiple_of(j * TM, TM), TM)
        return pltpu.make_async_copy(o_ref.at[j % 2], o_hbm.at[rows], sems.at[SEM_OUT + j % 2])

    @_when(step > N1 + 1, 'wait_out')
    def _():
        cp_out(step - N1 - 2).wait()

    @_when(step >= N1, 'phase2')
    def _():
        _phase2(step, x_v, wo_p, w1_v, w3_v, w2_v, s1_v, s3_v, s2_v, mod_v, q_s, k_s, v_s, o_s, flag_s,
                o_ref.at[(step - N1) % 2])
        cp_out(step - N1).start()

    @_when(step == N1 + NT - 1, 'wait_last')
    def _():
        cp_out(NT - 2).wait()
        cp_out(NT - 1).wait()


def _scratch_shapes():
    return [
        pltpu.VMEM((S, D), bf16),
        pltpu.VMEM((D, 3 * D), bf16),
        pltpu.VMEM((D // 2, 3 * D), u32),
        pltpu.VMEM((D, D), bf16),
        pltpu.VMEM((D // 2, D), u32),
        pltpu.VMEM((D, F), bf16),
        pltpu.VMEM((D, F), bf16),
        pltpu.VMEM((F, D), bf16),
        pltpu.VMEM((5, DH2 // PK, FH), bf16 if PK == 1 else u32),
        pltpu.VMEM((5, DH2 // PK, FH), bf16 if PK == 1 else u32),
        pltpu.VMEM((5, FH // PK, DH2), bf16 if PK == 1 else u32),
        pltpu.VMEM((D, 6 * D), bf16),
        pltpu.VMEM((8, 6 * D), f32),
        pltpu.VMEM((D, 128), f32),
        pltpu.VMEM((NG, T0 * TM, 128), f32),
        pltpu.VMEM((KC // 2, 3 * D), u32),
        pltpu.VMEM((TM // 2, KC), u32),
        pltpu.VMEM((TM, D), bf16),
        pltpu.VMEM((NG, TM, 128), f32),
        pltpu.VMEM((NG, HALO + TM, 128), f32),
        pltpu.VMEM((NG, HALO + TM, 128), f32),
        pltpu.VMEM((NG, S - TM, 128), f32),
        pltpu.VMEM((NG, HALO + S - TM, 128), f32),
        pltpu.VMEM((NG, HALO + S - TM, 128), f32),
        pltpu.VMEM((TM, D), bf16),
        pltpu.VMEM((2, TM, D), bf16),
        pltpu.VMEM((1, D), bf16),
        pltpu.SMEM((1,), jnp.int32),
        pltpu.SemaphoreType.DMA((NSEM,)),
    ]


@jax.jit
def pallas_adaLN_cond__sliding_local_dilated__glu_gated_swiglu__prompt_kernel(
    A_x: jax.Array,
    A_wqkv: jax.Array,
    A_wo: jax.Array,
    B_x: jax.Array,
    B_w1: jax.Array,
    B_w3: jax.Array,
    B_w2: jax.Array,
    c: jax.Array,
    w_mod: jax.Array,
):
    del B_x
    x = A_x.reshape(S, D)
    hbm = pl.BlockSpec(memory_space=pl.ANY)
    out = pl.pallas_call(
        _kernel,
        grid=(N1 + NT,),
        in_specs=[hbm] * 8,
        out_specs=hbm,
        out_shape=jax.ShapeDtypeStruct((S, D), A_x.dtype),
        scratch_shapes=_scratch_shapes(),
        compiler_params=pltpu.CompilerParams(
            dimension_semantics=("arbitrary",),
            vmem_limit_bytes=118 * 1024 * 1024,
        ),
        name="adaln_attn_ffn",
    )(x, c, A_wqkv, A_wo, B_w1, B_w3, B_w2, w_mod)
    return out.reshape(1, S, D)
```

```python
import jax
import jax.numpy as jnp
import jax.experimental.pallas as pl
import jax.experimental.pallas.tpu as pltpu

S, D, F = 2048, 1024, 3584
H, DH, W, DIL = 32, 32, 8, 2
NG = D // 128
TM = 256
NT = S // TM
T0 = 3
N1 = NT - T0 + 1
SUB = 64
HN = 256
FH = F // 2
DH2 = D // 2
KC = 128
NKC = D // KC
RU1 = 112
RU2 = 368
HALO = 16
PARTS = 'LMA'
SMODE = 'be'
EARLY = (0, 0)
PACE = 0
PK = 1
MR = 64
LN2CH = 32
NGRP = 2
NSEP = 1
UR = 8
UC = 256
NW = 1
PULL0 = 2
SLINK = True
SW = 256
WB1 = 1
WB2 = 1
LNR = 16
EPS = 1e-5
SCALE = DH ** -0.5
LOG2E = 1.4426950408889634
QSCALE = SCALE * LOG2E
NEG = -1000000000.0 * LOG2E

f32 = jnp.float32
bf16 = jnp.bfloat16
u32 = jnp.uint32

SEM_C = 0
SEM_X = 1
SEM_WQ0 = SEM_X + NT
SEM_CH = SEM_WQ0 + 1
SEM_WM = SEM_CH + NKC
SEM_WO = SEM_WM + 4
SEM_FF = SEM_WO + 2
SEM_OUT = SEM_FF + (N1 - 1)
NSEM = SEM_OUT + 2


def _when(cond, name):
    def deco(body):
        def scoped():
            with jax.named_scope(name):
                body()
        return pl.when(cond)(scoped)
    return deco


def _pack(x):
    return pltpu.bitcast(x, u32)


def _unpack(x):
    return pltpu.bitcast(x, bf16)


def _spack(x):
    return x if PK == 1 else _pack(x)


def _sunpack(x):
    return x if PK == 1 else _unpack(x)


def _dot(a, b):
    return jnp.dot(a, b, preferred_element_type=f32)


class _Chain:
    def __init__(self, always):
        self.always = always
        self.tok = None

    def after(self, x):
        if self.tok is None:
            return x
        t = self.tok if self.tok.dtype == x.dtype else pltpu.bitcast(self.tok, x.dtype)
        return jnp.where(self.always, x, t)

    def pace(self, done, n):
        t = done
        if self.tok is not None and n > 0:
            d = self.tok
            for _ in range(n):
                d = jnp.tanh(d)
            t = d + t
        self.tok = t

    def after_rows(self, x):
        x00 = self.after(x[0:8, 0:128])
        top = x00 if x.shape[1] == 128 else jnp.concatenate([x00, x[0:8, 128:]], axis=1)
        return top if x.shape[0] == 8 else jnp.concatenate([top, x[8:]], axis=0)


def _swap_stage(a, k, b, axis):
    n = 128 if axis == 1 else 8
    idx = jax.lax.broadcasted_iota(jnp.int32, a[0].shape, axis)
    m0 = (idx & (1 << b)) == 0
    out = list(a)
    for c in range(8):
        if c & (1 << k):
            continue
        lo, hi = a[c], a[c | (1 << k)]
        out[c] = jnp.where(m0, lo, pltpu.roll(hi, 1 << b, axis))
        out[c | (1 << k)] = jnp.where(m0, pltpu.roll(lo, n - (1 << b), axis), hi)
    return out


def _permute_qkv_section(w_ref, r0, sec):
    c0 = sec * D if isinstance(sec, int) else pl.multiple_of(sec * D, D)
    a = [_pack(w_ref[pl.ds(r0, KC), pl.ds(c0 + c * 128, 128)]) for c in range(8)]
    for k in range(3):
        a = _swap_stage(a, k, k + 1, 1)
    return jnp.concatenate(a, axis=1)


def _ln_stats(x):
    m = jnp.mean(x, axis=-1, keepdims=True)
    xc = x - m
    v = jnp.mean(xc * xc, axis=-1, keepdims=True)
    r = jax.lax.rsqrt(v + EPS)
    return r, m * r


def _modulated_ln(x, scale1, shift):
    r, mr = _ln_stats(x)
    return (x * r - mr) * scale1 + shift


def _attention_rows(q_s, k_s, v_s, q0, row0, wb, chain=None, nr=8):
    lane = jax.lax.broadcasted_iota(jnp.int32, (nr, 128), 1)
    m0 = (lane & 1) == 0
    m4 = (lane & 16) == 0
    qscale = QSCALE if chain is None else jnp.concatenate(
        [chain.after(jnp.full((8, 128), QSCALE, f32))] * (nr // 8), axis=0)
    q = q_s[:, pl.ds(q0, nr), :] * qscale
    logits = []
    for w0 in range(0, W, wb):
        zs = [jnp.sum(q * k_s[:, pl.ds(q0 + (HALO - DIL * w), nr), :], axis=0)
              for w in range(w0, w0 + wb)]
        zs = [z + jnp.where(m0, pltpu.roll(z, 127, 1), pltpu.roll(z, 1, 1)) for z in zs]
        zs = [z + jnp.where(m4, pltpu.roll(z, 112, 1), pltpu.roll(z, 16, 1)) for z in zs]
        for w, z in zip(range(w0, w0 + wb), zs):
            if w > 0 and row0 is not None:
                row = jax.lax.broadcasted_iota(jnp.int32, (nr, 128), 0) + row0
                z = jnp.where(row >= DIL * w, z, NEG)
            logits.append(z)
    m = logits[0]
    for w in range(1, W):
        m = jnp.maximum(m, logits[w])
    e = [jnp.exp2(logits[w] - m) for w in range(W)]
    den = e[0]
    for w in range(1, W):
        den = den + e[w]
    inv = pl.reciprocal(den, approx=False)
    o = None
    for w in range(W):
        p = e[w] * v_s[:, pl.ds(q0 + (HALO - DIL * w), nr), :]
        o = p if o is None else o + p
    o = o * inv
    if chain is not None:
        chain.tok = o[NG - 1, 0:8]
    return jnp.concatenate([o[g] for g in range(NG)], axis=1)


def _attention(q_s, k_s, v_s, o_s, q0, o0, nrows, wb, row0=None):
    for r in range(0, nrows, 8):
        o = _attention_rows(q_s, k_s, v_s, q0 + r,
                            None if (row0 is None or r >= HALO) else row0 + r, wb)
        o_s[pl.ds(o0 + r, 8), :] = o.astype(bf16)


def _mod_cols(wmod_v, st_v, col, n, chain=None):
    acc = None
    for r in range(0, D, MR):
        s = st_v[r:r + MR, :]
        if r == 0 and chain is not None:
            s = chain.after_rows(s)
        if n > 128:
            s = jnp.concatenate([s] * (n // 128), axis=1)
        p = wmod_v[r:r + MR, pl.ds(col, n)].astype(f32) * s
        for i in range(0, MR, 8):
            acc = p[i:i + 8] if acc is None else acc + p[i:i + 8]
    if chain is not None:
        chain.tok = acc[:, 0:128]
    return acc.sum(axis=0, keepdims=True)


def _lhs_operands(a11, a12, a21, a22):
    ops = (a11 + a22, a21 + a22, a11, a22, a11 + a12, a21 - a11, a12 - a22)
    return [v.astype(bf16) for v in ops]


def _rhs_sums(b11, b12, b21, b22):
    return (b11 + b22, b12 - b22, b21 - b11, b11 + b12, b21 + b22)


def _rhs_operands(sums, b11, b22):
    return [sums(0), b11, sums(1), sums(2), b22, sums(3), sums(4)]


def _combine(m):
    return (m[0] + m[3] - m[4] + m[6], m[2] + m[4], m[1] + m[3], m[0] - m[1] + m[2] + m[5])


def _new_chain(flag_s):
    return _Chain(jax.lax.broadcasted_iota(jnp.int32, (8, 128), 1) < flag_s[0])


def _ln1_next(x_v, mod_v, h_s, r0, chains, extra=None):
    sa = mod_v[0:1, 0 * D:1 * D]
    ca1 = 1.0 + mod_v[0:1, 1 * D:2 * D]
    for i, r in enumerate(range(0, TM, LNR)):
        chain = chains[i % len(chains)]
        x = chain.after_rows(x_v[pl.ds(r0 + r, LNR), :].astype(f32))
        h = _modulated_ln(x, ca1, sa)
        chain.tok = h[0:8, 0:128]
        h_s[pl.ds(r, LNR), :] = h.astype(bf16)
        if extra is not None:
            extra(i)


def _phase1(step, x_v, wqkv_p, wo_raw, wo_p, w1_v, w3_v, w2_v, s1_v, s3_v, s2_v, wmod_v, mod_v, st_v,
            h_s, q0_s, k0_s, v0_s, q_s, k_s, v_s, o_s, flag_s):
    step = jnp.clip(step, 1, N1 - 1)
    part = jnp.maximum(step - 2, 0)
    base = pl.multiple_of((step + T0 - 2) * TM, TM)
    h = h_s[...]
    chain = _new_chain(flag_s)

    ln_r0 = pl.multiple_of(jnp.minimum(step + T0, NT - 1) * TM, TM)
    sa = mod_v[0:1, 0 * D:1 * D]
    ca1 = 1.0 + mod_v[0:1, 1 * D:2 * D]

    def ln_unit(i, nr=LNR):
        x = x_v[pl.ds(ln_r0 + i * nr, nr), :].astype(f32)
        x = jnp.concatenate([chain.after_rows(x[r:r + 8]) for r in range(0, nr, 8)], axis=0)
        hn = _modulated_ln(x, ca1, sa)
        chain.tok = hn[0:8, 0:128]
        h_s[pl.ds(i * nr, nr), :] = hn.astype(bf16)

    def wo_unit(i):
        gg, mid = i // 8, i % 8
        col = pl.ds(pl.multiple_of(part * 256 + gg * 128, 128), 128)
        a = [_pack(wo_raw[pl.ds(c * 128 + mid * 16, 16), col]) for c in range(8)]
        a[0] = chain.after(a[0])
        for k in range(3):
            a = _swap_stage(a, k, k, 0)
        for s in range(8):
            wo_p[pl.ds(s * 64 + mid * 8, 8), col] = a[s]
        chain.tok = a[7]

    at_r0 = pl.multiple_of(part * 64, 64)

    def attn_unit(i, nr=8):
        o = _attention_rows(q0_s, k0_s, v0_s, at_r0 + i * nr,
                            at_r0 + i * nr if i * nr < HALO else None, WB1, chain, nr)
        o_s[pl.ds(at_r0 + i * nr, nr), :] = o.astype(bf16)

    mod_col = pl.multiple_of(step * D, D)

    def mod_unit(i):
        col = pl.multiple_of(mod_col + i * 256, 256)
        val = _mod_cols(wmod_v, st_v, col, 256, chain)
        mod_v[:, pl.ds(col, 256)] = jnp.broadcast_to(val, (8, 256))

    sum_units = []
    for w_v, s_v, half, ru, ch in ((w1_v, s1_v, DH2, RU1, FH), (w3_v, s3_v, DH2, RU1, FH),
                                   (w2_v, s2_v, FH, RU2, DH2)):
        r_lo = jnp.minimum((step - 1) * (ru // 16), (half - ru) // 16)
        srcs = [w_v.at[pl.ds(pl.multiple_of(i * half + r_lo * 16, 16), ru)] for i in range(2)]
        dst = s_v.at[:, pl.ds(pl.multiple_of(r_lo * (16 // PK), 16 // PK), ru // PK)]
        r_bk = jnp.clip(r_lo + flag_s[0] - 128, 0, (half - ru) // 16)
        back = s_v.at[:, pl.ds(pl.multiple_of(r_bk * (16 // PK), 16 // PK), ru // PK)]
        sum_units += [(srcs, dst, back, ch, r, c0)
                      for r in range(0, ru, UR) for c0 in range(0, ch, UC)]

    def sum_unit(u):
        srcs, dst, back, ch, r, c0 = sum_units[u]
        q = [srcs[i][r:r + UR, j * ch + c0:j * ch + c0 + UC].astype(f32)
             for i in range(2) for j in range(2)]
        q[0] = chain.after_rows(q[0])
        dst[:, r:r + UR, c0:c0 + UC] = jnp.stack(_rhs_sums(*q)).astype(bf16)
        bk = back[0, r // PK:r // PK + 8, c0:c0 + 128]
        chain.tok = bk.astype(f32) if PK == 1 else bk

    def mm_unit(t, gated):
        sec, g = t // NG, t % NG
        dst, off = (q_s, k_s, v_s)[sec], (0 if sec == 0 else HALO)
        w = wqkv_p[:, t * 128:(t + 1) * 128]
        if gated:
            w = chain.after_rows(w)
        res = _dot(h, _unpack(w))
        dst[g, pl.ds(base + off, TM), :] = res
        return res[0:8]

    PLAN(chain, mm_unit, ln_unit, wo_unit, attn_unit, mod_unit, sum_unit, len(sum_units))


def PLAN(chain, mm_unit, ln_unit, wo_unit, attn_unit, mod_unit, sum_unit, nsum):
    ticks = [mm_unit(t, False) for t in range(3 * NG)]
    done = 0
    for t in range(3 * NG - 1):
        chain.tok = ticks[t]
        if t < 8:
            ln_unit(t, 32)
            wo_unit(2 * t)
            wo_unit(2 * t + 1)
        if 15 <= t < 19:
            mod_unit(t - 15)
        n = 10 if (t < 8 or 15 <= t < 19) else -(-(nsum - 120) // 11)
        for u in range(done, min(done + n, nsum)):
            sum_unit(u)
        done = min(done + n, nsum)
    assert done == nsum
    for i in range(8):
        chain.tok = None
        attn_unit(i)


def _phase2(step, x_v, wo_p, w1_v, w3_v, w2_v, s1_v, s3_v, s2_v, mod_v, q_s, k_s, v_s, o_s, flag_s,
            o_ref):
    j2 = jnp.clip(step - N1, 0, NT - 1)
    ga = mod_v[0:1, 2 * D:3 * D]
    sb = mod_v[0:1, 3 * D:4 * D]
    cb1 = 1.0 + mod_v[0:1, 4 * D:5 * D]
    gb = mod_v[0:1, 5 * D:6 * D]
    row0 = pl.multiple_of(j2 * TM, TM)
    nsub = TM // SUB
    os_ = [o_s[pl.ds(s * SUB, SUB), :] for s in range(nsub)]
    x1s, blocks = [], []
    for s in range(nsub):
        att = _dot(os_[s], _unpack(wo_p[...]))
        x1 = x_v[pl.ds(row0 + s * SUB, SUB), :].astype(f32) + ga * att
        x1s.append(x1)
        chain = _new_chain(flag_s)
        for r in range(0, SUB, 32):
            hs = []
            for rr in (r, r + 16):
                hs.append(_modulated_ln(chain.after_rows(x1[rr:rr + 16]), cb1, sb))
                if LN2CH == 16 or rr > r:
                    chain.tok = hs[-1][0:8, 0:128]
            blocks.append(_lhs_operands(hs[0][:, :DH2], hs[0][:, DH2:],
                                        hs[1][:, :DH2], hs[1][:, DH2:]))

    nq = pl.multiple_of(jnp.minimum(j2, NT - 2) * TM, TM)
    _attention(q_s, k_s, v_s, o_s, nq, 0, TM, WB2)

    def stack(per_group):
        return [jnp.concatenate([ops[i] for ops in per_group], axis=0) for i in range(7)]

    nb = len(blocks) // NGRP
    groups = [stack(blocks[g * nb:(g + 1) * nb]) for g in range(NGRP)]

    def up_proj(a, w_v, s_v, j):
        c0 = j * HN
        b = _rhs_operands(lambda i: _sunpack(s_v[i, :, c0:c0 + HN]),
                          w_v[0:DH2, c0:c0 + HN], w_v[DH2:, FH + c0:FH + c0 + HN])
        return _combine([_dot(a[i], b[i]) for i in range(7)])

    def gate_up(a, j):
        act = []
        for g, u in zip(up_proj(a, w1_v, s1_v, j), up_proj(a, w3_v, s3_v, j)):
            hg = 0.5 * g
            act.append((hg + hg * jnp.tanh(hg)) * u)
        return _lhs_operands(*act)

    h_all = stack(groups)
    sep = [[gate_up(ops, j) for j in range(NSEP)] for ops in groups]
    acc = None
    for j in range(FH // HN):
        a = stack([sp[j] for sp in sep]) if j < NSEP else gate_up(h_all, j)
        r0 = j * HN
        b = _rhs_operands(lambda i: _sunpack(s2_v[i, r0 // PK:(r0 + HN) // PK, :]),
                          w2_v[r0:r0 + HN, 0:DH2], w2_v[FH + r0:FH + r0 + HN, DH2:])
        m = [_dot(a[i], b[i]) for i in range(7)]
        acc = m if acc is None else [p + q for p, q in zip(acc, m)]
    c11, c12, c21, c22 = _combine(acc)
    x1 = jnp.concatenate(x1s, axis=0)
    for blk in range(TM // 32):
        rows = slice(blk * 16, (blk + 1) * 16)
        for t, (left, right) in enumerate(((c11, c12), (c21, c22))):
            y = jnp.concatenate([left[rows], right[rows]], axis=1)
            r = blk * 32 + t * 16
            o_ref[r:r + 16, :] = (x1[r:r + 16] + gb * y).astype(o_ref.dtype)


def _kernel(x_hbm, c_hbm, wqkv_hbm, wo_hbm, w1_hbm, w3_hbm, w2_hbm, wmod_hbm, o_hbm,
            x_v, wqkv_raw, wqkv_p, wo_raw, wo_p, w1_v, w3_v, w2_v, s1_v, s3_v, s2_v,
            wmod_v, mod_v, st_v, xn_s, wcur_s, hl_s, h_s, q0_s, k0_s, v0_s, q_s, k_s, v_s,
            o_s, o_ref, c_v, flag_s, sems):
    step = pl.program_id(0)

    def new_chain():
        return _new_chain(flag_s)

    def cp_rows(src, dst, r0, n, sem):
        rows = pl.ds(r0, n)
        return pltpu.make_async_copy(src.at[rows], dst.at[rows], sems.at[sem])

    def cp_cols(src, dst, c0, n, sem):
        cols = pl.ds(c0, n)
        return pltpu.make_async_copy(src.at[:, cols], dst.at[:, cols], sems.at[sem])

    cp_c = lambda: [pltpu.make_async_copy(c_hbm, c_v, sems.at[SEM_C])]
    cp_x = lambda i: [cp_rows(x_hbm, x_v, i * TM, TM, SEM_X + i)]
    cp_wq0 = lambda: [cp_rows(wqkv_hbm, wqkv_raw, 0, KC, SEM_WQ0)]
    cp_wm = lambda p: [cp_cols(wmod_hbm, wmod_v, (2 + p) * D, D, SEM_WM + p)]

    def cp_chunk(k, with_wq=True):
        cps = [cp_rows(wqkv_hbm, wqkv_raw, k * KC, KC, SEM_CH + k)] if with_wq else []
        return cps + [cp_cols(wmod_hbm, wmod_v, k * KC, KC, SEM_CH + k),
                      cp_cols(wmod_hbm, wmod_v, D + k * KC, KC, SEM_CH + k)]

    def cp_wo(i):
        c0, n = (0, 256) if i == 0 else (256, D - 256)
        return [cp_cols(wo_hbm, wo_raw, c0, n, SEM_WO + i)]

    def cp_ff(i):
        cps = []
        for src, dst, half, ru in ((w1_hbm, w1_v, DH2, RU1), (w3_hbm, w3_v, DH2, RU1),
                                   (w2_hbm, w2_v, FH, RU2)):
            n = min(ru, half - i * ru)
            cps += [cp_rows(src, dst, h * half + i * ru, n, SEM_FF + i) for h in range(2)]
        return cps

    def wait(*groups):
        for cps in groups:
            for cp in cps:
                cp.wait()

    def qkv_dst(t, sec):
        off = 0 if sec == 0 else HALO
        if t == 0:
            return (q0_s, k0_s, v0_s)[sec], off
        return (q_s, k_s, v_s)[sec], off + (t - 1) * TM

    @_when(step == 0, 'first')
    def _first():
        order = cp_c() + cp_wq0() + cp_x(0) + cp_chunk(0, False) + cp_x(1) + cp_x(2)
        for k in range(1, NKC):
            order += cp_chunk(k)
        order += cp_x(3) + cp_x(4) + cp_wo(0) + cp_ff(0)
        order += cp_x(5) + cp_wm(0) + cp_ff(1)
        order += cp_x(6) + cp_wo(1) + cp_wm(1) + cp_ff(2)
        order += cp_x(7) + cp_wm(2) + cp_ff(3)
        order += cp_wm(3) + cp_ff(4)
        for cp in order:
            cp.start()
        flag_s[0] = 128

        last = T0 - 1

        def zero_body(g, carry):
            for sec in range(3):
                dst, off = qkv_dst(last, sec)
                dst[g, pl.ds(off, TM), :] = jnp.zeros((TM, 128), f32)
            return carry
        jax.lax.fori_loop(0, NG, zero_body, 0)
        wait(cp_c())
        c = c_v[...].astype(f32)
        sc = c * jax.nn.sigmoid(c)
        st_v[...] = jnp.transpose(jnp.broadcast_to(sc, (128, D)))

        def normalize(row0, nrows, chains=None):
            for i in range(nrows // LNR):
                r0 = row0 + i * LNR
                x = x_v[pl.ds(r0, LNR), :].astype(f32)
                if chains is not None:
                    x = chains[i % len(chains)].after_rows(x)
                r, mr = _ln_stats(x)
                xn = x * r - mr
                if chains is not None:
                    chains[i % len(chains)].tok = xn[0:8, 0:128]
                for g in range(NG):
                    xn_s[g, pl.ds(r0, LNR), :] = xn[:, g * 128:(g + 1) * 128]

        def mod_chunk(k):
            col = k * KC if isinstance(k, int) else pl.multiple_of(k * KC, KC)
            sa = _mod_cols(wmod_v, st_v, col, KC)
            ca = _mod_cols(wmod_v, st_v, D + col, KC)
            mod_v[:, pl.ds(col, KC)] = jnp.broadcast_to(sa, (8, KC))
            mod_v[:, pl.ds(D + col, KC)] = jnp.broadcast_to(ca, (8, KC))
            return sa, 1.0 + ca

        def h_chunk(k, t, n, sa, ca1):
            return (xn_s[k, pl.ds(t * TM, n * TM), :] * ca1 + sa).astype(bf16)

        def mm(h, w, sec, tiles, first):
            res = _dot(h, _unpack(w))
            for i, t in enumerate(tiles):
                dst, off = qkv_dst(t, sec)
                for g in range(NG):
                    blk = res[i * TM:(i + 1) * TM, g * 128:(g + 1) * 128]
                    if first:
                        dst[g, pl.ds(off, TM), :] = blk
                    else:
                        dst[g, pl.ds(off, TM), :] += blk

        def wcur(sec):
            return wcur_s[:, sec * D:(sec + 1) * D]

        def keep(k, sec, wp):
            r0 = k * (KC // 2) if isinstance(k, int) else pl.multiple_of(k * (KC // 2), KC // 2)
            cols = pl.ds(sec * D if isinstance(sec, int) else pl.multiple_of(sec * D, D), D)
            wcur_s[:, cols] = wp
            wqkv_p[pl.ds(r0, KC // 2), cols] = wp

        scope = jax.named_scope
        mod0 = lambda: (mod_v[0:1, 0:KC], 1.0 + mod_v[0:1, D:D + KC])
        with scope('w_wq0'):
            wait(cp_wq0())
        with scope('perm0'):
            def perm_body(sec, carry):
                keep(0, sec, _permute_qkv_section(wqkv_raw, 0, sec))
                return carry
            jax.lax.fori_loop(0, 3, perm_body, 0)
        with scope('w_x0'):
            wait(cp_x(0))
        with scope('norm0'):
            def norm_body(i, carry):
                normalize(pl.multiple_of(i * 64, 64), 64)
                return carry
            jax.lax.fori_loop(0, TM // 64, norm_body, 0)
        with scope('w_m0'):
            wait(cp_chunk(0, False), cp_x(1))
        with scope('mm00'):
            sa, ca1 = mod_chunk(0)
            h0 = h_chunk(0, 0, 1, sa, ca1)
            for sec in range(3):
                mm(h0, wcur(sec), sec, [0], True)
            normalize(TM, TM, [new_chain() for _ in range(4)])
        with scope('w_x2'):
            wait(cp_x(2))
        with scope('mm01'):
            h1 = h_chunk(0, 1, 1, *mod0())
            for sec in range(3):
                mm(h1, wcur(sec), sec, [1], True)
            normalize(2 * TM, TM, [new_chain() for _ in range(4)])
            hl_s[...] = _pack(h_chunk(0, last, 1, *mod0()))

        def chunk_body(k0, carry):
            k = k0 + 1
            with scope('w_chunk'):
                wait(cp_chunk(k))
            with scope('chunk'):
                hl = _unpack(hl_s[...])
                for sec in range(3):
                    mm(hl, wcur(sec), sec, [last], False)
                sa, ca1 = mod_chunk(k)
                hf = h_chunk(k, 0, last, sa, ca1)
                hl_s[...] = _pack(h_chunk(k, last, 1, sa, ca1))
                for sec in range(3):
                    wp = _permute_qkv_section(wqkv_raw, pl.multiple_of(k * KC, KC), sec)
                    mm(hf, wp, sec, list(range(last)), False)
                    keep(k, sec, wp)
            return carry
        jax.lax.fori_loop(0, NKC - 1, chunk_body, 0)

        with scope('w_x3'):
            wait(cp_x(T0))
        hl = _unpack(hl_s[...])
        for sec in range(3):
            mm(hl, wcur(sec), sec, [last], False)
        _ln1_next(x_v, mod_v, h_s, T0 * TM, [new_chain() for _ in range(4)])
        k0_s[:, 0:HALO, :] = jnp.zeros((NG, HALO, 128), f32)
        v0_s[:, 0:HALO, :] = jnp.broadcast_to(v0_s[:, HALO:HALO + 1, :], (NG, HALO, 128))
        k_s[:, 0:HALO, :] = k0_s[:, TM:TM + HALO, :]
        v_s[:, 0:HALO, :] = v0_s[:, TM:TM + HALO, :]

    @_when(step == 1, 'wait1')
    def _():
        wait(cp_x(4), cp_wo(0), cp_ff(0))

    @_when(step == 2, 'wait2')
    def _():
        wait(cp_x(5), cp_wm(0), cp_ff(1))

    @_when(step == 3, 'wait3')
    def _():
        wait(cp_x(6), cp_wo(1), cp_wm(1), cp_ff(2))

    @_when(step == 4, 'wait4')
    def _():
        wait(cp_x(7), cp_wm(2), cp_ff(3))

    @_when(step == 5, 'wait5')
    def _():
        wait(cp_wm(3), cp_ff(4))

    @_when(jnp.logical_and(step >= 1, step < N1), 'phase1')
    def _():
        _phase1(step, x_v, wqkv_p, wo_raw, wo_p, w1_v, w3_v, w2_v, s1_v, s3_v, s2_v, wmod_v, mod_v, st_v,
                h_s, q0_s, k0_s, v0_s, q_s, k_s, v_s, o_s, flag_s)

    def cp_out(j):
        rows = pl.ds(pl.multiple_of(j * TM, TM), TM)
        return pltpu.make_async_copy(o_ref.at[j % 2], o_hbm.at[rows], sems.at[SEM_OUT + j % 2])

    @_when(step > N1 + 1, 'wait_out')
    def _():
        cp_out(step - N1 - 2).wait()

    @_when(step >= N1, 'phase2')
    def _():
        _phase2(step, x_v, wo_p, w1_v, w3_v, w2_v, s1_v, s3_v, s2_v, mod_v, q_s, k_s, v_s, o_s, flag_s,
                o_ref.at[(step - N1) % 2])
        cp_out(step - N1).start()

    @_when(step == N1 + NT - 1, 'wait_last')
    def _():
        cp_out(NT - 2).wait()
        cp_out(NT - 1).wait()


def _scratch_shapes():
    return [
        pltpu.VMEM((S, D), bf16),
        pltpu.VMEM((D, 3 * D), bf16),
        pltpu.VMEM((D // 2, 3 * D), u32),
        pltpu.VMEM((D, D), bf16),
        pltpu.VMEM((D // 2, D), u32),
        pltpu.VMEM((D, F), bf16),
        pltpu.VMEM((D, F), bf16),
        pltpu.VMEM((F, D), bf16),
        pltpu.VMEM((5, DH2 // PK, FH), bf16 if PK == 1 else u32),
        pltpu.VMEM((5, DH2 // PK, FH), bf16 if PK == 1 else u32),
        pltpu.VMEM((5, FH // PK, DH2), bf16 if PK == 1 else u32),
        pltpu.VMEM((D, 6 * D), bf16),
        pltpu.VMEM((8, 6 * D), f32),
        pltpu.VMEM((D, 128), f32),
        pltpu.VMEM((NG, T0 * TM, 128), f32),
        pltpu.VMEM((KC // 2, 3 * D), u32),
        pltpu.VMEM((TM // 2, KC), u32),
        pltpu.VMEM((TM, D), bf16),
        pltpu.VMEM((NG, TM, 128), f32),
        pltpu.VMEM((NG, HALO + TM, 128), f32),
        pltpu.VMEM((NG, HALO + TM, 128), f32),
        pltpu.VMEM((NG, S - TM, 128), f32),
        pltpu.VMEM((NG, HALO + S - TM, 128), f32),
        pltpu.VMEM((NG, HALO + S - TM, 128), f32),
        pltpu.VMEM((TM, D), bf16),
        pltpu.VMEM((2, TM, D), bf16),
        pltpu.VMEM((1, D), bf16),
        pltpu.SMEM((1,), jnp.int32),
        pltpu.SemaphoreType.DMA((NSEM,)),
    ]


@jax.jit
def pallas_adaLN_cond__sliding_local_dilated__glu_gated_swiglu__prompt_kernel(
    A_x: jax.Array,
    A_wqkv: jax.Array,
    A_wo: jax.Array,
    B_x: jax.Array,
    B_w1: jax.Array,
    B_w3: jax.Array,
    B_w2: jax.Array,
    c: jax.Array,
    w_mod: jax.Array,
):
    del B_x
    x = A_x.reshape(S, D)
    hbm = pl.BlockSpec(memory_space=pl.ANY)
    out = pl.pallas_call(
        _kernel,
        grid=(N1 + NT,),
        in_specs=[hbm] * 8,
        out_specs=hbm,
        out_shape=jax.ShapeDtypeStruct((S, D), A_x.dtype),
        scratch_shapes=_scratch_shapes(),
        compiler_params=pltpu.CompilerParams(
            dimension_semantics=("arbitrary",),
            vmem_limit_bytes=118 * 1024 * 1024,
        ),
        name="adaln_attn_ffn",
    )(x, c, A_wqkv, A_wo, B_w1, B_w3, B_w2, w_mod)
    return out.reshape(1, S, D)
```

```python
import jax
import jax.numpy as jnp
import jax.experimental.pallas as pl
import jax.experimental.pallas.tpu as pltpu

S, D, F = 2048, 1024, 3584
H, DH, W, DIL = 32, 32, 8, 2
NG = D // 128
TM = 256
NT = S // TM
T0 = 3
N1 = NT - T0 + 1
SUB = 64
HN = 256
FH = F // 2
DH2 = D // 2
KC = 128
NKC = D // KC
RU1 = 112
RU2 = 368
HALO = 16
PARTS = 'LMA'
SMODE = 'be'
EARLY = (0, 0)
PACE = 0
PK = 1
APULL = 99
NPULL = 3
PVS = 4
MR = 64
LNS = 2
NGRP = 2
NSEP = 1
UR = 8
UC = 256
NW = 1
PULL0 = 2
SLINK = True
SW = 256
WB1 = 1
WB2 = 1
LNR = 16
EPS = 1e-5
SCALE = DH ** -0.5
LOG2E = 1.4426950408889634
QSCALE = SCALE * LOG2E
NEG = -1000000000.0 * LOG2E

f32 = jnp.float32
bf16 = jnp.bfloat16
u32 = jnp.uint32

SEM_C = 0
SEM_X = 1
SEM_WQ0 = SEM_X + NT
SEM_CH = SEM_WQ0 + 1
SEM_WM = SEM_CH + NKC
SEM_WO = SEM_WM + 4
SEM_FF = SEM_WO + 2
SEM_OUT = SEM_FF + (N1 - 1)
NSEM = SEM_OUT + 2


def _when(cond, name):
    def deco(body):
        def scoped():
            with jax.named_scope(name):
                body()
        return pl.when(cond)(scoped)
    return deco


def _pack(x):
    return pltpu.bitcast(x, u32)


def _unpack(x):
    return pltpu.bitcast(x, bf16)


def _spack(x):
    return x if PK == 1 else _pack(x)


def _sunpack(x):
    return x if PK == 1 else _unpack(x)


def _dot(a, b):
    return jnp.dot(a, b, preferred_element_type=f32)


class _Chain:
    def __init__(self, always):
        self.always = always
        self.tok = None

    def after(self, x):
        if self.tok is None:
            return x
        t = self.tok if self.tok.dtype == x.dtype else pltpu.bitcast(self.tok, x.dtype)
        return jnp.where(self.always, x, t)

    def pace(self, done, n):
        t = done
        if self.tok is not None and n > 0:
            d = self.tok
            for _ in range(n):
                d = jnp.tanh(d)
            t = d + t
        self.tok = t

    def after_rows(self, x):
        x00 = self.after(x[0:8, 0:128])
        top = x00 if x.shape[1] == 128 else jnp.concatenate([x00, x[0:8, 128:]], axis=1)
        return top if x.shape[0] == 8 else jnp.concatenate([top, x[8:]], axis=0)


def _swap_stage(a, k, b, axis):
    n = 128 if axis == 1 else 8
    idx = jax.lax.broadcasted_iota(jnp.int32, a[0].shape, axis)
    m0 = (idx & (1 << b)) == 0
    out = list(a)
    for c in range(8):
        if c & (1 << k):
            continue
        lo, hi = a[c], a[c | (1 << k)]
        out[c] = jnp.where(m0, lo, pltpu.roll(hi, 1 << b, axis))
        out[c | (1 << k)] = jnp.where(m0, pltpu.roll(lo, n - (1 << b), axis), hi)
    return out


def _permute_qkv_section(w_ref, r0, sec):
    c0 = sec * D if isinstance(sec, int) else pl.multiple_of(sec * D, D)
    a = [_pack(w_ref[pl.ds(r0, KC), pl.ds(c0 + c * 128, 128)]) for c in range(8)]
    for k in range(3):
        a = _swap_stage(a, k, k + 1, 1)
    return jnp.concatenate(a, axis=1)


def _ln_stats(x):
    m = jnp.mean(x, axis=-1, keepdims=True)
    xc = x - m
    v = jnp.mean(xc * xc, axis=-1, keepdims=True)
    r = jax.lax.rsqrt(v + EPS)
    return r, m * r


def _modulated_ln(x, scale1, shift):
    r, mr = _ln_stats(x)
    return (x * r - mr) * scale1 + shift


def _attention_rows(q_s, k_s, v_s, q0, row0, wb, pv, chain=None, nr=8):
    lane = jax.lax.broadcasted_iota(jnp.int32, (nr, 128), 1)
    m0 = (lane & 1) == 0
    m4 = (lane & 16) == 0
    qscale = QSCALE if chain is None else jnp.concatenate(
        [chain.after(jnp.full((8, 128), QSCALE, f32))] * (nr // 8), axis=0)
    q = q_s[:, pl.ds(q0, nr), :] * qscale
    logits = []
    for w0 in range(0, W, wb):
        zs = [jnp.sum(q * k_s[:, pl.ds(q0 + (HALO - DIL * w), nr), :], axis=0)
              for w in range(w0, w0 + wb)]
        zs = [z + jnp.where(m0, pltpu.roll(z, 127, 1), pltpu.roll(z, 1, 1)) for z in zs]
        zs = [z + jnp.where(m4, pltpu.roll(z, 112, 1), pltpu.roll(z, 16, 1)) for z in zs]
        for w, z in zip(range(w0, w0 + wb), zs):
            if w > 0 and row0 is not None:
                row = jax.lax.broadcasted_iota(jnp.int32, (nr, 128), 0) + row0
                z = jnp.where(row >= DIL * w, z, NEG)
            logits.append(z)
    m = logits[0]
    for w in range(1, W):
        m = jnp.maximum(m, logits[w])
    e = [jnp.exp2(logits[w] - m) for w in range(W)]
    den = e[0]
    for w in range(1, W):
        den = den + e[w]
    inv = pl.reciprocal(den, approx=False)
    outs = []
    gs = NG // PVS
    for g0 in range(0, NG, gs):
        o = None
        for w in range(W):
            ew = e[w]
            if w == 0:
                ew = pv.after(ew)
            p = ew * v_s[g0:g0 + gs, pl.ds(q0 + (HALO - DIL * w), nr), :]
            o = p if o is None else o + p
        o = o * inv
        outs += [o[g] for g in range(gs)]
        pv.tok = outs[-1]
    if chain is not None:
        chain.tok = outs[-1][0:8]
    return jnp.concatenate(outs, axis=1)


def _attention(q_s, k_s, v_s, o_s, q0, o0, nrows, wb, pv):
    toks = []
    for r in range(0, nrows, 8):
        pv.tok = None
        o = _attention_rows(q_s, k_s, v_s, q0 + r, None, wb, pv)
        o_s[pl.ds(o0 + r, 8), :] = o.astype(bf16)
        toks.append(pv.tok)
    return toks


def _mod_cols(wmod_v, st_v, col, n, chain=None):
    acc = None
    for r in range(0, D, MR):
        s = st_v[r:r + MR, :]
        if r == 0 and chain is not None:
            s = chain.after_rows(s)
        if n > 128:
            s = jnp.concatenate([s] * (n // 128), axis=1)
        p = wmod_v[r:r + MR, pl.ds(col, n)].astype(f32) * s
        for i in range(0, MR, 8):
            acc = p[i:i + 8] if acc is None else acc + p[i:i + 8]
    if chain is not None:
        chain.tok = acc[:, 0:128]
    return acc.sum(axis=0, keepdims=True)


def _lhs_operands(a11, a12, a21, a22):
    return [a11 + a22, a21 + a22, a11, a22, a11 + a12, a21 - a11, a12 - a22]


def _rhs_sums(b11, b12, b21, b22):
    return (b11 + b22, b12 - b22, b21 - b11, b11 + b12, b21 + b22)


def _rhs_operands(sums, b11, b22):
    return [sums(0), b11, sums(1), sums(2), b22, sums(3), sums(4)]


def _combine(m):
    return (m[0] + m[3] - m[4] + m[6], m[2] + m[4], m[1] + m[3], m[0] - m[1] + m[2] + m[5])


def _new_chain(flag_s):
    return _Chain(jax.lax.broadcasted_iota(jnp.int32, (8, 128), 1) < flag_s[0])


def _ln1_next(x_v, mod_v, h_s, r0, chains, extra=None):
    sa = mod_v[0:1, 0 * D:1 * D]
    ca1 = 1.0 + mod_v[0:1, 1 * D:2 * D]
    for i, r in enumerate(range(0, TM, LNR)):
        chain = chains[i % len(chains)]
        x = chain.after_rows(x_v[pl.ds(r0 + r, LNR), :].astype(f32))
        h = _modulated_ln(x, ca1, sa)
        chain.tok = h[0:8, 0:128]
        h_s[pl.ds(r, LNR), :] = h.astype(bf16)
        if extra is not None:
            extra(i)


def _phase1(step, x_v, wqkv_p, wo_raw, wo_p, w1_v, w3_v, w2_v, s1_v, s3_v, s2_v, wmod_v, mod_v, st_v,
            h_s, q0_s, k0_s, v0_s, q_s, k_s, v_s, o_s, flag_s):
    step = jnp.clip(step, 1, N1 - 1)
    part = jnp.maximum(step - 2, 0)
    base = pl.multiple_of((step + T0 - 2) * TM, TM)
    h = h_s[...]
    chain = _new_chain(flag_s)

    ln_r0 = pl.multiple_of(jnp.minimum(step + T0, NT - 1) * TM, TM)
    sa = mod_v[0:1, 0 * D:1 * D]
    ca1 = 1.0 + mod_v[0:1, 1 * D:2 * D]

    def ln_unit(i, nr=LNR):
        x = x_v[pl.ds(ln_r0 + i * nr, nr), :].astype(f32)
        x = jnp.concatenate([chain.after_rows(x[r:r + 8]) for r in range(0, nr, 8)], axis=0)
        hn = _modulated_ln(x, ca1, sa)
        chain.tok = hn[0:8, 0:128]
        h_s[pl.ds(i * nr, nr), :] = hn.astype(bf16)

    def wo_unit(i):
        gg, mid = i // 8, i % 8
        col = pl.ds(pl.multiple_of(part * 256 + gg * 128, 128), 128)
        a = [_pack(wo_raw[pl.ds(c * 128 + mid * 16, 16), col]) for c in range(8)]
        a[0] = chain.after(a[0])
        for k in range(3):
            a = _swap_stage(a, k, k, 0)
        for s in range(8):
            wo_p[pl.ds(s * 64 + mid * 8, 8), col] = a[s]
        chain.tok = a[7]

    at_r0 = pl.multiple_of(part * 64, 64)
    pv1 = _new_chain(flag_s)

    def attn_unit(i, nr=8):
        o = _attention_rows(q0_s, k0_s, v0_s, at_r0 + i * nr,
                            at_r0 + i * nr if i * nr < HALO else None, WB1, pv1, chain, nr)
        o_s[pl.ds(at_r0 + i * nr, nr), :] = o.astype(bf16)

    mod_col = pl.multiple_of(step * D, D)

    def mod_unit(i):
        col = pl.multiple_of(mod_col + i * 256, 256)
        val = _mod_cols(wmod_v, st_v, col, 256, chain)
        mod_v[:, pl.ds(col, 256)] = jnp.broadcast_to(val, (8, 256))

    sum_units = []
    for w_v, s_v, half, ru, ch in ((w1_v, s1_v, DH2, RU1, FH), (w3_v, s3_v, DH2, RU1, FH),
                                   (w2_v, s2_v, FH, RU2, DH2)):
        r_lo = jnp.minimum((step - 1) * (ru // 16), (half - ru) // 16)
        srcs = [w_v.at[pl.ds(pl.multiple_of(i * half + r_lo * 16, 16), ru)] for i in range(2)]
        dst = s_v.at[:, pl.ds(pl.multiple_of(r_lo * (16 // PK), 16 // PK), ru // PK)]
        r_bk = jnp.clip(r_lo + flag_s[0] - 128, 0, (half - ru) // 16)
        back = s_v.at[:, pl.ds(pl.multiple_of(r_bk * (16 // PK), 16 // PK), ru // PK)]
        sum_units += [(srcs, dst, back, ch, r, c0)
                      for r in range(0, ru, UR) for c0 in range(0, ch, UC)]

    def sum_unit(u):
        srcs, dst, back, ch, r, c0 = sum_units[u]
        q = [srcs[i][r:r + UR, j * ch + c0:j * ch + c0 + UC].astype(f32)
             for i in range(2) for j in range(2)]
        q[0] = chain.after_rows(q[0])
        dst[:, r:r + UR, c0:c0 + UC] = jnp.stack(_rhs_sums(*q)).astype(bf16)
        chain.tok = back[0, 0:8, 0:128].astype(f32)

    def mm_unit(t, gated):
        sec, g = t // NG, t % NG
        dst, off = (q_s, k_s, v_s)[sec], (0 if sec == 0 else HALO)
        w = wqkv_p[:, t * 128:(t + 1) * 128]
        if gated:
            w = chain.after_rows(w)
        res = _dot(h, _unpack(w))
        dst[g, pl.ds(base + off, TM), :] = res
        return res[0:8]

    PLAN(chain, mm_unit, ln_unit, wo_unit, attn_unit, mod_unit, sum_unit, len(sum_units))


def PLAN(chain, mm_unit, ln_unit, wo_unit, attn_unit, mod_unit, sum_unit, nsum):
    ticks = [mm_unit(t, False) for t in range(3 * NG)]
    done = 0
    for t in range(3 * NG - 1):
        chain.tok = ticks[t]
        if t < 8:
            ln_unit(t, 32)
            wo_unit(2 * t)
            wo_unit(2 * t + 1)
        if 15 <= t < 19:
            mod_unit(t - 15)
        n = 10 if (t < 8 or 15 <= t < 19) else -(-(nsum - 120) // 11)
        for u in range(done, min(done + n, nsum)):
            sum_unit(u)
        done = min(done + n, nsum)
    assert done == nsum
    for i in range(8):
        chain.tok = None
        attn_unit(i)


def _phase2(step, x_v, wo_p, w1_v, w3_v, w2_v, s1_v, s3_v, s2_v, mod_v, q_s, k_s, v_s, o_s, flag_s,
            o_ref):
    j2 = jnp.clip(step - N1, 0, NT - 1)
    ga = mod_v[0:1, 2 * D:3 * D]
    sb = mod_v[0:1, 3 * D:4 * D]
    cb1 = 1.0 + mod_v[0:1, 4 * D:5 * D]
    gb = mod_v[0:1, 5 * D:6 * D]
    row0 = pl.multiple_of(j2 * TM, TM)
    nsub = TM // SUB
    os_ = [o_s[pl.ds(s * SUB, SUB), :] for s in range(nsub)]
    x1s, blocks = [], []
    for s in range(nsub):
        att = _dot(os_[s], _unpack(wo_p[...]))
        x1 = x_v[pl.ds(row0 + s * SUB, SUB), :].astype(f32) + ga * att
        x1s.append(x1)
        chain = _new_chain(flag_s)
        for r in range(0, SUB, 32):
            xb = x1[r:r + 32]
            xb = jnp.concatenate([chain.after_rows(xb[0:16]), chain.after_rows(xb[16:32])], axis=0)
            rs, mr = _ln_stats(xb)
            chain.tok = None
            pieces = []
            cw = DH2 // LNS
            for c in range(0, DH2, cw):
                hl, hr = [(chain.after_rows(xb[:, c0:c0 + cw]) * rs - mr) * cb1[:, c0:c0 + cw]
                          + sb[:, c0:c0 + cw] for c0 in (c, DH2 + c)]
                pieces.append(_lhs_operands(hl[0:16], hr[0:16], hl[16:32], hr[16:32]))
                chain.tok = hr[24:32, cw - 128:cw]
            blocks.append([jnp.concatenate([pc[i] for pc in pieces], axis=1) for i in range(7)])

    nq = pl.multiple_of(jnp.minimum(j2, NT - 2) * TM, TM)

    def stack(per_group):
        return [jnp.concatenate([ops[i] for ops in per_group], axis=0) for i in range(7)]

    nb = len(blocks) // NGRP
    groups = [stack(blocks[g * nb:(g + 1) * nb]) for g in range(NGRP)]

    def up_proj(a, w_v, s_v, j):
        c0 = j * HN
        b = _rhs_operands(lambda i: _sunpack(s_v[i, :, c0:c0 + HN]),
                          w_v[0:DH2, c0:c0 + HN], w_v[DH2:, FH + c0:FH + c0 + HN])
        return _combine([_dot(a[i], b[i]) for i in range(7)])

    def to_mxu(ops):
        return [v.astype(bf16) for v in ops]

    def gate_up(a, j):
        act = []
        for g, u in zip(up_proj(a, w1_v, s1_v, j), up_proj(a, w3_v, s3_v, j)):
            hg = 0.5 * g
            act.append((hg + hg * jnp.tanh(hg)) * u)
        return _lhs_operands(*act)

    h_all = to_mxu(stack(groups))
    sep = []
    done = _new_chain(flag_s)
    for g, ops in enumerate(groups):
        sep.append([gate_up(to_mxu(ops), j) for j in range(NSEP)])
        rows = TM // NGRP
        toks = _attention(q_s, k_s, v_s, o_s, nq + g * rows, g * rows, rows, WB2, done)
    done.tok = sum(toks[-NPULL:-1], toks[-1])
    acc = None
    for j in range(FH // HN):
        a = stack([sp[j] for sp in sep]) if j < NSEP else gate_up(h_all, j)
        if j == APULL:
            a[0] = done.after_rows(a[0])
        a = to_mxu(a)
        r0 = j * HN
        b = _rhs_operands(lambda i: _sunpack(s2_v[i, r0 // PK:(r0 + HN) // PK, :]),
                          w2_v[r0:r0 + HN, 0:DH2], w2_v[FH + r0:FH + r0 + HN, DH2:])
        m = [_dot(a[i], b[i]) for i in range(7)]
        acc = m if acc is None else [p + q for p, q in zip(acc, m)]
    c11, c12, c21, c22 = _combine(acc)
    x1 = jnp.concatenate(x1s, axis=0)
    for blk in range(TM // 32):
        rows = slice(blk * 16, (blk + 1) * 16)
        for t, (left, right) in enumerate(((c11, c12), (c21, c22))):
            y = jnp.concatenate([left[rows], right[rows]], axis=1)
            r = blk * 32 + t * 16
            o_ref[r:r + 16, :] = (x1[r:r + 16] + gb * y).astype(o_ref.dtype)


def _kernel(x_hbm, c_hbm, wqkv_hbm, wo_hbm, w1_hbm, w3_hbm, w2_hbm, wmod_hbm, o_hbm,
            x_v, wqkv_raw, wqkv_p, wo_raw, wo_p, w1_v, w3_v, w2_v, s1_v, s3_v, s2_v,
            wmod_v, mod_v, st_v, xn_s, wcur_s, hl_s, h_s, q0_s, k0_s, v0_s, q_s, k_s, v_s,
            o_s, o_ref, c_v, flag_s, sems):
    step = pl.program_id(0)

    def new_chain():
        return _new_chain(flag_s)

    def cp_rows(src, dst, r0, n, sem):
        rows = pl.ds(r0, n)
        return pltpu.make_async_copy(src.at[rows], dst.at[rows], sems.at[sem])

    def cp_cols(src, dst, c0, n, sem):
        cols = pl.ds(c0, n)
        return pltpu.make_async_copy(src.at[:, cols], dst.at[:, cols], sems.at[sem])

    cp_c = lambda: [pltpu.make_async_copy(c_hbm, c_v, sems.at[SEM_C])]
    cp_x = lambda i: [cp_rows(x_hbm, x_v, i * TM, TM, SEM_X + i)]
    cp_wq0 = lambda: [cp_rows(wqkv_hbm, wqkv_raw, 0, KC, SEM_WQ0)]
    cp_wm = lambda p: [cp_cols(wmod_hbm, wmod_v, (2 + p) * D, D, SEM_WM + p)]

    def cp_chunk(k, with_wq=True):
        cps = [cp_rows(wqkv_hbm, wqkv_raw, k * KC, KC, SEM_CH + k)] if with_wq else []
        return cps + [cp_cols(wmod_hbm, wmod_v, k * KC, KC, SEM_CH + k),
                      cp_cols(wmod_hbm, wmod_v, D + k * KC, KC, SEM_CH + k)]

    def cp_wo(i):
        c0, n = (0, 256) if i == 0 else (256, D - 256)
        return [cp_cols(wo_hbm, wo_raw, c0, n, SEM_WO + i)]

    def cp_ff(i):
        cps = []
        for src, dst, half, ru in ((w1_hbm, w1_v, DH2, RU1), (w3_hbm, w3_v, DH2, RU1),
                                   (w2_hbm, w2_v, FH, RU2)):
            n = min(ru, half - i * ru)
            cps += [cp_rows(src, dst, h * half + i * ru, n, SEM_FF + i) for h in range(2)]
        return cps

    def wait(*groups):
        for cps in groups:
            for cp in cps:
                cp.wait()

    def qkv_dst(t, sec):
        off = 0 if sec == 0 else HALO
        if t == 0:
            return (q0_s, k0_s, v0_s)[sec], off
        return (q_s, k_s, v_s)[sec], off + (t - 1) * TM

    @_when(step == 0, 'first')
    def _first():
        order = cp_c() + cp_x(0) + cp_wq0() + cp_chunk(0, False) + cp_x(1) + cp_x(2)
        for k in range(1, NKC):
            order += cp_chunk(k)
        order += cp_x(3) + cp_x(4) + cp_wo(0) + cp_ff(0)
        order += cp_x(5) + cp_wm(0) + cp_ff(1)
        order += cp_x(6) + cp_wo(1) + cp_wm(1) + cp_ff(2)
        order += cp_x(7) + cp_wm(2) + cp_ff(3)
        order += cp_wm(3) + cp_ff(4)
        for cp in order:
            cp.start()
        flag_s[0] = 128

        last = T0 - 1

        def zero_body(g, carry):
            for sec in range(3):
                dst, off = qkv_dst(last, sec)
                dst[g, pl.ds(off, TM), :] = jnp.zeros((TM, 128), f32)
            return carry
        jax.lax.fori_loop(0, NG, zero_body, 0)
        wait(cp_c())
        c = c_v[...].astype(f32)
        sc = c * jax.nn.sigmoid(c)
        st_v[...] = jnp.transpose(jnp.broadcast_to(sc, (128, D)))

        def normalize(row0, nrows, chains=None):
            for i in range(nrows // LNR):
                r0 = row0 + i * LNR
                x = x_v[pl.ds(r0, LNR), :].astype(f32)
                if chains is not None:
                    x = chains[i % len(chains)].after_rows(x)
                r, mr = _ln_stats(x)
                xn = x * r - mr
                if chains is not None:
                    chains[i % len(chains)].tok = xn[0:8, 0:128]
                for g in range(NG):
                    xn_s[g, pl.ds(r0, LNR), :] = xn[:, g * 128:(g + 1) * 128]

        def mod_chunk(k):
            col = k * KC if isinstance(k, int) else pl.multiple_of(k * KC, KC)
            sa = _mod_cols(wmod_v, st_v, col, KC)
            ca = _mod_cols(wmod_v, st_v, D + col, KC)
            mod_v[:, pl.ds(col, KC)] = jnp.broadcast_to(sa, (8, KC))
            mod_v[:, pl.ds(D + col, KC)] = jnp.broadcast_to(ca, (8, KC))
            return sa, 1.0 + ca

        def h_chunk(k, t, n, sa, ca1):
            return (xn_s[k, pl.ds(t * TM, n * TM), :] * ca1 + sa).astype(bf16)

        def mm(h, w, sec, tiles, first):
            res = _dot(h, _unpack(w))
            for i, t in enumerate(tiles):
                dst, off = qkv_dst(t, sec)
                for g in range(NG):
                    blk = res[i * TM:(i + 1) * TM, g * 128:(g + 1) * 128]
                    if first:
                        dst[g, pl.ds(off, TM), :] = blk
                    else:
                        dst[g, pl.ds(off, TM), :] += blk

        def wcur(sec):
            return wcur_s[:, sec * D:(sec + 1) * D]

        def keep(k, sec, wp):
            r0 = k * (KC // 2) if isinstance(k, int) else pl.multiple_of(k * (KC // 2), KC // 2)
            cols = pl.ds(sec * D if isinstance(sec, int) else pl.multiple_of(sec * D, D), D)
            wcur_s[:, cols] = wp
            wqkv_p[pl.ds(r0, KC // 2), cols] = wp

        scope = jax.named_scope
        mod0 = lambda: (mod_v[0:1, 0:KC], 1.0 + mod_v[0:1, D:D + KC])
        with scope('w_x0'):
            wait(cp_x(0))
        with scope('norm0'):
            def norm_body(i, carry):
                normalize(pl.multiple_of(i * 64, 64), 64)
                return carry
            jax.lax.fori_loop(0, TM // 64, norm_body, 0)
        with scope('w_wq0'):
            wait(cp_wq0())
        with scope('perm0'):
            def perm_body(sec, carry):
                keep(0, sec, _permute_qkv_section(wqkv_raw, 0, sec))
                return carry
            jax.lax.fori_loop(0, 3, perm_body, 0)
        with scope('w_m0'):
            wait(cp_chunk(0, False), cp_x(1))
        with scope('mm00'):
            sa, ca1 = mod_chunk(0)
            h0 = h_chunk(0, 0, 1, sa, ca1)
            for sec in range(3):
                mm(h0, wcur(sec), sec, [0], True)
            normalize(TM, TM, [new_chain() for _ in range(4)])
        with scope('w_x2'):
            wait(cp_x(2))
        with scope('mm01'):
            h1 = h_chunk(0, 1, 1, *mod0())
            for sec in range(3):
                mm(h1, wcur(sec), sec, [1], True)
            normalize(2 * TM, TM, [new_chain() for _ in range(4)])
            hl_s[...] = _pack(h_chunk(0, last, 1, *mod0()))

        def chunk_body(k0, carry):
            k = k0 + 1
            with scope('w_chunk'):
                wait(cp_chunk(k))
            with scope('chunk'):
                hl = _unpack(hl_s[...])
                for sec in range(3):
                    mm(hl, wcur(sec), sec, [last], False)
                sa, ca1 = mod_chunk(k)
                hf = h_chunk(k, 0, last, sa, ca1)
                hl_s[...] = _pack(h_chunk(k, last, 1, sa, ca1))
                for sec in range(3):
                    wp = _permute_qkv_section(wqkv_raw, pl.multiple_of(k * KC, KC), sec)
                    mm(hf, wp, sec, list(range(last)), False)
                    keep(k, sec, wp)
            return carry
        jax.lax.fori_loop(0, NKC - 1, chunk_body, 0)

        with scope('w_x3'):
            wait(cp_x(T0))
        hl = _unpack(hl_s[...])
        for sec in range(3):
            mm(hl, wcur(sec), sec, [last], False)
        _ln1_next(x_v, mod_v, h_s, T0 * TM, [new_chain() for _ in range(4)])
        k0_s[:, 0:HALO, :] = jnp.zeros((NG, HALO, 128), f32)
        v0_s[:, 0:HALO, :] = jnp.broadcast_to(v0_s[:, HALO:HALO + 1, :], (NG, HALO, 128))
        k_s[:, 0:HALO, :] = k0_s[:, TM:TM + HALO, :]
        v_s[:, 0:HALO, :] = v0_s[:, TM:TM + HALO, :]

    @_when(step == 1, 'wait1')
    def _():
        wait(cp_x(4), cp_wo(0), cp_ff(0))

    @_when(step == 2, 'wait2')
    def _():
        wait(cp_x(5), cp_wm(0), cp_ff(1))

    @_when(step == 3, 'wait3')
    def _():
        wait(cp_x(6), cp_wo(1), cp_wm(1), cp_ff(2))

    @_when(step == 4, 'wait4')
    def _():
        wait(cp_x(7), cp_wm(2), cp_ff(3))

    @_when(step == 5, 'wait5')
    def _():
        wait(cp_wm(3), cp_ff(4))

    @_when(jnp.logical_and(step >= 1, step < N1), 'phase1')
    def _():
        _phase1(step, x_v, wqkv_p, wo_raw, wo_p, w1_v, w3_v, w2_v, s1_v, s3_v, s2_v, wmod_v, mod_v, st_v,
                h_s, q0_s, k0_s, v0_s, q_s, k_s, v_s, o_s, flag_s)

    def cp_out(j):
        rows = pl.ds(pl.multiple_of(j * TM, TM), TM)
        return pltpu.make_async_copy(o_ref.at[j % 2], o_hbm.at[rows], sems.at[SEM_OUT + j % 2])

    @_when(step > N1 + 1, 'wait_out')
    def _():
        cp_out(step - N1 - 2).wait()

    @_when(step >= N1, 'phase2')
    def _():
        _phase2(step, x_v, wo_p, w1_v, w3_v, w2_v, s1_v, s3_v, s2_v, mod_v, q_s, k_s, v_s, o_s, flag_s,
                o_ref.at[(step - N1) % 2])
        cp_out(step - N1).start()

    @_when(step == N1 + NT - 1, 'wait_last')
    def _():
        cp_out(NT - 2).wait()
        cp_out(NT - 1).wait()


def _scratch_shapes():
    return [
        pltpu.VMEM((S, D), bf16),
        pltpu.VMEM((D, 3 * D), bf16),
        pltpu.VMEM((D // 2, 3 * D), u32),
        pltpu.VMEM((D, D), bf16),
        pltpu.VMEM((D // 2, D), u32),
        pltpu.VMEM((D, F), bf16),
        pltpu.VMEM((D, F), bf16),
        pltpu.VMEM((F, D), bf16),
        pltpu.VMEM((5, DH2 // PK, FH), bf16 if PK == 1 else u32),
        pltpu.VMEM((5, DH2 // PK, FH), bf16 if PK == 1 else u32),
        pltpu.VMEM((5, FH // PK, DH2), bf16 if PK == 1 else u32),
        pltpu.VMEM((D, 6 * D), bf16),
        pltpu.VMEM((8, 6 * D), f32),
        pltpu.VMEM((D, 128), f32),
        pltpu.VMEM((NG, T0 * TM, 128), f32),
        pltpu.VMEM((KC // 2, 3 * D), u32),
        pltpu.VMEM((TM // 2, KC), u32),
        pltpu.VMEM((TM, D), bf16),
        pltpu.VMEM((NG, TM, 128), f32),
        pltpu.VMEM((NG, HALO + TM, 128), f32),
        pltpu.VMEM((NG, HALO + TM, 128), f32),
        pltpu.VMEM((NG, S - TM, 128), f32),
        pltpu.VMEM((NG, HALO + S - TM, 128), f32),
        pltpu.VMEM((NG, HALO + S - TM, 128), f32),
        pltpu.VMEM((TM, D), bf16),
        pltpu.VMEM((2, TM, D), bf16),
        pltpu.VMEM((1, D), bf16),
        pltpu.SMEM((1,), jnp.int32),
        pltpu.SemaphoreType.DMA((NSEM,)),
    ]


@jax.jit
def pallas_adaLN_cond__sliding_local_dilated__glu_gated_swiglu__prompt_kernel(
    A_x: jax.Array,
    A_wqkv: jax.Array,
    A_wo: jax.Array,
    B_x: jax.Array,
    B_w1: jax.Array,
    B_w3: jax.Array,
    B_w2: jax.Array,
    c: jax.Array,
    w_mod: jax.Array,
):
    del B_x
    x = A_x.reshape(S, D)
    hbm = pl.BlockSpec(memory_space=pl.ANY)
    out = pl.pallas_call(
        _kernel,
        grid=(N1 + NT,),
        in_specs=[hbm] * 8,
        out_specs=hbm,
        out_shape=jax.ShapeDtypeStruct((S, D), A_x.dtype),
        scratch_shapes=_scratch_shapes(),
        compiler_params=pltpu.CompilerParams(
            dimension_semantics=("arbitrary",),
            vmem_limit_bytes=118 * 1024 * 1024,
        ),
        name="adaln_attn_ffn",
    )(x, c, A_wqkv, A_wo, B_w1, B_w3, B_w2, w_mod)
    return out.reshape(1, S, D)
```

```python
import jax
import jax.numpy as jnp
import jax.experimental.pallas as pl
import jax.experimental.pallas.tpu as pltpu

S, D, F = 2048, 1024, 3584
H, DH, W, DIL = 32, 32, 8, 2
NG = D // 128
TM = 256
NT = S // TM
T0 = 3
N1 = NT - T0 + 1
SUB = 128
HN = 256
FH = F // 2
DH2 = D // 2
KC = 128
NKC = D // KC
RU1 = 112
RU2 = 368
HALO = 16
PARTS = 'LMA'
SMODE = 'be'
EARLY = (0, 0)
PACE = 0
PK = 1
PVS = 4
MR = 64
LNS = 2
NGRP = 2
NSEP = 1
UR = 8
UC = 256
NW = 1
PULL0 = 2
SLINK = True
SW = 256
WB1 = 1
WB2 = 1
LNR = 16
EPS = 1e-5
SCALE = DH ** -0.5
LOG2E = 1.4426950408889634
QSCALE = SCALE * LOG2E
NEG = -1000000000.0 * LOG2E

f32 = jnp.float32
bf16 = jnp.bfloat16
u32 = jnp.uint32

SEM_C = 0
SEM_X = 1
SEM_WQ0 = SEM_X + NT
SEM_CH = SEM_WQ0 + 1
SEM_WM = SEM_CH + NKC
SEM_WO = SEM_WM + 4
SEM_FF = SEM_WO + 2
SEM_OUT = SEM_FF + (N1 - 1)
NSEM = SEM_OUT + 2


def _when(cond, name):
    def deco(body):
        def scoped():
            with jax.named_scope(name):
                body()
        return pl.when(cond)(scoped)
    return deco


def _pack(x):
    return pltpu.bitcast(x, u32)


def _unpack(x):
    return pltpu.bitcast(x, bf16)


def _spack(x):
    return x if PK == 1 else _pack(x)


def _sunpack(x):
    return x if PK == 1 else _unpack(x)


def _dot(a, b):
    return jnp.dot(a, b, preferred_element_type=f32)


class _Chain:
    def __init__(self, always):
        self.always = always
        self.tok = None

    def after(self, x):
        if self.tok is None:
            return x
        t = self.tok if self.tok.dtype == x.dtype else pltpu.bitcast(self.tok, x.dtype)
        return jnp.where(self.always, x, t)

    def pace(self, done, n):
        t = done
        if self.tok is not None and n > 0:
            d = self.tok
            for _ in range(n):
                d = jnp.tanh(d)
            t = d + t
        self.tok = t

    def after_rows(self, x):
        x00 = self.after(x[0:8, 0:128])
        top = x00 if x.shape[1] == 128 else jnp.concatenate([x00, x[0:8, 128:]], axis=1)
        return top if x.shape[0] == 8 else jnp.concatenate([top, x[8:]], axis=0)


def _swap_stage(a, k, b, axis):
    n = 128 if axis == 1 else 8
    idx = jax.lax.broadcasted_iota(jnp.int32, a[0].shape, axis)
    m0 = (idx & (1 << b)) == 0
    out = list(a)
    for c in range(8):
        if c & (1 << k):
            continue
        lo, hi = a[c], a[c | (1 << k)]
        out[c] = jnp.where(m0, lo, pltpu.roll(hi, 1 << b, axis))
        out[c | (1 << k)] = jnp.where(m0, pltpu.roll(lo, n - (1 << b), axis), hi)
    return out


def _permute_qkv_section(w_ref, r0, sec):
    c0 = sec * D if isinstance(sec, int) else pl.multiple_of(sec * D, D)
    a = [_pack(w_ref[pl.ds(r0, KC), pl.ds(c0 + c * 128, 128)]) for c in range(8)]
    for k in range(3):
        a = _swap_stage(a, k, k + 1, 1)
    return jnp.concatenate(a, axis=1)


def _ln_stats(x):
    m = jnp.mean(x, axis=-1, keepdims=True)
    xc = x - m
    v = jnp.mean(xc * xc, axis=-1, keepdims=True)
    r = jax.lax.rsqrt(v + EPS)
    return r, m * r


def _modulated_ln(x, scale1, shift):
    r, mr = _ln_stats(x)
    return (x * r - mr) * scale1 + shift


def _attention_rows(q_s, k_s, v_s, q0, row0, wb, pv, chain=None, nr=8):
    lane = jax.lax.broadcasted_iota(jnp.int32, (nr, 128), 1)
    m0 = (lane & 1) == 0
    m4 = (lane & 16) == 0
    qscale = QSCALE if chain is None else jnp.concatenate(
        [chain.after(jnp.full((8, 128), QSCALE, f32))] * (nr // 8), axis=0)
    q = q_s[:, pl.ds(q0, nr), :] * qscale
    logits = []
    for w0 in range(0, W, wb):
        zs = [jnp.sum(q * k_s[:, pl.ds(q0 + (HALO - DIL * w), nr), :], axis=0)
              for w in range(w0, w0 + wb)]
        zs = [z + jnp.where(m0, pltpu.roll(z, 127, 1), pltpu.roll(z, 1, 1)) for z in zs]
        zs = [z + jnp.where(m4, pltpu.roll(z, 112, 1), pltpu.roll(z, 16, 1)) for z in zs]
        for w, z in zip(range(w0, w0 + wb), zs):
            if w > 0 and row0 is not None:
                row = jax.lax.broadcasted_iota(jnp.int32, (nr, 128), 0) + row0
                z = jnp.where(row >= DIL * w, z, NEG)
            logits.append(z)
    m = logits[0]
    for w in range(1, W):
        m = jnp.maximum(m, logits[w])
    e = [jnp.exp2(logits[w] - m) for w in range(W)]
    den = e[0]
    for w in range(1, W):
        den = den + e[w]
    inv = pl.reciprocal(den, approx=False)
    outs = []
    gs = NG // PVS
    for g0 in range(0, NG, gs):
        o = None
        for w in range(W):
            ew = e[w]
            if w == 0:
                ew = pv.after(ew)
            p = ew * v_s[g0:g0 + gs, pl.ds(q0 + (HALO - DIL * w), nr), :]
            o = p if o is None else o + p
        o = o * inv
        outs += [o[g] for g in range(gs)]
        pv.tok = outs[-1]
    if chain is not None:
        chain.tok = outs[-1][0:8]
    return jnp.concatenate(outs, axis=1)


def _store_attention(oa_s, m0, top, bot):
    ops = _lhs_operands(top[:, :DH2], top[:, DH2:], bot[:, :DH2], bot[:, DH2:])
    oa_s[:, pl.ds(m0, 8), :] = jnp.stack(ops).astype(bf16)


def _attention(q_s, k_s, v_s, oa_s, q0, o0, nrows, wb, pv):
    for r in range(0, nrows, 16):
        halves = []
        for t in (0, 8):
            pv.tok = None
            halves.append(_attention_rows(q_s, k_s, v_s, q0 + r + t, None, wb, pv))
        _store_attention(oa_s, (o0 + r) // 2, *halves)


def _mod_cols(wmod_v, st_v, col, n, chain=None):
    acc = None
    for r in range(0, D, MR):
        s = st_v[r:r + MR, :]
        if r == 0 and chain is not None:
            s = chain.after_rows(s)
        if n > 128:
            s = jnp.concatenate([s] * (n // 128), axis=1)
        p = wmod_v[r:r + MR, pl.ds(col, n)].astype(f32) * s
        for i in range(0, MR, 8):
            acc = p[i:i + 8] if acc is None else acc + p[i:i + 8]
    if chain is not None:
        chain.tok = acc[:, 0:128]
    return acc.sum(axis=0, keepdims=True)


def _lhs_operands(a11, a12, a21, a22):
    return [a11 + a22, a21 + a22, a11, a22, a11 + a12, a21 - a11, a12 - a22]


def _rhs_sums(b11, b12, b21, b22):
    return (b11 + b22, b12 - b22, b21 - b11, b11 + b12, b21 + b22)


def _rhs_operands(sums, b11, b22):
    return [sums(0), b11, sums(1), sums(2), b22, sums(3), sums(4)]


def _combine(m):
    return (m[0] + m[3] - m[4] + m[6], m[2] + m[4], m[1] + m[3], m[0] - m[1] + m[2] + m[5])


def _new_chain(flag_s):
    return _Chain(jax.lax.broadcasted_iota(jnp.int32, (8, 128), 1) < flag_s[0])


def _ln1_next(x_v, mod_v, h_s, r0, chains, extra=None):
    sa = mod_v[0:1, 0 * D:1 * D]
    ca1 = 1.0 + mod_v[0:1, 1 * D:2 * D]
    for i, r in enumerate(range(0, TM, LNR)):
        chain = chains[i % len(chains)]
        x = chain.after_rows(x_v[pl.ds(r0 + r, LNR), :].astype(f32))
        h = _modulated_ln(x, ca1, sa)
        chain.tok = h[0:8, 0:128]
        h_s[pl.ds(r, LNR), :] = h.astype(bf16)
        if extra is not None:
            extra(i)


def _phase1(step, x_v, wqkv_p, wo_raw, wo_p, so_v, w1_v, w3_v, w2_v, s1_v, s3_v, s2_v, wmod_v, mod_v, st_v,
            h_s, q0_s, k0_s, v0_s, q_s, k_s, v_s, o_s, flag_s):
    step = jnp.clip(step, 1, N1 - 1)
    part = jnp.maximum(step - 2, 0)
    base = pl.multiple_of((step + T0 - 2) * TM, TM)
    h = h_s[...]
    chain = _new_chain(flag_s)

    ln_r0 = pl.multiple_of(jnp.minimum(step + T0, NT - 1) * TM, TM)
    sa = mod_v[0:1, 0 * D:1 * D]
    ca1 = 1.0 + mod_v[0:1, 1 * D:2 * D]

    def ln_unit(i, nr=LNR):
        x = x_v[pl.ds(ln_r0 + i * nr, nr), :].astype(f32)
        x = jnp.concatenate([chain.after_rows(x[r:r + 8]) for r in range(0, nr, 8)], axis=0)
        hn = _modulated_ln(x, ca1, sa)
        chain.tok = hn[0:8, 0:128]
        h_s[pl.ds(i * nr, nr), :] = hn.astype(bf16)

    def wo_unit(mid):
        col = pl.multiple_of(part * 128, 128)
        lr = []
        for c0 in (col, DH2 + col):
            a = [_pack(wo_raw[pl.ds(c * 128 + mid * 16, 16), pl.ds(c0, 128)]) for c in range(8)]
            a[0] = chain.after(a[0])
            for k in range(3):
                a = _swap_stage(a, k, k, 0)
            chain.tok = a[7]
            lr.append(a)
        for s in range(4):
            q = [lr[0][s], lr[1][s], lr[0][s + 4], lr[1][s + 4]]
            wo_p[0, pl.ds(s * 64 + mid * 8, 8), pl.ds(col, 128)] = q[0]
            wo_p[1, pl.ds(s * 64 + mid * 8, 8), pl.ds(col, 128)] = q[3]
            q[0] = chain.after(q[0])
            sums = _rhs_sums(*[_unpack(v).astype(f32) for v in q])
            chain.tok = sums[0][0:8]
            so_v[:, pl.ds(s * 128 + mid * 16, 16), pl.ds(col, 128)] = jnp.stack(sums).astype(bf16)

    at_r0 = pl.multiple_of(part * 64, 64)
    pv1 = _new_chain(flag_s)

    def attn_unit(i):
        halves = [_attention_rows(q0_s, k0_s, v0_s, at_r0 + i * 16 + t,
                                  at_r0 + t if i == 0 else None, WB1, pv1) for t in (0, 8)]
        _store_attention(o_s, pl.multiple_of(part * 32 + i * 8, 8), *halves)

    mod_col = pl.multiple_of(step * D, D)

    def mod_unit(i):
        col = pl.multiple_of(mod_col + i * 256, 256)
        val = _mod_cols(wmod_v, st_v, col, 256, chain)
        mod_v[:, pl.ds(col, 256)] = jnp.broadcast_to(val, (8, 256))

    sum_units = []
    for w_v, s_v, half, ru, ch in ((w1_v, s1_v, DH2, RU1, FH), (w3_v, s3_v, DH2, RU1, FH),
                                   (w2_v, s2_v, FH, RU2, DH2)):
        r_lo = jnp.minimum((step - 1) * (ru // 16), (half - ru) // 16)
        srcs = [w_v.at[pl.ds(pl.multiple_of(i * half + r_lo * 16, 16), ru)] for i in range(2)]
        dst = s_v.at[:, pl.ds(pl.multiple_of(r_lo * (16 // PK), 16 // PK), ru // PK)]
        r_bk = jnp.clip(r_lo + flag_s[0] - 128, 0, (half - ru) // 16)
        back = s_v.at[:, pl.ds(pl.multiple_of(r_bk * (16 // PK), 16 // PK), ru // PK)]
        sum_units += [(srcs, dst, back, ch, r, c0)
                      for r in range(0, ru, UR) for c0 in range(0, ch, UC)]

    def sum_unit(u):
        srcs, dst, back, ch, r, c0 = sum_units[u]
        q = [srcs[i][r:r + UR, j * ch + c0:j * ch + c0 + UC].astype(f32)
             for i in range(2) for j in range(2)]
        q[0] = chain.after_rows(q[0])
        dst[:, r:r + UR, c0:c0 + UC] = jnp.stack(_rhs_sums(*q)).astype(bf16)
        chain.tok = back[0, 0:8, 0:128].astype(f32)

    def mm_unit(t, gated):
        sec, g = t // NG, t % NG
        dst, off = (q_s, k_s, v_s)[sec], (0 if sec == 0 else HALO)
        w = wqkv_p[:, t * 128:(t + 1) * 128]
        if gated:
            w = chain.after_rows(w)
        res = _dot(h, _unpack(w))
        dst[g, pl.ds(base + off, TM), :] = res
        return res[0:8]

    PLAN(chain, mm_unit, ln_unit, wo_unit, attn_unit, mod_unit, sum_unit, len(sum_units))


def PLAN(chain, mm_unit, ln_unit, wo_unit, attn_unit, mod_unit, sum_unit, nsum):
    ticks = [mm_unit(t, False) for t in range(3 * NG)]
    done = 0
    for t in range(3 * NG - 1):
        chain.tok = ticks[t]
        if t < 8:
            ln_unit(t, 32)
            wo_unit(t)
        if 15 <= t < 19:
            mod_unit(t - 15)
        n = 10 if (t < 8 or 15 <= t < 19) else -(-(nsum - 120) // 11)
        for u in range(done, min(done + n, nsum)):
            sum_unit(u)
        done = min(done + n, nsum)
    assert done == nsum
    for i in range(4):
        attn_unit(i)


def _phase2(step, x_v, wo_p, so_v, w1_v, w3_v, w2_v, s1_v, s3_v, s2_v, mod_v, q_s, k_s, v_s, o_s, note_s,
            flag_s, o_ref):
    j2 = jnp.clip(step - N1, 0, NT - 1)
    ga = mod_v[0:1, 2 * D:3 * D]
    sb = mod_v[0:1, 3 * D:4 * D]
    cb1 = 1.0 + mod_v[0:1, 4 * D:5 * D]
    gb = mod_v[0:1, 5 * D:6 * D]
    row0 = pl.multiple_of(j2 * TM, TM)
    nsub = TM // SUB
    hs = SUB // 2
    os_ = [[o_s[i, pl.ds(s * hs, hs), :] for i in range(7)] for s in range(nsub)]
    x1s, blocks = [], []
    for s in range(nsub):
        b = _rhs_operands(lambda i: so_v[i], _unpack(wo_p[0]), _unpack(wo_p[1]))
        c11, c12, c21, c22 = _combine([_dot(os_[s][i], b[i]) for i in range(7)])
        top = jnp.concatenate([c11, c12], axis=1)
        bot = jnp.concatenate([c21, c22], axis=1)
        att = jnp.concatenate([h[r:r + 8] for r in range(0, hs, 8) for h in (top, bot)], axis=0)
        note_s[...] = att[0:8, 0:128]
        x1 = x_v[pl.ds(row0 + s * SUB, SUB), :].astype(f32) + ga * att
        x1s.append(x1)
        chain = _new_chain(flag_s)
        for r in range(0, SUB, 32):
            xb = x1[r:r + 32]
            xb = jnp.concatenate([chain.after_rows(xb[0:16]), chain.after_rows(xb[16:32])], axis=0)
            rs, mr = _ln_stats(xb)
            chain.tok = None
            pieces = []
            cw = DH2 // LNS
            for c in range(0, DH2, cw):
                hl, hr = [(chain.after_rows(xb[:, c0:c0 + cw]) * rs - mr) * cb1[:, c0:c0 + cw]
                          + sb[:, c0:c0 + cw] for c0 in (c, DH2 + c)]
                pieces.append(_lhs_operands(hl[0:16], hr[0:16], hl[16:32], hr[16:32]))
                chain.tok = hr[24:32, cw - 128:cw]
            blocks.append([jnp.concatenate([pc[i] for pc in pieces], axis=1) for i in range(7)])

    nq = pl.multiple_of(jnp.minimum(j2, NT - 2) * TM, TM)

    def stack(per_group):
        return [jnp.concatenate([ops[i] for ops in per_group], axis=0) for i in range(7)]

    nb = len(blocks) // NGRP
    groups = [stack(blocks[g * nb:(g + 1) * nb]) for g in range(NGRP)]

    def up_proj(a, w_v, s_v, j):
        c0 = j * HN
        b = _rhs_operands(lambda i: _sunpack(s_v[i, :, c0:c0 + HN]),
                          w_v[0:DH2, c0:c0 + HN], w_v[DH2:, FH + c0:FH + c0 + HN])
        return _combine([_dot(a[i], b[i]) for i in range(7)])

    def to_mxu(ops):
        return [v.astype(bf16) for v in ops]

    def gate_up(a, j):
        act = []
        for g, u in zip(up_proj(a, w1_v, s1_v, j), up_proj(a, w3_v, s3_v, j)):
            hg = 0.5 * g
            act.append((hg + hg * jnp.tanh(hg)) * u)
        return _lhs_operands(*act)

    h_all = to_mxu(stack(groups))
    sep = []
    for g, ops in enumerate(groups):
        sep.append([gate_up(to_mxu(ops), j) for j in range(NSEP)])
        rows = TM // NGRP
        _attention(q_s, k_s, v_s, o_s, nq + g * rows, g * rows, rows, WB2, _new_chain(flag_s))
    acc = None
    for j in range(FH // HN):
        a = stack([sp[j] for sp in sep]) if j < NSEP else gate_up(h_all, j)
        a = to_mxu(a)
        r0 = j * HN
        b = _rhs_operands(lambda i: _sunpack(s2_v[i, r0 // PK:(r0 + HN) // PK, :]),
                          w2_v[r0:r0 + HN, 0:DH2], w2_v[FH + r0:FH + r0 + HN, DH2:])
        m = [_dot(a[i], b[i]) for i in range(7)]
        acc = m if acc is None else [p + q for p, q in zip(acc, m)]
    c11, c12, c21, c22 = _combine(acc)
    x1 = jnp.concatenate(x1s, axis=0)
    for blk in range(TM // 32):
        rows = slice(blk * 16, (blk + 1) * 16)
        for t, (left, right) in enumerate(((c11, c12), (c21, c22))):
            y = jnp.concatenate([left[rows], right[rows]], axis=1)
            r = blk * 32 + t * 16
            o_ref[r:r + 16, :] = (x1[r:r + 16] + gb * y).astype(o_ref.dtype)


def _kernel(x_hbm, c_hbm, wqkv_hbm, wo_hbm, w1_hbm, w3_hbm, w2_hbm, wmod_hbm, o_hbm,
            x_v, wqkv_raw, wqkv_p, wo_raw, wo_p, so_v, w1_v, w3_v, w2_v, s1_v, s3_v, s2_v,
            wmod_v, mod_v, st_v, xn_s, wcur_s, hl_s, h_s, q0_s, k0_s, v0_s, q_s, k_s, v_s,
            o_s, o_ref, c_v, note_s, flag_s, sems):
    step = pl.program_id(0)

    def new_chain():
        return _new_chain(flag_s)

    def cp_rows(src, dst, r0, n, sem):
        rows = pl.ds(r0, n)
        return pltpu.make_async_copy(src.at[rows], dst.at[rows], sems.at[sem])

    def cp_cols(src, dst, c0, n, sem):
        cols = pl.ds(c0, n)
        return pltpu.make_async_copy(src.at[:, cols], dst.at[:, cols], sems.at[sem])

    cp_c = lambda: [pltpu.make_async_copy(c_hbm, c_v, sems.at[SEM_C])]
    cp_x = lambda i: [cp_rows(x_hbm, x_v, i * TM, TM, SEM_X + i)]
    cp_wq0 = lambda: [cp_rows(wqkv_hbm, wqkv_raw, 0, KC, SEM_WQ0)]
    cp_wm = lambda p: [cp_cols(wmod_hbm, wmod_v, (2 + p) * D, D, SEM_WM + p)]

    def cp_chunk(k, with_wq=True):
        cps = [cp_rows(wqkv_hbm, wqkv_raw, k * KC, KC, SEM_CH + k)] if with_wq else []
        return cps + [cp_cols(wmod_hbm, wmod_v, k * KC, KC, SEM_CH + k),
                      cp_cols(wmod_hbm, wmod_v, D + k * KC, KC, SEM_CH + k)]

    def cp_wo(i):
        c0, n = (0, 128) if i == 0 else (128, DH2 - 128)
        return [cp_cols(wo_hbm, wo_raw, h + c0, n, SEM_WO + i) for h in (0, DH2)]

    def cp_ff(i):
        cps = []
        for src, dst, half, ru in ((w1_hbm, w1_v, DH2, RU1), (w3_hbm, w3_v, DH2, RU1),
                                   (w2_hbm, w2_v, FH, RU2)):
            n = min(ru, half - i * ru)
            cps += [cp_rows(src, dst, h * half + i * ru, n, SEM_FF + i) for h in range(2)]
        return cps

    def wait(*groups):
        for cps in groups:
            for cp in cps:
                cp.wait()

    def qkv_dst(t, sec):
        off = 0 if sec == 0 else HALO
        if t == 0:
            return (q0_s, k0_s, v0_s)[sec], off
        return (q_s, k_s, v_s)[sec], off + (t - 1) * TM

    @_when(step == 0, 'first')
    def _first():
        order = cp_c() + cp_x(0) + cp_wq0() + cp_chunk(0, False) + cp_x(1) + cp_x(2)
        for k in range(1, NKC):
            order += cp_chunk(k)
        order += cp_x(3) + cp_x(4) + cp_wo(0) + cp_ff(0)
        order += cp_x(5) + cp_wm(0) + cp_ff(1)
        order += cp_x(6) + cp_wo(1) + cp_wm(1) + cp_ff(2)
        order += cp_x(7) + cp_wm(2) + cp_ff(3)
        order += cp_wm(3) + cp_ff(4)
        for cp in order:
            cp.start()
        flag_s[0] = 128

        last = T0 - 1

        def zero_body(g, carry):
            for sec in range(3):
                dst, off = qkv_dst(last, sec)
                dst[g, pl.ds(off, TM), :] = jnp.zeros((TM, 128), f32)
            return carry
        jax.lax.fori_loop(0, NG, zero_body, 0)
        wait(cp_c())
        c = c_v[...].astype(f32)
        sc = c * jax.nn.sigmoid(c)
        st_v[...] = jnp.transpose(jnp.broadcast_to(sc, (128, D)))

        def normalize(row0, nrows, chains=None):
            for i in range(nrows // LNR):
                r0 = row0 + i * LNR
                x = x_v[pl.ds(r0, LNR), :].astype(f32)
                if chains is not None:
                    x = chains[i % len(chains)].after_rows(x)
                r, mr = _ln_stats(x)
                xn = x * r - mr
                if chains is not None:
                    chains[i % len(chains)].tok = xn[0:8, 0:128]
                for g in range(NG):
                    xn_s[g, pl.ds(r0, LNR), :] = xn[:, g * 128:(g + 1) * 128]

        def mod_chunk(k):
            col = k * KC if isinstance(k, int) else pl.multiple_of(k * KC, KC)
            sa = _mod_cols(wmod_v, st_v, col, KC)
            ca = _mod_cols(wmod_v, st_v, D + col, KC)
            mod_v[:, pl.ds(col, KC)] = jnp.broadcast_to(sa, (8, KC))
            mod_v[:, pl.ds(D + col, KC)] = jnp.broadcast_to(ca, (8, KC))
            return sa, 1.0 + ca

        def h_chunk(k, t, n, sa, ca1):
            return (xn_s[k, pl.ds(t * TM, n * TM), :] * ca1 + sa).astype(bf16)

        def mm(h, w, sec, tiles, first):
            res = _dot(h, _unpack(w))
            for i, t in enumerate(tiles):
                dst, off = qkv_dst(t, sec)
                for g in range(NG):
                    blk = res[i * TM:(i + 1) * TM, g * 128:(g + 1) * 128]
                    if first:
                        dst[g, pl.ds(off, TM), :] = blk
                    else:
                        dst[g, pl.ds(off, TM), :] += blk

        def wcur(sec):
            return wcur_s[:, sec * D:(sec + 1) * D]

        def keep(k, sec, wp):
            r0 = k * (KC // 2) if isinstance(k, int) else pl.multiple_of(k * (KC // 2), KC // 2)
            cols = pl.ds(sec * D if isinstance(sec, int) else pl.multiple_of(sec * D, D), D)
            wcur_s[:, cols] = wp
            wqkv_p[pl.ds(r0, KC // 2), cols] = wp

        scope = jax.named_scope
        mod0 = lambda: (mod_v[0:1, 0:KC], 1.0 + mod_v[0:1, D:D + KC])
        with scope('w_x0'):
            wait(cp_x(0))
        with scope('norm0'):
            def norm_body(i, carry):
                normalize(pl.multiple_of(i * 64, 64), 64)
                return carry
            jax.lax.fori_loop(0, TM // 64, norm_body, 0)
        with scope('w_wq0'):
            wait(cp_wq0())
        with scope('perm0'):
            def perm_body(sec, carry):
                keep(0, sec, _permute_qkv_section(wqkv_raw, 0, sec))
                return carry
            jax.lax.fori_loop(0, 3, perm_body, 0)
        with scope('w_m0'):
            wait(cp_chunk(0, False), cp_x(1))
        with scope('mm00'):
            sa, ca1 = mod_chunk(0)
            h0 = h_chunk(0, 0, 1, sa, ca1)
            for sec in range(3):
                mm(h0, wcur(sec), sec, [0], True)
            normalize(TM, TM, [new_chain() for _ in range(4)])
        with scope('w_x2'):
            wait(cp_x(2))
        with scope('mm01'):
            h1 = h_chunk(0, 1, 1, *mod0())
            for sec in range(3):
                mm(h1, wcur(sec), sec, [1], True)
            normalize(2 * TM, TM, [new_chain() for _ in range(4)])
            hl_s[...] = _pack(h_chunk(0, last, 1, *mod0()))

        def chunk_body(k0, carry):
            k = k0 + 1
            with scope('w_chunk'):
                wait(cp_chunk(k))
            with scope('chunk'):
                hl = _unpack(hl_s[...])
                for sec in range(3):
                    mm(hl, wcur(sec), sec, [last], False)
                sa, ca1 = mod_chunk(k)
                hf = h_chunk(k, 0, last, sa, ca1)
                hl_s[...] = _pack(h_chunk(k, last, 1, sa, ca1))
                for sec in range(3):
                    wp = _permute_qkv_section(wqkv_raw, pl.multiple_of(k * KC, KC), sec)
                    mm(hf, wp, sec, list(range(last)), False)
                    keep(k, sec, wp)
            return carry
        jax.lax.fori_loop(0, NKC - 1, chunk_body, 0)

        with scope('w_x3'):
            wait(cp_x(T0))
        hl = _unpack(hl_s[...])
        for sec in range(3):
            mm(hl, wcur(sec), sec, [last], False)
        _ln1_next(x_v, mod_v, h_s, T0 * TM, [new_chain() for _ in range(4)])
        k0_s[:, 0:HALO, :] = jnp.zeros((NG, HALO, 128), f32)
        v0_s[:, 0:HALO, :] = jnp.broadcast_to(v0_s[:, HALO:HALO + 1, :], (NG, HALO, 128))
        k_s[:, 0:HALO, :] = k0_s[:, TM:TM + HALO, :]
        v_s[:, 0:HALO, :] = v0_s[:, TM:TM + HALO, :]

    @_when(step == 1, 'wait1')
    def _():
        wait(cp_x(4), cp_wo(0), cp_ff(0))

    @_when(step == 2, 'wait2')
    def _():
        wait(cp_x(5), cp_wm(0), cp_ff(1))

    @_when(step == 3, 'wait3')
    def _():
        wait(cp_x(6), cp_wo(1), cp_wm(1), cp_ff(2))

    @_when(step == 4, 'wait4')
    def _():
        wait(cp_x(7), cp_wm(2), cp_ff(3))

    @_when(step == 5, 'wait5')
    def _():
        wait(cp_wm(3), cp_ff(4))

    @_when(jnp.logical_and(step >= 1, step < N1), 'phase1')
    def _():
        _phase1(step, x_v, wqkv_p, wo_raw, wo_p, so_v, w1_v, w3_v, w2_v, s1_v, s3_v, s2_v, wmod_v, mod_v, st_v,
                h_s, q0_s, k0_s, v0_s, q_s, k_s, v_s, o_s, flag_s)

    def cp_out(j):
        rows = pl.ds(pl.multiple_of(j * TM, TM), TM)
        return pltpu.make_async_copy(o_ref.at[j % 2], o_hbm.at[rows], sems.at[SEM_OUT + j % 2])

    @_when(step > N1 + 1, 'wait_out')
    def _():
        cp_out(step - N1 - 2).wait()

    @_when(step >= N1, 'phase2')
    def _():
        _phase2(step, x_v, wo_p, so_v, w1_v, w3_v, w2_v, s1_v, s3_v, s2_v, mod_v, q_s, k_s, v_s, o_s, note_s,
                flag_s, o_ref.at[(step - N1) % 2])
        cp_out(step - N1).start()

    @_when(step == N1 + NT - 1, 'wait_last')
    def _():
        cp_out(NT - 2).wait()
        cp_out(NT - 1).wait()


def _scratch_shapes():
    return [
        pltpu.VMEM((S, D), bf16),
        pltpu.VMEM((D, 3 * D), bf16),
        pltpu.VMEM((D // 2, 3 * D), u32),
        pltpu.VMEM((D, D), bf16),
        pltpu.VMEM((2, DH2 // 2, DH2), u32),
        pltpu.VMEM((5, DH2, DH2), bf16),
        pltpu.VMEM((D, F), bf16),
        pltpu.VMEM((D, F), bf16),
        pltpu.VMEM((F, D), bf16),
        pltpu.VMEM((5, DH2 // PK, FH), bf16 if PK == 1 else u32),
        pltpu.VMEM((5, DH2 // PK, FH), bf16 if PK == 1 else u32),
        pltpu.VMEM((5, FH // PK, DH2), bf16 if PK == 1 else u32),
        pltpu.VMEM((D, 6 * D), bf16),
        pltpu.VMEM((8, 6 * D), f32),
        pltpu.VMEM((D, 128), f32),
        pltpu.VMEM((NG, T0 * TM, 128), f32),
        pltpu.VMEM((KC // 2, 3 * D), u32),
        pltpu.VMEM((TM // 2, KC), u32),
        pltpu.VMEM((TM, D), bf16),
        pltpu.VMEM((NG, TM, 128), f32),
        pltpu.VMEM((NG, HALO + TM, 128), f32),
        pltpu.VMEM((NG, HALO + TM, 128), f32),
        pltpu.VMEM((NG, S - TM, 128), f32),
        pltpu.VMEM((NG, HALO + S - TM, 128), f32),
        pltpu.VMEM((NG, HALO + S - TM, 128), f32),
        pltpu.VMEM((7, TM // 2, DH2), bf16),
        pltpu.VMEM((2, TM, D), bf16),
        pltpu.VMEM((1, D), bf16),
        pltpu.VMEM((8, 128), f32),
        pltpu.SMEM((1,), jnp.int32),
        pltpu.SemaphoreType.DMA((NSEM,)),
    ]


@jax.jit
def pallas_adaLN_cond__sliding_local_dilated__glu_gated_swiglu__prompt_kernel(
    A_x: jax.Array,
    A_wqkv: jax.Array,
    A_wo: jax.Array,
    B_x: jax.Array,
    B_w1: jax.Array,
    B_w3: jax.Array,
    B_w2: jax.Array,
    c: jax.Array,
    w_mod: jax.Array,
):
    del B_x
    x = A_x.reshape(S, D)
    hbm = pl.BlockSpec(memory_space=pl.ANY)
    out = pl.pallas_call(
        _kernel,
        grid=(N1 + NT,),
        in_specs=[hbm] * 8,
        out_specs=hbm,
        out_shape=jax.ShapeDtypeStruct((S, D), A_x.dtype),
        scratch_shapes=_scratch_shapes(),
        compiler_params=pltpu.CompilerParams(
            dimension_semantics=("arbitrary",),
            vmem_limit_bytes=122 * 1024 * 1024,
        ),
        name="adaln_attn_ffn",
    )(x, c, A_wqkv, A_wo, B_w1, B_w3, B_w2, w_mod)
    return out.reshape(1, S, D)
```

```python
import jax
import jax.numpy as jnp
import jax.experimental.pallas as pl
import jax.experimental.pallas.tpu as pltpu

S, D, F = 2048, 1024, 3584
H, DH, W, DIL = 32, 32, 8, 2
NG = D // 128
TM = 256
NT = S // TM
T0 = 3
N1 = NT - T0 + 1
SUB = 128
HN = 256
FH = F // 2
DH2 = D // 2
KC = 128
NKC = D // KC
RU1 = 112
RU2 = 368
HALO = 16
PVS = 4
MR = 64
LNS = 2
NGRP = 2
UR, UC = 8, 256
WB1 = 1
WB2 = 1
LNR = 16
EPS = 1e-5
SCALE = DH ** -0.5
LOG2E = 1.4426950408889634
QSCALE = SCALE * LOG2E
NEG = -1000000000.0 * LOG2E

f32 = jnp.float32
bf16 = jnp.bfloat16
u32 = jnp.uint32

SEM_C = 0
SEM_X = 1
SEM_WQ0 = SEM_X + NT
SEM_CH = SEM_WQ0 + 1
SEM_WM = SEM_CH + NKC
SEM_WO = SEM_WM + 4
SEM_FF = SEM_WO + 2
SEM_OUT = SEM_FF + (N1 - 1)
NSEM = SEM_OUT + 2


def _when(cond, name):
    def deco(body):
        def scoped():
            with jax.named_scope(name):
                body()
        return pl.when(cond)(scoped)
    return deco


def _pack(x):
    return pltpu.bitcast(x, u32)


def _unpack(x):
    return pltpu.bitcast(x, bf16)


def _dot(a, b):
    return jnp.dot(a, b, preferred_element_type=f32)


class _Chain:
    def __init__(self, always):
        self.always = always
        self.tok = None

    def after(self, x):
        if self.tok is None:
            return x
        t = self.tok if self.tok.dtype == x.dtype else pltpu.bitcast(self.tok, x.dtype)
        return jnp.where(self.always, x, t)

    def after_rows(self, x):
        x00 = self.after(x[0:8, 0:128])
        top = x00 if x.shape[1] == 128 else jnp.concatenate([x00, x[0:8, 128:]], axis=1)
        return top if x.shape[0] == 8 else jnp.concatenate([top, x[8:]], axis=0)


def _swap_stage(a, k, b, axis):
    n = 128 if axis == 1 else 8
    idx = jax.lax.broadcasted_iota(jnp.int32, a[0].shape, axis)
    m0 = (idx & (1 << b)) == 0
    out = list(a)
    for c in range(8):
        if c & (1 << k):
            continue
        lo, hi = a[c], a[c | (1 << k)]
        out[c] = jnp.where(m0, lo, pltpu.roll(hi, 1 << b, axis))
        out[c | (1 << k)] = jnp.where(m0, pltpu.roll(lo, n - (1 << b), axis), hi)
    return out


def _permute_qkv_section(w_ref, r0, sec):
    c0 = sec * D if isinstance(sec, int) else pl.multiple_of(sec * D, D)
    a = [_pack(w_ref[pl.ds(r0, KC), pl.ds(c0 + c * 128, 128)]) for c in range(8)]
    for k in range(3):
        a = _swap_stage(a, k, k + 1, 1)
    return jnp.concatenate(a, axis=1)


def _ln_stats(x):
    m = jnp.mean(x, axis=-1, keepdims=True)
    xc = x - m
    v = jnp.mean(xc * xc, axis=-1, keepdims=True)
    r = jax.lax.rsqrt(v + EPS)
    return r, m * r


def _modulated_ln(x, scale1, shift):
    r, mr = _ln_stats(x)
    return (x * r - mr) * scale1 + shift


def _attention_rows(q_s, k_s, v_s, q0, row0, wb, pv):
    lane = jax.lax.broadcasted_iota(jnp.int32, (8, 128), 1)
    m0 = (lane & 1) == 0
    m4 = (lane & 16) == 0
    q = q_s[:, pl.ds(q0, 8), :] * QSCALE
    logits = []
    for w0 in range(0, W, wb):
        zs = [jnp.sum(q * k_s[:, pl.ds(q0 + (HALO - DIL * w), 8), :], axis=0)
              for w in range(w0, w0 + wb)]
        zs = [z + jnp.where(m0, pltpu.roll(z, 127, 1), pltpu.roll(z, 1, 1)) for z in zs]
        zs = [z + jnp.where(m4, pltpu.roll(z, 112, 1), pltpu.roll(z, 16, 1)) for z in zs]
        for w, z in zip(range(w0, w0 + wb), zs):
            if w > 0 and row0 is not None:
                row = jax.lax.broadcasted_iota(jnp.int32, (8, 128), 0) + row0
                z = jnp.where(row >= DIL * w, z, NEG)
            logits.append(z)
    m = logits[0]
    for w in range(1, W):
        m = jnp.maximum(m, logits[w])
    e = [jnp.exp2(logits[w] - m) for w in range(W)]
    den = e[0]
    for w in range(1, W):
        den = den + e[w]
    inv = pl.reciprocal(den, approx=False)
    outs = []
    gs = NG // PVS
    for g0 in range(0, NG, gs):
        o = None
        for w in range(W):
            ew = e[w]
            if w == 0:
                ew = pv.after(ew)
            p = ew * v_s[g0:g0 + gs, pl.ds(q0 + (HALO - DIL * w), 8), :]
            o = p if o is None else o + p
        o = o * inv
        outs += [o[g] for g in range(gs)]
        pv.tok = outs[-1]
    return jnp.concatenate(outs, axis=1)


def _store_attention(oa_s, m0, top, bot):
    ops = _lhs_operands(top[:, :DH2], top[:, DH2:], bot[:, :DH2], bot[:, DH2:])
    oa_s[:, pl.ds(m0, 8), :] = jnp.stack(ops).astype(bf16)


def _attention(q_s, k_s, v_s, oa_s, q0, o0, nrows, wb, pv):
    for r in range(0, nrows, 16):
        halves = []
        for t in (0, 8):
            pv.tok = None
            halves.append(_attention_rows(q_s, k_s, v_s, q0 + r + t, None, wb, pv))
        _store_attention(oa_s, (o0 + r) // 2, *halves)


def _mod_cols(wmod_v, st_v, col, n, chain=None):
    acc = None
    for r in range(0, D, MR):
        s = st_v[r:r + MR, :]
        if r == 0 and chain is not None:
            s = chain.after_rows(s)
        if n > 128:
            s = jnp.concatenate([s] * (n // 128), axis=1)
        p = wmod_v[r:r + MR, pl.ds(col, n)].astype(f32) * s
        for i in range(0, MR, 8):
            acc = p[i:i + 8] if acc is None else acc + p[i:i + 8]
    if chain is not None:
        chain.tok = acc[:, 0:128]
    return acc.sum(axis=0, keepdims=True)


ORD_O = ORD_D = (0, 5, 6, 4, 2, 3, 1)
ORD_U = (0, 1, 2, 3, 4, 5, 6)
NS = 4


def _lhs_operands(a11, a12, a21, a22):
    s1 = a21 + a22
    s2 = s1 - a11
    return [a11, a12, a12 - s2, a22, s1, s2, a11 - a21]


def _rhs_sums(b11, b12, b21, b22):
    t1 = b12 - b11
    t2 = b22 - t1
    return (t2 - b21, t1, t2, b22 - b12)


def _rhs_operands(sums, b11, b21, b22):
    return [b11, b21, b22, sums(0), sums(1), sums(2), sums(3)]


def _products(a, b, order):
    m = {i: _dot(a[i], b[i]) for i in order}
    return [m[i] for i in range(7)]


def _combine(p):
    u2 = p[0] + p[5]
    u3 = u2 + p[6]
    return (p[0] + p[1], u2 + p[4] + p[2], u3 - p[3], u3 + p[4])


def _new_chain(flag_s):
    return _Chain(jax.lax.broadcasted_iota(jnp.int32, (8, 128), 1) < flag_s[0])


def _ln1_next(x_v, mod_v, h_s, r0, chains):
    sa = mod_v[0:1, 0 * D:1 * D]
    ca1 = 1.0 + mod_v[0:1, 1 * D:2 * D]
    for i, r in enumerate(range(0, TM, LNR)):
        chain = chains[i % len(chains)]
        x = chain.after_rows(x_v[pl.ds(r0 + r, LNR), :].astype(f32))
        h = _modulated_ln(x, ca1, sa)
        chain.tok = h[0:8, 0:128]
        h_s[pl.ds(r, LNR), :] = h.astype(bf16)


def _phase1(step, x_v, wqkv_p, wo_raw, wo_p, so_v, w1_v, w3_v, w2_v, s1_v, s3_v, s2_v, wmod_v, mod_v, st_v,
            h_s, q0_s, k0_s, v0_s, q_s, k_s, v_s, o_s, flag_s):
    step = jnp.clip(step, 1, N1 - 1)
    part = jnp.maximum(step - 2, 0)
    base = pl.multiple_of((step + T0 - 2) * TM, TM)
    h = h_s[...]
    chain = _new_chain(flag_s)

    ln_r0 = pl.multiple_of(jnp.minimum(step + T0, NT - 1) * TM, TM)
    sa = mod_v[0:1, 0 * D:1 * D]
    ca1 = 1.0 + mod_v[0:1, 1 * D:2 * D]

    def ln_unit(i):
        x = x_v[pl.ds(ln_r0 + i * 32, 32), :].astype(f32)
        x = jnp.concatenate([chain.after_rows(x[r:r + 8]) for r in range(0, 32, 8)], axis=0)
        hn = _modulated_ln(x, ca1, sa)
        chain.tok = hn[0:8, 0:128]
        h_s[pl.ds(i * 32, 32), :] = hn.astype(bf16)

    def wo_unit(mid):
        col = pl.multiple_of(part * 128, 128)
        lr = []
        for c0 in (col, DH2 + col):
            a = [_pack(wo_raw[pl.ds(c * 128 + mid * 16, 16), pl.ds(c0, 128)]) for c in range(8)]
            a[0] = chain.after(a[0])
            for k in range(3):
                a = _swap_stage(a, k, k, 0)
            chain.tok = a[7]
            lr.append(a)
        for s in range(4):
            q = [lr[0][s], lr[1][s], lr[0][s + 4], lr[1][s + 4]]
            wo_p[0, pl.ds(s * 64 + mid * 8, 8), pl.ds(col, 128)] = q[0]
            wo_p[1, pl.ds(s * 64 + mid * 8, 8), pl.ds(col, 128)] = q[2]
            wo_p[2, pl.ds(s * 64 + mid * 8, 8), pl.ds(col, 128)] = q[3]
            q[0] = chain.after(q[0])
            sums = _rhs_sums(*[_unpack(v).astype(f32) for v in q])
            chain.tok = sums[0][0:8]
            so_v[:, pl.ds(s * 128 + mid * 16, 16), pl.ds(col, 128)] = jnp.stack(sums).astype(bf16)

    at_r0 = pl.multiple_of(part * 64, 64)
    pv1 = _new_chain(flag_s)

    def attn_unit(i):
        halves = [_attention_rows(q0_s, k0_s, v0_s, at_r0 + i * 16 + t,
                                  at_r0 + t if i == 0 else None, WB1, pv1) for t in (0, 8)]
        _store_attention(o_s, pl.multiple_of(part * 32 + i * 8, 8), *halves)

    mod_col = pl.multiple_of(step * D, D)

    def mod_unit(i):
        col = pl.multiple_of(mod_col + i * 256, 256)
        val = _mod_cols(wmod_v, st_v, col, 256, chain)
        mod_v[:, pl.ds(col, 256)] = jnp.broadcast_to(val, (8, 256))

    sum_units = []
    for w_v, s_v, half, ru, ch in ((w1_v, s1_v, DH2, RU1, FH), (w3_v, s3_v, DH2, RU1, FH),
                                   (w2_v, s2_v, FH, RU2, DH2)):
        r_lo = jnp.minimum((step - 1) * (ru // 16), (half - ru) // 16)
        srcs = [w_v.at[pl.ds(pl.multiple_of(i * half + r_lo * 16, 16), ru)] for i in range(2)]
        dst = s_v.at[:, pl.ds(pl.multiple_of(r_lo * 16, 16), ru)]
        r_bk = jnp.clip(r_lo + flag_s[0] - 128, 0, (half - ru) // 16)
        back = s_v.at[:, pl.ds(pl.multiple_of(r_bk * 16, 16), ru)]
        sum_units += [(srcs, dst, back, ch, r, c0)
                      for r in range(0, ru, UR) for c0 in range(0, ch, UC)]

    def sum_unit(u):
        srcs, dst, back, ch, r, c0 = sum_units[u]
        q = [srcs[i][r:r + UR, j * ch + c0:j * ch + c0 + UC].astype(f32)
             for i in range(2) for j in range(2)]
        q[0] = chain.after_rows(q[0])
        dst[:, r:r + UR, c0:c0 + UC] = jnp.stack(_rhs_sums(*q)).astype(bf16)
        chain.tok = back[0, 0:8, 0:128].astype(f32)

    def mm_unit(t):
        sec, g = t // NG, t % NG
        dst, off = (q_s, k_s, v_s)[sec], (0 if sec == 0 else HALO)
        res = _dot(h, _unpack(wqkv_p[:, t * 128:(t + 1) * 128]))
        dst[g, pl.ds(base + off, TM), :] = res
        return res[0:8]

    _plan(chain, mm_unit, ln_unit, wo_unit, attn_unit, mod_unit, sum_unit, len(sum_units))


def _plan(chain, mm_unit, ln_unit, wo_unit, attn_unit, mod_unit, sum_unit, nsum):
    ticks = [mm_unit(t) for t in range(3 * NG)]
    done = 0
    for t in range(3 * NG - 1):
        chain.tok = ticks[t]
        if t < 8:
            ln_unit(t)
            wo_unit(t)
        if 15 <= t < 19:
            mod_unit(t - 15)
        n = 8 if t < 8 else 12 if 15 <= t < 19 else -(-(nsum - 112) // 11)
        for u in range(done, min(done + n, nsum)):
            sum_unit(u)
        done = min(done + n, nsum)
    assert done == nsum
    for i in range(4):
        attn_unit(i)


def _phase2(step, x_v, wo_p, so_v, w1_v, w3_v, w2_v, s1_v, s3_v, s2_v, mod_v, q_s, k_s, v_s, o_s, note_s,
            flag_s, o_ref):
    j2 = jnp.clip(step - N1, 0, NT - 1)
    ga = mod_v[0:1, 2 * D:3 * D]
    sb = mod_v[0:1, 3 * D:4 * D]
    cb1 = 1.0 + mod_v[0:1, 4 * D:5 * D]
    gb = mod_v[0:1, 5 * D:6 * D]
    row0 = pl.multiple_of(j2 * TM, TM)
    nsub = TM // SUB
    hs = SUB // 2
    os_ = [[o_s[i, pl.ds(s * hs, hs), :] for i in range(7)] for s in range(nsub)]
    x1s, blocks = [], []
    for s in range(nsub):
        b = _rhs_operands(lambda i: so_v[i], *[_unpack(wo_p[i]) for i in range(3)])
        c11, c12, c21, c22 = _combine(_products(os_[s], b, ORD_O))
        top = jnp.concatenate([c11, c12], axis=1)
        bot = jnp.concatenate([c21, c22], axis=1)
        att = jnp.concatenate([h[r:r + 8] for r in range(0, hs, 8) for h in (top, bot)], axis=0)
        note_s[...] = att[0:8, 0:128]
        x1 = x_v[pl.ds(row0 + s * SUB, SUB), :].astype(f32) + ga * att
        x1s.append(x1)
        chain = _new_chain(flag_s)
        for r in range(0, SUB, 32):
            xb = x1[r:r + 32]
            xb = jnp.concatenate([chain.after_rows(xb[0:16]), chain.after_rows(xb[16:32])], axis=0)
            rs, mr = _ln_stats(xb)
            chain.tok = None
            pieces = []
            cw = DH2 // LNS
            for c in range(0, DH2, cw):
                hl, hr = [(chain.after_rows(xb[:, c0:c0 + cw]) * rs - mr) * cb1[:, c0:c0 + cw]
                          + sb[:, c0:c0 + cw] for c0 in (c, DH2 + c)]
                pieces.append(_lhs_operands(hl[0:16], hr[0:16], hl[16:32], hr[16:32]))
                chain.tok = hr[24:32, cw - 128:cw]
            blocks.append([jnp.concatenate([pc[i] for pc in pieces], axis=1) for i in range(7)])

    nq = pl.multiple_of(jnp.minimum(j2, NT - 2) * TM, TM)

    def stack(per_group):
        return [jnp.concatenate([ops[i] for ops in per_group], axis=0) for i in range(7)]

    nb = len(blocks) // NGRP
    groups = [stack(blocks[g * nb:(g + 1) * nb]) for g in range(NGRP)]

    def up_proj(a, w_v, s_v, j):
        c0 = j * HN
        b = _rhs_operands(lambda i: s_v[i, :, c0:c0 + HN],
                          w_v[0:DH2, c0:c0 + HN],
                          w_v[DH2:, c0:c0 + HN], w_v[DH2:, FH + c0:FH + c0 + HN])
        return _combine(_products(a, b, ORD_U))

    def to_mxu(ops):
        return [v.astype(bf16) for v in ops]

    def gate_up(a, j):
        act = []
        for g, u in zip(up_proj(a, w1_v, s1_v, j), up_proj(a, w3_v, s3_v, j)):
            hg = 0.5 * g
            act.append((hg + hg * jnp.tanh(hg)) * u)
        return _lhs_operands(*act)

    h_all = to_mxu(stack(groups))
    first = []
    for g, ops in enumerate(groups):
        first.append(gate_up(to_mxu(ops), 0))
        rows = TM // NGRP
        _attention(q_s, k_s, v_s, o_s, nq + g * rows, g * rows, rows, WB2, _new_chain(flag_s))
    acc = None
    for j in range(FH // HN):
        a = to_mxu(stack(first) if j == 0 else gate_up(h_all, j))
        r0 = j * HN
        b = _rhs_operands(lambda i: s2_v[i, r0:r0 + HN, :],
                          w2_v[r0:r0 + HN, 0:DH2], w2_v[FH + r0:FH + r0 + HN, 0:DH2],
                          w2_v[FH + r0:FH + r0 + HN, DH2:])
        m = _products(a, b, ORD_D)
        acc = m if acc is None else [p + q for p, q in zip(acc, m)]
    c11, c12, c21, c22 = _combine(acc)
    x1 = jnp.concatenate(x1s, axis=0)
    for blk in range(TM // 32):
        rows = slice(blk * 16, (blk + 1) * 16)
        for t, (left, right) in enumerate(((c11, c12), (c21, c22))):
            y = jnp.concatenate([left[rows], right[rows]], axis=1)
            r = blk * 32 + t * 16
            o_ref[r:r + 16, :] = (x1[r:r + 16] + gb * y).astype(o_ref.dtype)


def _kernel(x_hbm, c_hbm, wqkv_hbm, wo_hbm, w1_hbm, w3_hbm, w2_hbm, wmod_hbm, o_hbm,
            x_v, wqkv_raw, wqkv_p, wo_raw, wo_p, so_v, w1_v, w3_v, w2_v, s1_v, s3_v, s2_v,
            wmod_v, mod_v, st_v, xn_s, wcur_s, hl_s, h_s, q0_s, k0_s, v0_s, q_s, k_s, v_s,
            o_s, o_ref, c_v, note_s, flag_s, sems):
    step = pl.program_id(0)

    def new_chain():
        return _new_chain(flag_s)

    def cp_rows(src, dst, r0, n, sem):
        rows = pl.ds(r0, n)
        return pltpu.make_async_copy(src.at[rows], dst.at[rows], sems.at[sem])

    def cp_cols(src, dst, c0, n, sem):
        cols = pl.ds(c0, n)
        return pltpu.make_async_copy(src.at[:, cols], dst.at[:, cols], sems.at[sem])

    cp_c = lambda: [pltpu.make_async_copy(c_hbm, c_v, sems.at[SEM_C])]
    cp_x = lambda i: [cp_rows(x_hbm, x_v, i * TM, TM, SEM_X + i)]
    cp_wq0 = lambda: [cp_rows(wqkv_hbm, wqkv_raw, 0, KC, SEM_WQ0)]
    cp_wm = lambda p: [cp_cols(wmod_hbm, wmod_v, (2 + p) * D, D, SEM_WM + p)]

    def cp_chunk(k, with_wq=True):
        cps = [cp_rows(wqkv_hbm, wqkv_raw, k * KC, KC, SEM_CH + k)] if with_wq else []
        return cps + [cp_cols(wmod_hbm, wmod_v, k * KC, KC, SEM_CH + k),
                      cp_cols(wmod_hbm, wmod_v, D + k * KC, KC, SEM_CH + k)]

    def cp_wo(i):
        c0, n = (0, 128) if i == 0 else (128, DH2 - 128)
        return [cp_cols(wo_hbm, wo_raw, h + c0, n, SEM_WO + i) for h in (0, DH2)]

    def cp_ff(i):
        cps = []
        for src, dst, half, ru in ((w1_hbm, w1_v, DH2, RU1), (w3_hbm, w3_v, DH2, RU1),
                                   (w2_hbm, w2_v, FH, RU2)):
            n = min(ru, half - i * ru)
            cps += [cp_rows(src, dst, h * half + i * ru, n, SEM_FF + i) for h in range(2)]
        return cps

    def wait(*groups):
        for cps in groups:
            for cp in cps:
                cp.wait()

    def qkv_dst(t, sec):
        off = 0 if sec == 0 else HALO
        if t == 0:
            return (q0_s, k0_s, v0_s)[sec], off
        return (q_s, k_s, v_s)[sec], off + (t - 1) * TM

    @_when(step == 0, 'first')
    def _first():
        order = cp_c() + cp_x(0) + cp_wq0() + cp_chunk(0, False) + cp_x(1) + cp_x(2)
        for k in range(1, NKC):
            order += cp_chunk(k)
        order += cp_x(3) + cp_x(4) + cp_wo(0) + cp_ff(0)
        order += cp_x(5) + cp_wm(0) + cp_ff(1)
        order += cp_x(6) + cp_wo(1) + cp_wm(1) + cp_ff(2)
        order += cp_x(7) + cp_wm(2) + cp_ff(3)
        order += cp_wm(3) + cp_ff(4)
        for cp in order:
            cp.start()
        flag_s[0] = 128

        last = T0 - 1

        def zero_body(g, carry):
            for sec in range(3):
                dst, off = qkv_dst(last, sec)
                dst[g, pl.ds(off, TM), :] = jnp.zeros((TM, 128), f32)
            return carry
        jax.lax.fori_loop(0, NG, zero_body, 0)
        wait(cp_c())
        c = c_v[...].astype(f32)
        sc = c * jax.nn.sigmoid(c)
        st_v[...] = jnp.transpose(jnp.broadcast_to(sc, (128, D)))

        def normalize(row0, nrows, chains=None):
            for i in range(nrows // LNR):
                r0 = row0 + i * LNR
                x = x_v[pl.ds(r0, LNR), :].astype(f32)
                if chains is not None:
                    x = chains[i % len(chains)].after_rows(x)
                r, mr = _ln_stats(x)
                xn = x * r - mr
                if chains is not None:
                    chains[i % len(chains)].tok = xn[0:8, 0:128]
                for g in range(NG):
                    xn_s[g, pl.ds(r0, LNR), :] = xn[:, g * 128:(g + 1) * 128]

        def mod_chunk(k):
            col = k * KC if isinstance(k, int) else pl.multiple_of(k * KC, KC)
            sa = _mod_cols(wmod_v, st_v, col, KC)
            ca = _mod_cols(wmod_v, st_v, D + col, KC)
            mod_v[:, pl.ds(col, KC)] = jnp.broadcast_to(sa, (8, KC))
            mod_v[:, pl.ds(D + col, KC)] = jnp.broadcast_to(ca, (8, KC))
            return sa, 1.0 + ca

        def h_chunk(k, t, n, sa, ca1):
            return (xn_s[k, pl.ds(t * TM, n * TM), :] * ca1 + sa).astype(bf16)

        def mm(h, w, sec, tiles, first):
            res = _dot(h, _unpack(w))
            for i, t in enumerate(tiles):
                dst, off = qkv_dst(t, sec)
                for g in range(NG):
                    blk = res[i * TM:(i + 1) * TM, g * 128:(g + 1) * 128]
                    if first:
                        dst[g, pl.ds(off, TM), :] = blk
                    else:
                        dst[g, pl.ds(off, TM), :] += blk

        def wcur(sec):
            return wcur_s[:, sec * D:(sec + 1) * D]

        def keep(k, sec, wp):
            r0 = k * (KC // 2) if isinstance(k, int) else pl.multiple_of(k * (KC // 2), KC // 2)
            cols = pl.ds(sec * D if isinstance(sec, int) else pl.multiple_of(sec * D, D), D)
            wcur_s[:, cols] = wp
            wqkv_p[pl.ds(r0, KC // 2), cols] = wp

        scope = jax.named_scope
        mod0 = lambda: (mod_v[0:1, 0:KC], 1.0 + mod_v[0:1, D:D + KC])
        with scope('w_x0'):
            wait(cp_x(0))
        with scope('norm0'):
            def norm_body(i, carry):
                normalize(pl.multiple_of(i * 64, 64), 64)
                return carry
            jax.lax.fori_loop(0, TM // 64, norm_body, 0)
        with scope('w_wq0'):
            wait(cp_wq0())
        with scope('perm0'):
            def perm_body(sec, carry):
                keep(0, sec, _permute_qkv_section(wqkv_raw, 0, sec))
                return carry
            jax.lax.fori_loop(0, 2, perm_body, 0)
        with scope('w_m0'):
            wait(cp_chunk(0, False))
        with scope('mm00'):
            wp = _permute_qkv_section(wqkv_raw, 0, 2)
            sa, ca1 = mod_chunk(0)
            h0 = h_chunk(0, 0, 1, sa, ca1)
            for sec in range(3):
                mm(h0, wcur(sec) if sec < 2 else wp, sec, [0], True)
            keep(0, 2, wp)
        with scope('w_x12'):
            wait(cp_x(1), cp_x(2))
        with scope('mm01'):
            normalize(TM, TM)
            h1 = h_chunk(0, 1, 1, *mod0())
            for sec in range(3):
                mm(h1, wcur(sec), sec, [1], True)
            normalize(2 * TM, TM, [new_chain() for _ in range(4)])
            hl_s[...] = _pack(h_chunk(0, last, 1, *mod0()))

        def chunk_body(k0, carry):
            k = k0 + 1
            with scope('w_chunk'):
                wait(cp_chunk(k))
            with scope('chunk'):
                hl = _unpack(hl_s[...])
                for sec in range(3):
                    mm(hl, wcur(sec), sec, [last], False)
                sa, ca1 = mod_chunk(k)
                hf = h_chunk(k, 0, last, sa, ca1)
                hl_s[...] = _pack(h_chunk(k, last, 1, sa, ca1))
                for sec in range(3):
                    wp = _permute_qkv_section(wqkv_raw, pl.multiple_of(k * KC, KC), sec)
                    mm(hf, wp, sec, list(range(last)), False)
                    keep(k, sec, wp)
            return carry
        jax.lax.fori_loop(0, NKC - 1, chunk_body, 0)

        with scope('w_x3'):
            wait(cp_x(T0))
        hl = _unpack(hl_s[...])
        for sec in range(3):
            mm(hl, wcur(sec), sec, [last], False)
        _ln1_next(x_v, mod_v, h_s, T0 * TM, [new_chain() for _ in range(4)])
        k0_s[:, 0:HALO, :] = jnp.zeros((NG, HALO, 128), f32)
        v0_s[:, 0:HALO, :] = jnp.broadcast_to(v0_s[:, HALO:HALO + 1, :], (NG, HALO, 128))
        k_s[:, 0:HALO, :] = k0_s[:, TM:TM + HALO, :]
        v_s[:, 0:HALO, :] = v0_s[:, TM:TM + HALO, :]

    @_when(step == 1, 'wait1')
    def _():
        wait(cp_x(4), cp_wo(0), cp_ff(0))

    @_when(step == 2, 'wait2')
    def _():
        wait(cp_x(5), cp_wm(0), cp_ff(1))

    @_when(step == 3, 'wait3')
    def _():
        wait(cp_x(6), cp_wo(1), cp_wm(1), cp_ff(2))

    @_when(step == 4, 'wait4')
    def _():
        wait(cp_x(7), cp_wm(2), cp_ff(3))

    @_when(step == 5, 'wait5')
    def _():
        wait(cp_wm(3), cp_ff(4))

    @_when(jnp.logical_and(step >= 1, step < N1), 'phase1')
    def _():
        _phase1(step, x_v, wqkv_p, wo_raw, wo_p, so_v, w1_v, w3_v, w2_v, s1_v, s3_v, s2_v, wmod_v, mod_v, st_v,
                h_s, q0_s, k0_s, v0_s, q_s, k_s, v_s, o_s, flag_s)

    def cp_out(j):
        rows = pl.ds(pl.multiple_of(j * TM, TM), TM)
        return pltpu.make_async_copy(o_ref.at[j % 2], o_hbm.at[rows], sems.at[SEM_OUT + j % 2])

    @_when(step > N1 + 1, 'wait_out')
    def _():
        cp_out(step - N1 - 2).wait()

    @_when(step >= N1, 'phase2')
    def _():
        _phase2(step, x_v, wo_p, so_v, w1_v, w3_v, w2_v, s1_v, s3_v, s2_v, mod_v, q_s, k_s, v_s, o_s, note_s,
                flag_s, o_ref.at[(step - N1) % 2])
        cp_out(step - N1).start()

    @_when(step == N1 + NT - 1, 'wait_last')
    def _():
        cp_out(NT - 2).wait()
        cp_out(NT - 1).wait()


def _scratch_shapes():
    return [
        pltpu.VMEM((S, D), bf16),
        pltpu.VMEM((D, 3 * D), bf16),
        pltpu.VMEM((D // 2, 3 * D), u32),
        pltpu.VMEM((D, D), bf16),
        pltpu.VMEM((3, DH2 // 2, DH2), u32),
        pltpu.VMEM((NS, DH2, DH2), bf16),
        pltpu.VMEM((D, F), bf16),
        pltpu.VMEM((D, F), bf16),
        pltpu.VMEM((F, D), bf16),
        pltpu.VMEM((NS, DH2, FH), bf16),
        pltpu.VMEM((NS, DH2, FH), bf16),
        pltpu.VMEM((NS, FH, DH2), bf16),
        pltpu.VMEM((D, 6 * D), bf16),
        pltpu.VMEM((8, 6 * D), f32),
        pltpu.VMEM((D, 128), f32),
        pltpu.VMEM((NG, T0 * TM, 128), f32),
        pltpu.VMEM((KC // 2, 3 * D), u32),
        pltpu.VMEM((TM // 2, KC), u32),
        pltpu.VMEM((TM, D), bf16),
        pltpu.VMEM((NG, TM, 128), f32),
        pltpu.VMEM((NG, HALO + TM, 128), f32),
        pltpu.VMEM((NG, HALO + TM, 128), f32),
        pltpu.VMEM((NG, S - TM, 128), f32),
        pltpu.VMEM((NG, HALO + S - TM, 128), f32),
        pltpu.VMEM((NG, HALO + S - TM, 128), f32),
        pltpu.VMEM((7, TM // 2, DH2), bf16),
        pltpu.VMEM((2, TM, D), bf16),
        pltpu.VMEM((1, D), bf16),
        pltpu.VMEM((8, 128), f32),
        pltpu.SMEM((1,), jnp.int32),
        pltpu.SemaphoreType.DMA((NSEM,)),
    ]


@jax.jit
def pallas_adaLN_cond__sliding_local_dilated__glu_gated_swiglu__prompt_kernel(
    A_x: jax.Array,
    A_wqkv: jax.Array,
    A_wo: jax.Array,
    B_x: jax.Array,
    B_w1: jax.Array,
    B_w3: jax.Array,
    B_w2: jax.Array,
    c: jax.Array,
    w_mod: jax.Array,
):
    del B_x
    x = A_x.reshape(S, D)
    hbm = pl.BlockSpec(memory_space=pl.ANY)
    out = pl.pallas_call(
        _kernel,
        grid=(N1 + NT,),
        in_specs=[hbm] * 8,
        out_specs=hbm,
        out_shape=jax.ShapeDtypeStruct((S, D), A_x.dtype),
        scratch_shapes=_scratch_shapes(),
        compiler_params=pltpu.CompilerParams(
            dimension_semantics=("arbitrary",),
            vmem_limit_bytes=122 * 1024 * 1024,
        ),
        name="adaln_attn_ffn",
    )(x, c, A_wqkv, A_wo, B_w1, B_w3, B_w2, w_mod)
    return out.reshape(1, S, D)
```

```python
import jax
import jax.numpy as jnp
import jax.experimental.pallas as pl
import jax.experimental.pallas.tpu as pltpu

S, D, F = 2048, 1024, 3584
H, DH, W, DIL = 32, 32, 8, 2
NG = D // 128
TM = 256
NT = S // TM
T0 = 3
N1 = NT - T0 + 1
SUB = 128
HN = 256
FH = F // 2
DH2 = D // 2
KC = 128
NKC = D // KC
RU1 = 112
RU2 = 368
HALO = 16
PVS = 4
MR = 64
LNS = 2
NGRP = 2
UR, UC = 8, 256
WB1 = 1
WB2 = 1
LNR = 16
EPS = 1e-5
SCALE = DH ** -0.5
LOG2E = 1.4426950408889634
QSCALE = SCALE * LOG2E
NEG = -1000000000.0 * LOG2E

f32 = jnp.float32
bf16 = jnp.bfloat16
u32 = jnp.uint32

SEM_C = 0
SEM_X = 1
SEM_WQ0 = SEM_X + NT
SEM_CH = SEM_WQ0 + 1
SEM_WM = SEM_CH + NKC
SEM_WO = SEM_WM + 4
SEM_FF = SEM_WO + 2
SEM_OUT = SEM_FF + (N1 - 1)
NSEM = SEM_OUT + 2


def _when(cond, name):
    def deco(body):
        def scoped():
            with jax.named_scope(name):
                body()
        return pl.when(cond)(scoped)
    return deco


def _pack(x):
    return pltpu.bitcast(x, u32)


def _unpack(x):
    return pltpu.bitcast(x, bf16)


def _dot(a, b):
    return jnp.dot(a, b, preferred_element_type=f32)


class _Chain:
    def __init__(self, always):
        self.always = always
        self.tok = None

    def after(self, x):
        if self.tok is None:
            return x
        t = self.tok if self.tok.dtype == x.dtype else pltpu.bitcast(self.tok, x.dtype)
        return jax.lax.select(self.always, x, t)

    def after_rows(self, x):
        x00 = self.after(x[0:8, 0:128])
        top = x00 if x.shape[1] == 128 else jnp.concatenate([x00, x[0:8, 128:]], axis=1)
        return top if x.shape[0] == 8 else jnp.concatenate([top, x[8:]], axis=0)


def _swap_stage(a, k, b, axis):
    n = 128 if axis == 1 else 8
    idx = jax.lax.broadcasted_iota(jnp.int32, a[0].shape, axis)
    m0 = (idx & (1 << b)) == 0
    out = list(a)
    for c in range(8):
        if c & (1 << k):
            continue
        lo, hi = a[c], a[c | (1 << k)]
        out[c] = jax.lax.select(m0, lo, pltpu.roll(hi, 1 << b, axis))
        out[c | (1 << k)] = jax.lax.select(m0, pltpu.roll(lo, n - (1 << b), axis), hi)
    return out


def _permute_qkv_section(w_ref, r0, sec):
    c0 = sec * D if isinstance(sec, int) else pl.multiple_of(sec * D, D)
    a = [_pack(w_ref[pl.ds(r0, KC), pl.ds(c0 + c * 128, 128)]) for c in range(8)]
    for k in range(3):
        a = _swap_stage(a, k, k + 1, 1)
    return jnp.concatenate(a, axis=1)


def _ln_stats(x):
    m = jnp.mean(x, axis=-1, keepdims=True)
    xc = x - m
    v = jnp.mean(xc * xc, axis=-1, keepdims=True)
    r = jax.lax.rsqrt(v + EPS)
    return r, m * r


def _modulated_ln(x, scale1, shift):
    r, mr = _ln_stats(x)
    return (x * r - mr) * scale1 + shift


def _attention_rows(q_s, k_s, v_s, q0, row0, wb, pv):
    lane = jax.lax.broadcasted_iota(jnp.int32, (8, 128), 1)
    m0 = (lane & 1) == 0
    m4 = (lane & 16) == 0
    q = q_s[:, pl.ds(q0, 8), :] * QSCALE
    rows = [pl.ds(q0 + (HALO - DIL * w), 8) for w in range(W)]
    logits = []
    for w0 in range(0, W, wb):
        zs = [jnp.sum(q * k_s[:, rows[w], :], axis=0) for w in range(w0, w0 + wb)]
        zs = [z + jax.lax.select(m0, pltpu.roll(z, 127, 1), pltpu.roll(z, 1, 1)) for z in zs]
        zs = [z + jax.lax.select(m4, pltpu.roll(z, 112, 1), pltpu.roll(z, 16, 1)) for z in zs]
        for w, z in zip(range(w0, w0 + wb), zs):
            if w > 0 and row0 is not None:
                row = jax.lax.broadcasted_iota(jnp.int32, (8, 128), 0) + row0
                z = jnp.where(row >= DIL * w, z, NEG)
            logits.append(z)
    m = logits[0]
    for w in range(1, W):
        m = jnp.maximum(m, logits[w])
    e = [jnp.exp2(logits[w] - m) for w in range(W)]
    den = e[0]
    for w in range(1, W):
        den = den + e[w]
    inv = pl.reciprocal(den, approx=False)
    outs = []
    gs = NG // PVS
    eb = [None] + [jnp.broadcast_to(e[w], (gs, 8, 128)) for w in range(1, W)]
    for g0 in range(0, NG, gs):
        o = pv.after(e[0]) * v_s[g0:g0 + gs, rows[0], :]
        for w in range(1, W):
            o = o + eb[w] * v_s[g0:g0 + gs, rows[w], :]
        o = o * inv
        outs += [o[g] for g in range(gs)]
        pv.tok = outs[-1]
    return jnp.concatenate(outs, axis=1)


def _store_attention(oa_s, m0, top, bot):
    ops = _lhs_operands(top[:, :DH2], top[:, DH2:], bot[:, :DH2], bot[:, DH2:])
    oa_s[:, pl.ds(m0, 8), :] = jnp.stack(ops).astype(bf16)


def _attention(q_s, k_s, v_s, oa_s, q0, o0, nrows, wb, pv):
    for r in range(0, nrows, 16):
        halves = []
        for t in (0, 8):
            pv.tok = None
            halves.append(_attention_rows(q_s, k_s, v_s, q0 + r + t, None, wb, pv))
        _store_attention(oa_s, (o0 + r) // 2, *halves)


def _mod_cols(wmod_v, st_v, col, n, chain=None):
    acc = None
    for r in range(0, D, MR):
        s = st_v[r:r + MR, :]
        if r == 0 and chain is not None:
            s = chain.after_rows(s)
        if n > 128:
            s = jnp.concatenate([s] * (n // 128), axis=1)
        p = wmod_v[r:r + MR, pl.ds(col, n)].astype(f32) * s
        for i in range(0, MR, 8):
            acc = p[i:i + 8] if acc is None else acc + p[i:i + 8]
    if chain is not None:
        chain.tok = acc[:, 0:128]
    return acc.sum(axis=0, keepdims=True)


ORD_O = ORD_D = (0, 5, 6, 4, 2, 3, 1)
ORD_U = (0, 1, 2, 3, 4, 5, 6)
NS = 4


def _lhs_operands(a11, a12, a21, a22):
    s1 = a21 + a22
    s2 = s1 - a11
    return [a11, a12, a12 - s2, a22, s1, s2, a11 - a21]


def _rhs_sums(b11, b12, b21, b22):
    t1 = b12 - b11
    t2 = b22 - t1
    return (t2 - b21, t1, t2, b22 - b12)


def _rhs_operands(sums, b11, b21, b22):
    return [b11, b21, b22, sums(0), sums(1), sums(2), sums(3)]


def _products(a, b, order):
    m = {i: _dot(a[i], b[i]) for i in order}
    return [m[i] for i in range(7)]


def _combine(p):
    u2 = p[0] + p[5]
    u3 = u2 + p[6]
    return (p[0] + p[1], u2 + p[4] + p[2], u3 - p[3], u3 + p[4])


def _new_chain(flag_s):
    return _Chain(jax.lax.broadcasted_iota(jnp.int32, (8, 128), 1) < flag_s[0])


def _ln1_next(x_v, mod_v, h_s, r0, chains):
    sa = mod_v[0:1, 0 * D:1 * D]
    ca1 = 1.0 + mod_v[0:1, 1 * D:2 * D]
    for i, r in enumerate(range(0, TM, LNR)):
        chain = chains[i % len(chains)]
        x = chain.after_rows(x_v[pl.ds(r0 + r, LNR), :].astype(f32))
        h = _modulated_ln(x, ca1, sa)
        chain.tok = h[0:8, 0:128]
        h_s[pl.ds(r, LNR), :] = h.astype(bf16)


def _phase1(step, x_v, wqkv_p, wo_raw, wo_p, so_v, w1_v, w3_v, w2_v, s1_v, s3_v, s2_v, wmod_v, mod_v, st_v,
            h_s, q0_s, k0_s, v0_s, q_s, k_s, v_s, o_s, flag_s):
    step = jnp.clip(step, 1, N1 - 1)
    part = jnp.maximum(step - 2, 0)
    base = pl.multiple_of((step + T0 - 2) * TM, TM)
    h = h_s[...]
    chain = _new_chain(flag_s)

    ln_r0 = pl.multiple_of(jnp.minimum(step + T0, NT - 1) * TM, TM)
    sa = mod_v[0:1, 0 * D:1 * D]
    ca1 = 1.0 + mod_v[0:1, 1 * D:2 * D]

    def ln_unit(i):
        x = x_v[pl.ds(ln_r0 + i * 32, 32), :].astype(f32)
        x = jnp.concatenate([chain.after_rows(x[r:r + 8]) for r in range(0, 32, 8)], axis=0)
        hn = _modulated_ln(x, ca1, sa)
        chain.tok = hn[0:8, 0:128]
        h_s[pl.ds(i * 32, 32), :] = hn.astype(bf16)

    def wo_unit(mid):
        col = pl.multiple_of(part * 128, 128)
        lr = []
        for c0 in (col, DH2 + col):
            a = [_pack(wo_raw[pl.ds(c * 128 + mid * 16, 16), pl.ds(c0, 128)]) for c in range(8)]
            a[0] = chain.after(a[0])
            for k in range(3):
                a = _swap_stage(a, k, k, 0)
            chain.tok = a[7]
            lr.append(a)
        for s in range(4):
            q = [lr[0][s], lr[1][s], lr[0][s + 4], lr[1][s + 4]]
            wo_p[0, pl.ds(s * 64 + mid * 8, 8), pl.ds(col, 128)] = q[0]
            wo_p[1, pl.ds(s * 64 + mid * 8, 8), pl.ds(col, 128)] = q[2]
            wo_p[2, pl.ds(s * 64 + mid * 8, 8), pl.ds(col, 128)] = q[3]
            q[0] = chain.after(q[0])
            sums = _rhs_sums(*[_unpack(v).astype(f32) for v in q])
            chain.tok = sums[0][0:8]
            so_v[:, pl.ds(s * 128 + mid * 16, 16), pl.ds(col, 128)] = jnp.stack(sums).astype(bf16)

    at_r0 = pl.multiple_of(part * 64, 64)
    pv1 = _new_chain(flag_s)

    def attn_unit(i):
        halves = [_attention_rows(q0_s, k0_s, v0_s, at_r0 + i * 16 + t,
                                  at_r0 + t if i == 0 else None, WB1, pv1) for t in (0, 8)]
        _store_attention(o_s, pl.multiple_of(part * 32 + i * 8, 8), *halves)

    mod_col = pl.multiple_of(step * D, D)

    def mod_unit(i):
        col = pl.multiple_of(mod_col + i * 256, 256)
        val = _mod_cols(wmod_v, st_v, col, 256, chain)
        mod_v[:, pl.ds(col, 256)] = jnp.broadcast_to(val, (8, 256))

    sum_units = []
    for w_v, s_v, half, ru, ch in ((w1_v, s1_v, DH2, RU1, FH), (w3_v, s3_v, DH2, RU1, FH),
                                   (w2_v, s2_v, FH, RU2, DH2)):
        r_lo = jnp.minimum((step - 1) * (ru // 16), (half - ru) // 16)
        srcs = [w_v.at[pl.ds(pl.multiple_of(i * half + r_lo * 16, 16), ru)] for i in range(2)]
        dst = s_v.at[:, pl.ds(pl.multiple_of(r_lo * 16, 16), ru)]
        r_bk = jnp.clip(r_lo + flag_s[0] - 128, 0, (half - ru) // 16)
        back = s_v.at[:, pl.ds(pl.multiple_of(r_bk * 16, 16), ru)]
        sum_units += [(srcs, dst, back, ch, r, c0)
                      for r in range(0, ru, UR) for c0 in range(0, ch, UC)]

    def sum_unit(u):
        srcs, dst, back, ch, r, c0 = sum_units[u]
        q = [srcs[i][r:r + UR, j * ch + c0:j * ch + c0 + UC].astype(f32)
             for i in range(2) for j in range(2)]
        q[0] = chain.after_rows(q[0])
        dst[:, r:r + UR, c0:c0 + UC] = jnp.stack(_rhs_sums(*q)).astype(bf16)
        chain.tok = back[0, 0:8, 0:128].astype(f32)

    def mm_unit(t):
        sec, g = t // NG, t % NG
        dst, off = (q_s, k_s, v_s)[sec], (0 if sec == 0 else HALO)
        res = _dot(h, _unpack(wqkv_p[:, t * 128:(t + 1) * 128]))
        dst[g, pl.ds(base + off, TM), :] = res
        return res[0:8]

    _plan(chain, mm_unit, ln_unit, wo_unit, attn_unit, mod_unit, sum_unit, len(sum_units))


def _plan(chain, mm_unit, ln_unit, wo_unit, attn_unit, mod_unit, sum_unit, nsum):
    ticks = [mm_unit(t) for t in range(3 * NG)]
    done = 0
    for t in range(3 * NG - 1):
        chain.tok = ticks[t]
        if t < 8:
            ln_unit(t)
            wo_unit(t)
        if 15 <= t < 19:
            mod_unit(t - 15)
        n = 8 if t < 8 else 12 if 15 <= t < 19 else -(-(nsum - 112) // 11)
        for u in range(done, min(done + n, nsum)):
            sum_unit(u)
        done = min(done + n, nsum)
    assert done == nsum
    for i in range(4):
        attn_unit(i)


def _phase2(step, x_v, wo_p, so_v, w1_v, w3_v, w2_v, s1_v, s3_v, s2_v, mod_v, q_s, k_s, v_s, o_s, note_s,
            flag_s, o_ref):
    j2 = jnp.clip(step - N1, 0, NT - 1)
    ga = mod_v[0:1, 2 * D:3 * D]
    sb = mod_v[0:1, 3 * D:4 * D]
    cb1 = 1.0 + mod_v[0:1, 4 * D:5 * D]
    gb = mod_v[0:1, 5 * D:6 * D]
    row0 = pl.multiple_of(j2 * TM, TM)
    nsub = TM // SUB
    hs = SUB // 2
    os_ = [[o_s[i, pl.ds(s * hs, hs), :] for i in range(7)] for s in range(nsub)]
    x1s, blocks = [], []
    for s in range(nsub):
        b = _rhs_operands(lambda i: so_v[i], *[_unpack(wo_p[i]) for i in range(3)])
        c11, c12, c21, c22 = _combine(_products(os_[s], b, ORD_O))
        top = jnp.concatenate([c11, c12], axis=1)
        bot = jnp.concatenate([c21, c22], axis=1)
        att = jnp.concatenate([h[r:r + 8] for r in range(0, hs, 8) for h in (top, bot)], axis=0)
        note_s[...] = att[0:8, 0:128]
        x1 = x_v[pl.ds(row0 + s * SUB, SUB), :].astype(f32) + ga * att
        x1s.append(x1)
        chain = _new_chain(flag_s)
        for r in range(0, SUB, 32):
            xb = x1[r:r + 32]
            xb = jnp.concatenate([chain.after_rows(xb[0:16]), chain.after_rows(xb[16:32])], axis=0)
            rs, mr = _ln_stats(xb)
            chain.tok = None
            pieces = []
            cw = DH2 // LNS
            for c in range(0, DH2, cw):
                hl, hr = [(chain.after_rows(xb[:, c0:c0 + cw]) * rs - mr) * cb1[:, c0:c0 + cw]
                          + sb[:, c0:c0 + cw] for c0 in (c, DH2 + c)]
                pieces.append(_lhs_operands(hl[0:16], hr[0:16], hl[16:32], hr[16:32]))
                chain.tok = hr[24:32, cw - 128:cw]
            blocks.append([jnp.concatenate([pc[i] for pc in pieces], axis=1) for i in range(7)])

    nq = pl.multiple_of(jnp.minimum(j2, NT - 2) * TM, TM)

    def stack(per_group):
        return [jnp.concatenate([ops[i] for ops in per_group], axis=0) for i in range(7)]

    nb = len(blocks) // NGRP
    groups = [stack(blocks[g * nb:(g + 1) * nb]) for g in range(NGRP)]

    def up_proj(a, w_v, s_v, j):
        c0 = j * HN
        b = _rhs_operands(lambda i: s_v[i, :, c0:c0 + HN],
                          w_v[0:DH2, c0:c0 + HN],
                          w_v[DH2:, c0:c0 + HN], w_v[DH2:, FH + c0:FH + c0 + HN])
        return _combine(_products(a, b, ORD_U))

    def to_mxu(ops):
        return [v.astype(bf16) for v in ops]

    def gate_up(a, j):
        act = []
        for g, u in zip(up_proj(a, w1_v, s1_v, j), up_proj(a, w3_v, s3_v, j)):
            hg = 0.5 * g
            act.append((hg + hg * jnp.tanh(hg)) * u)
        return _lhs_operands(*act)

    h_all = to_mxu(stack(groups))
    first = []
    for g, ops in enumerate(groups):
        first.append(gate_up(to_mxu(ops), 0))
        rows = TM // NGRP
        _attention(q_s, k_s, v_s, o_s, nq + g * rows, g * rows, rows, WB2, _new_chain(flag_s))
    acc = None
    for j in range(FH // HN):
        a = to_mxu(stack(first) if j == 0 else gate_up(h_all, j))
        r0 = j * HN
        b = _rhs_operands(lambda i: s2_v[i, r0:r0 + HN, :],
                          w2_v[r0:r0 + HN, 0:DH2], w2_v[FH + r0:FH + r0 + HN, 0:DH2],
                          w2_v[FH + r0:FH + r0 + HN, DH2:])
        m = _products(a, b, ORD_D)
        acc = m if acc is None else [p + q for p, q in zip(acc, m)]
    c11, c12, c21, c22 = _combine(acc)
    x1 = jnp.concatenate(x1s, axis=0)
    for blk in range(TM // 32):
        rows = slice(blk * 16, (blk + 1) * 16)
        for t, (left, right) in enumerate(((c11, c12), (c21, c22))):
            y = jnp.concatenate([left[rows], right[rows]], axis=1)
            r = blk * 32 + t * 16
            o_ref[r:r + 16, :] = (x1[r:r + 16] + gb * y).astype(o_ref.dtype)


def _kernel(x_hbm, c_hbm, wqkv_hbm, wo_hbm, w1_hbm, w3_hbm, w2_hbm, wmod_hbm, o_hbm,
            x_v, wqkv_raw, wqkv_p, wo_raw, wo_p, so_v, w1_v, w3_v, w2_v, s1_v, s3_v, s2_v,
            wmod_v, mod_v, st_v, xn_s, wcur_s, hl_s, h_s, q0_s, k0_s, v0_s, q_s, k_s, v_s,
            o_s, o_ref, c_v, note_s, flag_s, sems):
    step = pl.program_id(0)

    def new_chain():
        return _new_chain(flag_s)

    def cp_rows(src, dst, r0, n, sem):
        rows = pl.ds(r0, n)
        return pltpu.make_async_copy(src.at[rows], dst.at[rows], sems.at[sem])

    def cp_cols(src, dst, c0, n, sem):
        cols = pl.ds(c0, n)
        return pltpu.make_async_copy(src.at[:, cols], dst.at[:, cols], sems.at[sem])

    cp_c = lambda: [pltpu.make_async_copy(c_hbm, c_v, sems.at[SEM_C])]
    cp_x = lambda i: [cp_rows(x_hbm, x_v, i * TM, TM, SEM_X + i)]
    cp_wq0 = lambda: [cp_rows(wqkv_hbm, wqkv_raw, 0, KC, SEM_WQ0)]
    cp_wm = lambda p: [cp_cols(wmod_hbm, wmod_v, (2 + p) * D, D, SEM_WM + p)]

    def cp_chunk(k, with_wq=True):
        cps = [cp_rows(wqkv_hbm, wqkv_raw, k * KC, KC, SEM_CH + k)] if with_wq else []
        return cps + [cp_cols(wmod_hbm, wmod_v, k * KC, KC, SEM_CH + k),
                      cp_cols(wmod_hbm, wmod_v, D + k * KC, KC, SEM_CH + k)]

    def cp_wo(i):
        c0, n = (0, 128) if i == 0 else (128, DH2 - 128)
        return [cp_cols(wo_hbm, wo_raw, h + c0, n, SEM_WO + i) for h in (0, DH2)]

    def cp_ff(i):
        cps = []
        for src, dst, half, ru in ((w1_hbm, w1_v, DH2, RU1), (w3_hbm, w3_v, DH2, RU1),
                                   (w2_hbm, w2_v, FH, RU2)):
            n = min(ru, half - i * ru)
            cps += [cp_rows(src, dst, h * half + i * ru, n, SEM_FF + i) for h in range(2)]
        return cps

    def wait(*groups):
        for cps in groups:
            for cp in cps:
                cp.wait()

    def qkv_dst(t, sec):
        off = 0 if sec == 0 else HALO
        if t == 0:
            return (q0_s, k0_s, v0_s)[sec], off
        return (q_s, k_s, v_s)[sec], off + (t - 1) * TM

    @_when(step == 0, 'first')
    def _first():
        order = cp_c() + cp_x(0) + cp_wq0() + cp_chunk(0, False) + cp_x(1) + cp_x(2)
        for k in range(1, NKC):
            order += cp_chunk(k)
        order += cp_x(3) + cp_x(4) + cp_wo(0) + cp_ff(0)
        order += cp_x(5) + cp_wm(0) + cp_ff(1)
        order += cp_x(6) + cp_wo(1) + cp_wm(1) + cp_ff(2)
        order += cp_x(7) + cp_wm(2) + cp_ff(3)
        order += cp_wm(3) + cp_ff(4)
        for cp in order:
            cp.start()
        flag_s[0] = 128

        last = T0 - 1

        def zero_body(g, carry):
            for sec in range(3):
                dst, off = qkv_dst(last, sec)
                dst[g, pl.ds(off, TM), :] = jnp.zeros((TM, 128), f32)
            return carry
        jax.lax.fori_loop(0, NG, zero_body, 0)
        wait(cp_c())
        c = c_v[...].astype(f32)
        sc = c * jax.nn.sigmoid(c)
        st_v[...] = jnp.transpose(jnp.broadcast_to(sc, (128, D)))

        def normalize(row0, nrows, chains=None):
            for i in range(nrows // LNR):
                r0 = row0 + i * LNR
                x = x_v[pl.ds(r0, LNR), :].astype(f32)
                if chains is not None:
                    x = chains[i % len(chains)].after_rows(x)
                r, mr = _ln_stats(x)
                xn = x * r - mr
                if chains is not None:
                    chains[i % len(chains)].tok = xn[0:8, 0:128]
                for g in range(NG):
                    xn_s[g, pl.ds(r0, LNR), :] = xn[:, g * 128:(g + 1) * 128]

        def mod_chunk(k):
            col = k * KC if isinstance(k, int) else pl.multiple_of(k * KC, KC)
            sa = _mod_cols(wmod_v, st_v, col, KC)
            ca = _mod_cols(wmod_v, st_v, D + col, KC)
            mod_v[:, pl.ds(col, KC)] = jnp.broadcast_to(sa, (8, KC))
            mod_v[:, pl.ds(D + col, KC)] = jnp.broadcast_to(ca, (8, KC))
            return sa, 1.0 + ca

        def h_chunk(k, t, n, sa, ca1):
            return (xn_s[k, pl.ds(t * TM, n * TM), :] * ca1 + sa).astype(bf16)

        def mm(h, w, sec, tiles, first):
            res = _dot(h, _unpack(w))
            for i, t in enumerate(tiles):
                dst, off = qkv_dst(t, sec)
                for g in range(NG):
                    blk = res[i * TM:(i + 1) * TM, g * 128:(g + 1) * 128]
                    if first:
                        dst[g, pl.ds(off, TM), :] = blk
                    else:
                        dst[g, pl.ds(off, TM), :] += blk

        def wcur(sec):
            return wcur_s[:, sec * D:(sec + 1) * D]

        def keep(k, sec, wp):
            r0 = k * (KC // 2) if isinstance(k, int) else pl.multiple_of(k * (KC // 2), KC // 2)
            cols = pl.ds(sec * D if isinstance(sec, int) else pl.multiple_of(sec * D, D), D)
            wcur_s[:, cols] = wp
            wqkv_p[pl.ds(r0, KC // 2), cols] = wp

        scope = jax.named_scope
        mod0 = lambda: (mod_v[0:1, 0:KC], 1.0 + mod_v[0:1, D:D + KC])
        with scope('w_x0'):
            wait(cp_x(0))
        with scope('norm0'):
            def norm_body(i, carry):
                normalize(pl.multiple_of(i * 64, 64), 64)
                return carry
            jax.lax.fori_loop(0, TM // 64, norm_body, 0)
        with scope('w_wq0'):
            wait(cp_wq0())
        with scope('perm0'):
            def perm_body(sec, carry):
                keep(0, sec, _permute_qkv_section(wqkv_raw, 0, sec))
                return carry
            jax.lax.fori_loop(0, 2, perm_body, 0)
        with scope('w_m0'):
            wait(cp_chunk(0, False))
        with scope('mm00'):
            wp = _permute_qkv_section(wqkv_raw, 0, 2)
            sa, ca1 = mod_chunk(0)
            h0 = h_chunk(0, 0, 1, sa, ca1)
            for sec in range(3):
                mm(h0, wcur(sec) if sec < 2 else wp, sec, [0], True)
            keep(0, 2, wp)
        with scope('w_x12'):
            wait(cp_x(1), cp_x(2))
        with scope('mm01'):
            normalize(TM, TM)
            h1 = h_chunk(0, 1, 1, *mod0())
            for sec in range(3):
                mm(h1, wcur(sec), sec, [1], True)
            normalize(2 * TM, TM, [new_chain() for _ in range(4)])
            hl_s[...] = _pack(h_chunk(0, last, 1, *mod0()))

        def chunk_body(k0, carry):
            k = k0 + 1
            with scope('w_chunk'):
                wait(cp_chunk(k))
            with scope('chunk'):
                hl = _unpack(hl_s[...])
                for sec in range(3):
                    mm(hl, wcur(sec), sec, [last], False)
                sa, ca1 = mod_chunk(k)
                hf = h_chunk(k, 0, last, sa, ca1)
                hl_s[...] = _pack(h_chunk(k, last, 1, sa, ca1))
                for sec in range(3):
                    wp = _permute_qkv_section(wqkv_raw, pl.multiple_of(k * KC, KC), sec)
                    mm(hf, wp, sec, list(range(last)), False)
                    keep(k, sec, wp)
            return carry
        jax.lax.fori_loop(0, NKC - 1, chunk_body, 0)

        with scope('w_x3'):
            wait(cp_x(T0))
        hl = _unpack(hl_s[...])
        for sec in range(3):
            mm(hl, wcur(sec), sec, [last], False)
        _ln1_next(x_v, mod_v, h_s, T0 * TM, [new_chain() for _ in range(4)])
        k0_s[:, 0:HALO, :] = jnp.zeros((NG, HALO, 128), f32)
        v0_s[:, 0:HALO, :] = jnp.broadcast_to(v0_s[:, HALO:HALO + 1, :], (NG, HALO, 128))
        k_s[:, 0:HALO, :] = k0_s[:, TM:TM + HALO, :]
        v_s[:, 0:HALO, :] = v0_s[:, TM:TM + HALO, :]

    @_when(step == 1, 'wait1')
    def _():
        wait(cp_x(4), cp_wo(0), cp_ff(0))

    @_when(step == 2, 'wait2')
    def _():
        wait(cp_x(5), cp_wm(0), cp_ff(1))

    @_when(step == 3, 'wait3')
    def _():
        wait(cp_x(6), cp_wo(1), cp_wm(1), cp_ff(2))

    @_when(step == 4, 'wait4')
    def _():
        wait(cp_x(7), cp_wm(2), cp_ff(3))

    @_when(step == 5, 'wait5')
    def _():
        wait(cp_wm(3), cp_ff(4))

    @_when(jnp.logical_and(step >= 1, step < N1), 'phase1')
    def _():
        _phase1(step, x_v, wqkv_p, wo_raw, wo_p, so_v, w1_v, w3_v, w2_v, s1_v, s3_v, s2_v, wmod_v, mod_v, st_v,
                h_s, q0_s, k0_s, v0_s, q_s, k_s, v_s, o_s, flag_s)

    def cp_out(j):
        rows = pl.ds(pl.multiple_of(j * TM, TM), TM)
        return pltpu.make_async_copy(o_ref.at[j % 2], o_hbm.at[rows], sems.at[SEM_OUT + j % 2])

    @_when(step > N1 + 1, 'wait_out')
    def _():
        cp_out(step - N1 - 2).wait()

    @_when(step >= N1, 'phase2')
    def _():
        _phase2(step, x_v, wo_p, so_v, w1_v, w3_v, w2_v, s1_v, s3_v, s2_v, mod_v, q_s, k_s, v_s, o_s, note_s,
                flag_s, o_ref.at[(step - N1) % 2])
        cp_out(step - N1).start()

    @_when(step == N1 + NT - 1, 'wait_last')
    def _():
        cp_out(NT - 2).wait()
        cp_out(NT - 1).wait()


def _scratch_shapes():
    return [
        pltpu.VMEM((S, D), bf16),
        pltpu.VMEM((D, 3 * D), bf16),
        pltpu.VMEM((D // 2, 3 * D), u32),
        pltpu.VMEM((D, D), bf16),
        pltpu.VMEM((3, DH2 // 2, DH2), u32),
        pltpu.VMEM((NS, DH2, DH2), bf16),
        pltpu.VMEM((D, F), bf16),
        pltpu.VMEM((D, F), bf16),
        pltpu.VMEM((F, D), bf16),
        pltpu.VMEM((NS, DH2, FH), bf16),
        pltpu.VMEM((NS, DH2, FH), bf16),
        pltpu.VMEM((NS, FH, DH2), bf16),
        pltpu.VMEM((D, 6 * D), bf16),
        pltpu.VMEM((8, 6 * D), f32),
        pltpu.VMEM((D, 128), f32),
        pltpu.VMEM((NG, T0 * TM, 128), f32),
        pltpu.VMEM((KC // 2, 3 * D), u32),
        pltpu.VMEM((TM // 2, KC), u32),
        pltpu.VMEM((TM, D), bf16),
        pltpu.VMEM((NG, TM, 128), f32),
        pltpu.VMEM((NG, HALO + TM, 128), f32),
        pltpu.VMEM((NG, HALO + TM, 128), f32),
        pltpu.VMEM((NG, S - TM, 128), f32),
        pltpu.VMEM((NG, HALO + S - TM, 128), f32),
        pltpu.VMEM((NG, HALO + S - TM, 128), f32),
        pltpu.VMEM((7, TM // 2, DH2), bf16),
        pltpu.VMEM((2, TM, D), bf16),
        pltpu.VMEM((1, D), bf16),
        pltpu.VMEM((8, 128), f32),
        pltpu.SMEM((1,), jnp.int32),
        pltpu.SemaphoreType.DMA((NSEM,)),
    ]


@jax.jit
def pallas_adaLN_cond__sliding_local_dilated__glu_gated_swiglu__prompt_kernel(
    A_x: jax.Array,
    A_wqkv: jax.Array,
    A_wo: jax.Array,
    B_x: jax.Array,
    B_w1: jax.Array,
    B_w3: jax.Array,
    B_w2: jax.Array,
    c: jax.Array,
    w_mod: jax.Array,
):
    del B_x
    x = A_x.reshape(S, D)
    hbm = pl.BlockSpec(memory_space=pl.ANY)
    out = pl.pallas_call(
        _kernel,
        grid=(N1 + NT,),
        in_specs=[hbm] * 8,
        out_specs=hbm,
        out_shape=jax.ShapeDtypeStruct((S, D), A_x.dtype),
        scratch_shapes=_scratch_shapes(),
        compiler_params=pltpu.CompilerParams(
            dimension_semantics=("arbitrary",),
            vmem_limit_bytes=122 * 1024 * 1024,
        ),
        name="adaln_attn_ffn",
    )(x, c, A_wqkv, A_wo, B_w1, B_w3, B_w2, w_mod)
    return out.reshape(1, S, D)
```

```python
import jax
import jax.numpy as jnp
import jax.experimental.pallas as pl
import jax.experimental.pallas.tpu as pltpu

S, D, F = 2048, 1024, 3584
H, DH, W, DIL = 32, 32, 8, 2
NG = D // 128
TM = 256
NT = S // TM
T0 = 3
N1 = NT - T0 + 1
SUB = 128
HN = 256
FH = F // 2
DH2 = D // 2
KC = 128
NKC = D // KC
RU1 = 112
RU2 = 368
HALO = 16
PVS = 4
MR = 64
LNS = 2
NGRP = 2
UR, UC = 8, 256
WB1 = 1
WB2 = 1
LNR = 16
EPS = 1e-5
SCALE = DH ** -0.5
LOG2E = 1.4426950408889634
QSCALE = SCALE * LOG2E
NEG = -1000000000.0 * LOG2E

f32 = jnp.float32
bf16 = jnp.bfloat16
u32 = jnp.uint32

SEM_C = 0
SEM_X = 1
SEM_WQ0 = SEM_X + NT
SEM_CH = SEM_WQ0 + 1
SEM_WM = SEM_CH + NKC
SEM_WO = SEM_WM + 4
SEM_FF = SEM_WO + 2
SEM_OUT = SEM_FF + (N1 - 1)
NSEM = SEM_OUT + 2


def _when(cond, name):
    def deco(body):
        def scoped():
            with jax.named_scope(name):
                body()
        return pl.when(cond)(scoped)
    return deco


def _pack(x):
    return pltpu.bitcast(x, u32)


def _unpack(x):
    return pltpu.bitcast(x, bf16)


def _dot(a, b):
    return jnp.dot(a, b, preferred_element_type=f32)


class _Chain:
    def __init__(self, always):
        self.always = always
        self.tok = None

    def after(self, x):
        if self.tok is None:
            return x
        t = self.tok if self.tok.dtype == x.dtype else pltpu.bitcast(self.tok, x.dtype)
        return jax.lax.select(self.always, x, t)

    def after_rows(self, x):
        x00 = self.after(x[0:8, 0:128])
        top = x00 if x.shape[1] == 128 else jnp.concatenate([x00, x[0:8, 128:]], axis=1)
        return top if x.shape[0] == 8 else jnp.concatenate([top, x[8:]], axis=0)


def _swap_stage(a, k, b, axis):
    n = 128 if axis == 1 else 8
    idx = jax.lax.broadcasted_iota(jnp.int32, a[0].shape, axis)
    m0 = (idx & (1 << b)) == 0
    out = list(a)
    for c in range(8):
        if c & (1 << k):
            continue
        lo, hi = a[c], a[c | (1 << k)]
        out[c] = jax.lax.select(m0, lo, pltpu.roll(hi, 1 << b, axis))
        out[c | (1 << k)] = jax.lax.select(m0, pltpu.roll(lo, n - (1 << b), axis), hi)
    return out


def _permute_qkv_section(w_ref, r0, sec):
    c0 = sec * D if isinstance(sec, int) else pl.multiple_of(sec * D, D)
    a = [_pack(w_ref[pl.ds(r0, KC), pl.ds(c0 + c * 128, 128)]) for c in range(8)]
    for k in range(3):
        a = _swap_stage(a, k, k + 1, 1)
    return jnp.concatenate(a, axis=1)


def _ln_stats(x):
    m = jnp.mean(x, axis=-1, keepdims=True)
    xc = x - m
    v = jnp.mean(xc * xc, axis=-1, keepdims=True)
    r = jax.lax.rsqrt(v + EPS)
    return r, m * r


def _modulated_ln(x, scale1, shift):
    r, mr = _ln_stats(x)
    return (x * r - mr) * scale1 + shift


def _attention_rows(q_s, k_s, v_s, q0, row0, wb, pv):
    lane = jax.lax.broadcasted_iota(jnp.int32, (8, 128), 1)
    m0 = (lane & 1) == 0
    m4 = (lane & 16) == 0
    q = q_s[:, pl.ds(q0, 8), :] * QSCALE
    rows = [pl.ds(q0 + (HALO - DIL * w), 8) for w in range(W)]
    logits = []
    for w0 in range(0, W, wb):
        zs = [jnp.sum(q * k_s[:, rows[w], :], axis=0) for w in range(w0, w0 + wb)]
        zs = [z + jax.lax.select(m0, pltpu.roll(z, 127, 1), pltpu.roll(z, 1, 1)) for z in zs]
        zs = [z + jax.lax.select(m4, pltpu.roll(z, 112, 1), pltpu.roll(z, 16, 1)) for z in zs]
        for w, z in zip(range(w0, w0 + wb), zs):
            if w > 0 and row0 is not None:
                row = jax.lax.broadcasted_iota(jnp.int32, (8, 128), 0) + row0
                z = jnp.where(row >= DIL * w, z, NEG)
            logits.append(z)
    m = logits[0]
    for w in range(1, W):
        m = jnp.maximum(m, logits[w])
    e = [jnp.exp2(logits[w] - m) for w in range(W)]
    den = e[0]
    for w in range(1, W):
        den = den + e[w]
    inv = pl.reciprocal(den, approx=False)
    outs = []
    gs = NG // PVS
    eb = [None] + [jnp.broadcast_to(e[w], (gs, 8, 128)) for w in range(1, W)]
    for g0 in range(0, NG, gs):
        o = pv.after(e[0]) * v_s[g0:g0 + gs, rows[0], :]
        for w in range(1, W):
            o = o + eb[w] * v_s[g0:g0 + gs, rows[w], :]
        o = o * inv
        outs += [o[g] for g in range(gs)]
        pv.tok = outs[-1]
    return jnp.concatenate(outs, axis=1)


def _store_attention(oa_s, m0, top, bot):
    ops = _lhs_operands(top[:, :DH2], top[:, DH2:], bot[:, :DH2], bot[:, DH2:])
    oa_s[:, pl.ds(m0, 8), :] = jnp.stack(ops).astype(bf16)


def _attention(q_s, k_s, v_s, oa_s, q0, o0, nrows, wb, pv):
    for r in range(0, nrows, 16):
        halves = []
        for t in (0, 8):
            pv.tok = None
            halves.append(_attention_rows(q_s, k_s, v_s, q0 + r + t, None, wb, pv))
        _store_attention(oa_s, (o0 + r) // 2, *halves)


def _mod_cols(wmod_v, st_v, col, n, chain=None):
    acc = None
    for r in range(0, D, MR):
        s = st_v[r:r + MR, :]
        if r == 0 and chain is not None:
            s = chain.after_rows(s)
        if n > 128:
            s = jnp.concatenate([s] * (n // 128), axis=1)
        p = wmod_v[r:r + MR, pl.ds(col, n)].astype(f32) * s
        for i in range(0, MR, 8):
            acc = p[i:i + 8] if acc is None else acc + p[i:i + 8]
    if chain is not None:
        chain.tok = acc[:, 0:128]
    return acc.sum(axis=0, keepdims=True)


ORD_O = ORD_D = (0, 5, 6, 4, 2, 3, 1)
ORD_U = (0, 1, 2, 3, 4, 5, 6)
NS = 4


def _lhs_operands(a11, a12, a21, a22):
    s1 = a21 + a22
    s2 = s1 - a11
    return [a11, a12, a12 - s2, a22, s1, s2, a11 - a21]


def _rhs_sums(b11, b12, b21, b22):
    t1 = b12 - b11
    t2 = b22 - t1
    return (t2 - b21, t1, t2, b22 - b12)


def _rhs_operands(sums, b11, b21, b22):
    return [b11, b21, b22, sums(0), sums(1), sums(2), sums(3)]


def _products(a, b, order):
    m = {i: _dot(a[i], b[i]) for i in order}
    return [m[i] for i in range(7)]


def _combine(p):
    u2 = p[0] + p[5]
    u3 = u2 + p[6]
    return (p[0] + p[1], u2 + p[4] + p[2], u3 - p[3], u3 + p[4])


def _new_chain(flag_s):
    return _Chain(jax.lax.broadcasted_iota(jnp.int32, (8, 128), 1) < flag_s[0])


def _ln1_next(x_v, mod_v, h_s, r0, chains):
    sa = mod_v[0:1, 0 * D:1 * D]
    ca1 = 1.0 + mod_v[0:1, 1 * D:2 * D]
    for i, r in enumerate(range(0, TM, LNR)):
        chain = chains[i % len(chains)]
        x = chain.after_rows(x_v[pl.ds(r0 + r, LNR), :].astype(f32))
        h = _modulated_ln(x, ca1, sa)
        chain.tok = h[0:8, 0:128]
        h_s[pl.ds(r, LNR), :] = h.astype(bf16)


def _phase1(step, x_v, wqkv_p, wo_raw, wo_p, so_v, w1_v, w3_v, w2_v, s1_v, s3_v, s2_v, wmod_v, mod_v, st_v,
            h_s, q0_s, k0_s, v0_s, q_s, k_s, v_s, o_s, flag_s):
    step = jnp.clip(step, 1, N1 - 1)
    part = jnp.maximum(step - 2, 0)
    base = pl.multiple_of((step + T0 - 2) * TM, TM)
    h = h_s[...]
    chain = _new_chain(flag_s)

    ln_r0 = pl.multiple_of(jnp.minimum(step + T0, NT - 1) * TM, TM)
    sa = mod_v[0:1, 0 * D:1 * D]
    ca1 = 1.0 + mod_v[0:1, 1 * D:2 * D]

    def ln_unit(i):
        x = x_v[pl.ds(ln_r0 + i * 32, 32), :].astype(f32)
        x = jnp.concatenate([chain.after_rows(x[r:r + 8]) for r in range(0, 32, 8)], axis=0)
        hn = _modulated_ln(x, ca1, sa)
        chain.tok = hn[0:8, 0:128]
        h_s[pl.ds(i * 32, 32), :] = hn.astype(bf16)

    def wo_unit(mid):
        col = pl.multiple_of(part * 128, 128)
        lr = []
        for c0 in (col, DH2 + col):
            a = [_pack(wo_raw[pl.ds(c * 128 + mid * 16, 16), pl.ds(c0, 128)]) for c in range(8)]
            a[0] = chain.after(a[0])
            for k in range(3):
                a = _swap_stage(a, k, k, 0)
            chain.tok = a[7]
            lr.append(a)
        for s in range(4):
            q = [lr[0][s], lr[1][s], lr[0][s + 4], lr[1][s + 4]]
            wo_p[0, pl.ds(s * 64 + mid * 8, 8), pl.ds(col, 128)] = q[0]
            wo_p[1, pl.ds(s * 64 + mid * 8, 8), pl.ds(col, 128)] = q[2]
            wo_p[2, pl.ds(s * 64 + mid * 8, 8), pl.ds(col, 128)] = q[3]
            q[0] = chain.after(q[0])
            sums = _rhs_sums(*[_unpack(v).astype(f32) for v in q])
            chain.tok = sums[0][0:8]
            so_v[:, pl.ds(s * 128 + mid * 16, 16), pl.ds(col, 128)] = jnp.stack(sums).astype(bf16)

    at_r0 = pl.multiple_of(part * 64, 64)
    pv1 = _new_chain(flag_s)

    def attn_unit(i):
        halves = [_attention_rows(q0_s, k0_s, v0_s, at_r0 + i * 16 + t,
                                  at_r0 + t if i == 0 else None, WB1, pv1) for t in (0, 8)]
        _store_attention(o_s, pl.multiple_of(part * 32 + i * 8, 8), *halves)

    mod_col = pl.multiple_of(step * D, D)

    def mod_unit(i):
        col = pl.multiple_of(mod_col + i * 256, 256)
        val = _mod_cols(wmod_v, st_v, col, 256, chain)
        mod_v[:, pl.ds(col, 256)] = jnp.broadcast_to(val, (8, 256))

    sum_units = []
    for w_v, s_v, half, ru, ch in ((w1_v, s1_v, DH2, RU1, FH), (w3_v, s3_v, DH2, RU1, FH),
                                   (w2_v, s2_v, FH, RU2, DH2)):
        r_lo = jnp.minimum((step - 1) * (ru // 16), (half - ru) // 16)
        srcs = [w_v.at[pl.ds(pl.multiple_of(i * half + r_lo * 16, 16), ru)] for i in range(2)]
        dst = s_v.at[:, pl.ds(pl.multiple_of(r_lo * 16, 16), ru)]
        r_bk = jnp.clip(r_lo + flag_s[0] - 128, 0, (half - ru) // 16)
        back = s_v.at[:, pl.ds(pl.multiple_of(r_bk * 16, 16), ru)]
        sum_units += [(srcs, dst, back, ch, r, c0)
                      for r in range(0, ru, UR) for c0 in range(0, ch, UC)]

    def sum_unit(u):
        srcs, dst, back, ch, r, c0 = sum_units[u]
        q = [srcs[i][r:r + UR, j * ch + c0:j * ch + c0 + UC].astype(f32)
             for i in range(2) for j in range(2)]
        q[0] = chain.after_rows(q[0])
        dst[:, r:r + UR, c0:c0 + UC] = jnp.stack(_rhs_sums(*q)).astype(bf16)
        chain.tok = back[0, 0:8, 0:128].astype(f32)

    def mm_unit(t):
        sec, g = t // NG, t % NG
        dst, off = (q_s, k_s, v_s)[sec], (0 if sec == 0 else HALO)
        res = _dot(h, _unpack(wqkv_p[:, t * 128:(t + 1) * 128]))
        dst[g, pl.ds(base + off, TM), :] = res
        return res[0:8]

    _plan(chain, mm_unit, ln_unit, wo_unit, attn_unit, mod_unit, sum_unit, len(sum_units))


def _plan(chain, mm_unit, ln_unit, wo_unit, attn_unit, mod_unit, sum_unit, nsum):
    ticks = [mm_unit(t) for t in range(3 * NG)]
    done = 0
    for t in range(3 * NG - 1):
        chain.tok = ticks[t]
        if t < 8:
            ln_unit(t)
            wo_unit(t)
        if 15 <= t < 19:
            mod_unit(t - 15)
        n = 8 if t < 8 else 12 if 15 <= t < 19 else -(-(nsum - 112) // 11)
        for u in range(done, min(done + n, nsum)):
            sum_unit(u)
        done = min(done + n, nsum)
    assert done == nsum
    for i in range(4):
        attn_unit(i)


def _phase2(step, x_v, wo_p, so_v, w1_v, w3_v, w2_v, s1_v, s3_v, s2_v, mod_v, q_s, k_s, v_s, o_s, note_s,
            flag_s, o_ref):
    j2 = jnp.clip(step - N1, 0, NT - 1)
    ga = mod_v[0:1, 2 * D:3 * D]
    sb = mod_v[0:1, 3 * D:4 * D]
    cb1 = 1.0 + mod_v[0:1, 4 * D:5 * D]
    gb = mod_v[0:1, 5 * D:6 * D]
    row0 = pl.multiple_of(j2 * TM, TM)
    nsub = TM // SUB
    hs = SUB // 2
    os_ = [[o_s[i, pl.ds(s * hs, hs), :] for i in range(7)] for s in range(nsub)]
    x1s, blocks = [], []
    for s in range(nsub):
        b = _rhs_operands(lambda i: so_v[i], *[_unpack(wo_p[i]) for i in range(3)])
        c11, c12, c21, c22 = _combine(_products(os_[s], b, ORD_O))
        top = jnp.concatenate([c11, c12], axis=1)
        bot = jnp.concatenate([c21, c22], axis=1)
        att = jnp.concatenate([h[r:r + 8] for r in range(0, hs, 8) for h in (top, bot)], axis=0)
        note_s[...] = att[0:8, 0:128]
        x1 = x_v[pl.ds(row0 + s * SUB, SUB), :].astype(f32) + ga * att
        x1s.append(x1)
        chain = _new_chain(flag_s)
        for r in range(0, SUB, 32):
            xb = x1[r:r + 32]
            xb = jnp.concatenate([chain.after_rows(xb[0:16]), chain.after_rows(xb[16:32])], axis=0)
            rs, mr = _ln_stats(xb)
            chain.tok = None
            pieces = []
            cw = DH2 // LNS
            for c in range(0, DH2, cw):
                hl, hr = [(chain.after_rows(xb[:, c0:c0 + cw]) * rs - mr) * cb1[:, c0:c0 + cw]
                          + sb[:, c0:c0 + cw] for c0 in (c, DH2 + c)]
                pieces.append(_lhs_operands(hl[0:16], hr[0:16], hl[16:32], hr[16:32]))
                chain.tok = hr[24:32, cw - 128:cw]
            blocks.append([jnp.concatenate([pc[i] for pc in pieces], axis=1) for i in range(7)])

    nq = pl.multiple_of(jnp.minimum(j2, NT - 2) * TM, TM)

    def stack(per_group):
        return [jnp.concatenate([ops[i] for ops in per_group], axis=0) for i in range(7)]

    nb = len(blocks) // NGRP
    groups = [stack(blocks[g * nb:(g + 1) * nb]) for g in range(NGRP)]

    def up_proj(a, w_v, s_v, j):
        c0 = j * HN
        b = _rhs_operands(lambda i: s_v[i, :, c0:c0 + HN],
                          w_v[0:DH2, c0:c0 + HN],
                          w_v[DH2:, c0:c0 + HN], w_v[DH2:, FH + c0:FH + c0 + HN])
        return _combine(_products(a, b, ORD_U))

    def to_mxu(ops):
        return [v.astype(bf16) for v in ops]

    def gate_up(a, j):
        act = []
        for g, u in zip(up_proj(a, w1_v, s1_v, j), up_proj(a, w3_v, s3_v, j)):
            hg = 0.5 * g
            act.append((hg + hg * jnp.tanh(hg)) * u)
        return _lhs_operands(*act)

    h_all = to_mxu(stack(groups))
    first = []
    for g, ops in enumerate(groups):
        first.append(gate_up(to_mxu(ops), 0))
        rows = TM // NGRP
        _attention(q_s, k_s, v_s, o_s, nq + g * rows, g * rows, rows, WB2, _new_chain(flag_s))
    acc = None
    for j in range(FH // HN):
        a = to_mxu(stack(first) if j == 0 else gate_up(h_all, j))
        r0 = j * HN
        b = _rhs_operands(lambda i: s2_v[i, r0:r0 + HN, :],
                          w2_v[r0:r0 + HN, 0:DH2], w2_v[FH + r0:FH + r0 + HN, 0:DH2],
                          w2_v[FH + r0:FH + r0 + HN, DH2:])
        m = _products(a, b, ORD_D)
        acc = m if acc is None else [p + q for p, q in zip(acc, m)]
    c11, c12, c21, c22 = _combine(acc)
    x1 = jnp.concatenate(x1s, axis=0)
    for blk in range(TM // 32):
        rows = slice(blk * 16, (blk + 1) * 16)
        for t, (left, right) in enumerate(((c11, c12), (c21, c22))):
            y = jnp.concatenate([left[rows], right[rows]], axis=1)
            r = blk * 32 + t * 16
            o_ref[r:r + 16, :] = (x1[r:r + 16] + gb * y).astype(o_ref.dtype)


def _kernel(x_hbm, c_hbm, wqkv_hbm, wo_hbm, w1_hbm, w3_hbm, w2_hbm, wmod_hbm, o_hbm,
            x_v, wqkv_raw, wqkv_p, wo_raw, wo_p, so_v, w1_v, w3_v, w2_v, s1_v, s3_v, s2_v,
            wmod_v, mod_v, st_v, xn_s, wcur_s, hl_s, h_s, q0_s, k0_s, v0_s, q_s, k_s, v_s,
            o_s, o_ref, c_v, note_s, flag_s, sems):
    step = pl.program_id(0)

    def new_chain():
        return _new_chain(flag_s)

    def cp_rows(src, dst, r0, n, sem):
        rows = pl.ds(r0, n)
        return pltpu.make_async_copy(src.at[rows], dst.at[rows], sems.at[sem])

    def cp_cols(src, dst, c0, n, sem):
        cols = pl.ds(c0, n)
        return pltpu.make_async_copy(src.at[:, cols], dst.at[:, cols], sems.at[sem])

    cp_c = lambda: [pltpu.make_async_copy(c_hbm, c_v, sems.at[SEM_C])]
    cp_x = lambda i: [cp_rows(x_hbm, x_v, i * TM, TM, SEM_X + i)]
    cp_wq0 = lambda: [cp_rows(wqkv_hbm, wqkv_raw, 0, KC, SEM_WQ0)]
    cp_wm = lambda p: [cp_cols(wmod_hbm, wmod_v, (2 + p) * D, D, SEM_WM + p)]

    def cp_chunk(k, with_wq=True):
        cps = [cp_rows(wqkv_hbm, wqkv_raw, k * KC, KC, SEM_CH + k)] if with_wq else []
        return cps + [cp_cols(wmod_hbm, wmod_v, k * KC, KC, SEM_CH + k),
                      cp_cols(wmod_hbm, wmod_v, D + k * KC, KC, SEM_CH + k)]

    def cp_wo(i):
        c0, n = (0, 128) if i == 0 else (128, DH2 - 128)
        return [cp_cols(wo_hbm, wo_raw, h + c0, n, SEM_WO + i) for h in (0, DH2)]

    def cp_ff(i):
        cps = []
        for src, dst, half, ru in ((w1_hbm, w1_v, DH2, RU1), (w3_hbm, w3_v, DH2, RU1),
                                   (w2_hbm, w2_v, FH, RU2)):
            n = min(ru, half - i * ru)
            cps += [cp_rows(src, dst, h * half + i * ru, n, SEM_FF + i) for h in range(2)]
        return cps

    def wait(*groups):
        for cps in groups:
            for cp in cps:
                cp.wait()

    def qkv_dst(t, sec):
        off = 0 if sec == 0 else HALO
        if t == 0:
            return (q0_s, k0_s, v0_s)[sec], off
        return (q_s, k_s, v_s)[sec], off + (t - 1) * TM

    @_when(step == 0, 'first')
    def _first():
        order = cp_c() + cp_x(0) + cp_wq0() + cp_chunk(0, False) + cp_x(1) + cp_x(2)
        for k in range(1, NKC):
            order += cp_chunk(k)
        order += cp_x(3) + cp_x(4) + cp_wo(0) + cp_ff(0)
        order += cp_x(5) + cp_wm(0) + cp_ff(1)
        order += cp_x(6) + cp_wo(1) + cp_wm(1) + cp_ff(2)
        order += cp_x(7) + cp_wm(2) + cp_ff(3)
        order += cp_wm(3) + cp_ff(4)
        for cp in order:
            cp.start()
        flag_s[0] = 128

        last = T0 - 1

        def zero_body(g, carry):
            for sec in range(3):
                dst, off = qkv_dst(last, sec)
                dst[g, pl.ds(off, TM), :] = jnp.zeros((TM, 128), f32)
            return carry
        jax.lax.fori_loop(0, NG, zero_body, 0)
        wait(cp_c())
        c = c_v[...].astype(f32)
        sc = c * jax.nn.sigmoid(c)
        st_v[...] = jnp.transpose(jnp.broadcast_to(sc, (128, D)))

        def normalize(row0, nrows, chains=None):
            for i in range(nrows // LNR):
                r0 = row0 + i * LNR
                x = x_v[pl.ds(r0, LNR), :].astype(f32)
                if chains is not None:
                    x = chains[i % len(chains)].after_rows(x)
                r, mr = _ln_stats(x)
                xn = x * r - mr
                if chains is not None:
                    chains[i % len(chains)].tok = xn[0:8, 0:128]
                for g in range(NG):
                    xn_s[g, pl.ds(r0, LNR), :] = xn[:, g * 128:(g + 1) * 128]

        def mod_chunk(k):
            col = k * KC if isinstance(k, int) else pl.multiple_of(k * KC, KC)
            sa = _mod_cols(wmod_v, st_v, col, KC)
            ca = _mod_cols(wmod_v, st_v, D + col, KC)
            mod_v[:, pl.ds(col, KC)] = jnp.broadcast_to(sa, (8, KC))
            mod_v[:, pl.ds(D + col, KC)] = jnp.broadcast_to(ca, (8, KC))
            return sa, 1.0 + ca

        def h_chunk(k, t, n, sa, ca1):
            return (xn_s[k, pl.ds(t * TM, n * TM), :] * ca1 + sa).astype(bf16)

        def mm(h, w, sec, tiles, first):
            res = _dot(h, _unpack(w))
            for i, t in enumerate(tiles):
                dst, off = qkv_dst(t, sec)
                for g in range(NG):
                    blk = res[i * TM:(i + 1) * TM, g * 128:(g + 1) * 128]
                    if first:
                        dst[g, pl.ds(off, TM), :] = blk
                    else:
                        dst[g, pl.ds(off, TM), :] += blk

        def wcur(sec):
            return wcur_s[:, sec * D:(sec + 1) * D]

        def keep(k, sec, wp):
            r0 = k * (KC // 2) if isinstance(k, int) else pl.multiple_of(k * (KC // 2), KC // 2)
            cols = pl.ds(sec * D if isinstance(sec, int) else pl.multiple_of(sec * D, D), D)
            wcur_s[:, cols] = wp
            wqkv_p[pl.ds(r0, KC // 2), cols] = wp

        scope = jax.named_scope
        mod0 = lambda: (mod_v[0:1, 0:KC], 1.0 + mod_v[0:1, D:D + KC])
        with scope('w_x0'):
            wait(cp_x(0))
        with scope('norm0'):
            def norm_body(i, carry):
                normalize(pl.multiple_of(i * 64, 64), 64)
                return carry
            jax.lax.fori_loop(0, TM // 64, norm_body, 0)
        with scope('w_wq0'):
            wait(cp_wq0())
        with scope('perm0'):
            def perm_body(sec, carry):
                keep(0, sec, _permute_qkv_section(wqkv_raw, 0, sec))
                return carry
            jax.lax.fori_loop(0, 2, perm_body, 0)
        with scope('w_m0'):
            wait(cp_chunk(0, False))
        with scope('mm00'):
            wp = _permute_qkv_section(wqkv_raw, 0, 2)
            sa, ca1 = mod_chunk(0)
            h0 = h_chunk(0, 0, 1, sa, ca1)
            for sec in range(3):
                mm(h0, wcur(sec) if sec < 2 else wp, sec, [0], True)
            keep(0, 2, wp)
        with scope('w_x12'):
            wait(cp_x(1), cp_x(2))
        with scope('mm01'):
            normalize(TM, TM)
            h1 = h_chunk(0, 1, 1, *mod0())
            for sec in range(3):
                mm(h1, wcur(sec), sec, [1], True)
            normalize(2 * TM, TM, [new_chain() for _ in range(4)])
            hl_s[...] = _pack(h_chunk(0, last, 1, *mod0()))

        def chunk_body(k0, carry):
            k = k0 + 1
            with scope('w_chunk'):
                wait(cp_chunk(k))
            with scope('chunk'):
                hl = _unpack(hl_s[...])
                for sec in range(3):
                    mm(hl, wcur(sec), sec, [last], False)
                sa, ca1 = mod_chunk(k)
                hf = h_chunk(k, 0, last, sa, ca1)
                hl_s[...] = _pack(h_chunk(k, last, 1, sa, ca1))
                for sec in range(3):
                    wp = _permute_qkv_section(wqkv_raw, pl.multiple_of(k * KC, KC), sec)
                    mm(hf, wp, sec, list(range(last)), False)
                    keep(k, sec, wp)
            return carry
        jax.lax.fori_loop(0, NKC - 1, chunk_body, 0)

        with scope('w_x3'):
            wait(cp_x(T0))
        hl = _unpack(hl_s[...])
        for sec in range(3):
            mm(hl, wcur(sec), sec, [last], False)
        _ln1_next(x_v, mod_v, h_s, T0 * TM, [new_chain() for _ in range(4)])
        k0_s[:, 0:HALO, :] = jnp.zeros((NG, HALO, 128), f32)
        v0_s[:, 0:HALO, :] = jnp.broadcast_to(v0_s[:, HALO:HALO + 1, :], (NG, HALO, 128))
        k_s[:, 0:HALO, :] = k0_s[:, TM:TM + HALO, :]
        v_s[:, 0:HALO, :] = v0_s[:, TM:TM + HALO, :]

    @_when(jnp.logical_and(step >= 1, step < N1), 'phase1')
    def _():
        needs = ((cp_x(4), cp_wo(0), cp_ff(0)),
                 (cp_x(5), cp_wm(0), cp_ff(1)),
                 (cp_x(6), cp_wo(1), cp_wm(1), cp_ff(2)),
                 (cp_x(7), cp_wm(2), cp_ff(3)),
                 (cp_wm(3), cp_ff(4)))
        for i, groups in enumerate(needs):
            pl.when(step == i + 1)(lambda groups=groups: wait(*groups))
        _phase1(step, x_v, wqkv_p, wo_raw, wo_p, so_v, w1_v, w3_v, w2_v, s1_v, s3_v, s2_v,
                wmod_v, mod_v, st_v, h_s, q0_s, k0_s, v0_s, q_s, k_s, v_s, o_s, flag_s)

    def cp_out(j):
        rows = pl.ds(pl.multiple_of(j * TM, TM), TM)
        return pltpu.make_async_copy(o_ref.at[j % 2], o_hbm.at[rows], sems.at[SEM_OUT + j % 2])

    @_when(step >= N1, 'phase2')
    def _():
        pl.when(step > N1 + 1)(lambda: cp_out(step - N1 - 2).wait())
        _phase2(step, x_v, wo_p, so_v, w1_v, w3_v, w2_v, s1_v, s3_v, s2_v, mod_v, q_s, k_s, v_s,
                o_s, note_s, flag_s, o_ref.at[(step - N1) % 2])
        cp_out(step - N1).start()

        @pl.when(step == N1 + NT - 1)
        def _():
            cp_out(NT - 2).wait()
            cp_out(NT - 1).wait()


def _scratch_shapes():
    return [
        pltpu.VMEM((S, D), bf16),
        pltpu.VMEM((D, 3 * D), bf16),
        pltpu.VMEM((D // 2, 3 * D), u32),
        pltpu.VMEM((D, D), bf16),
        pltpu.VMEM((3, DH2 // 2, DH2), u32),
        pltpu.VMEM((NS, DH2, DH2), bf16),
        pltpu.VMEM((D, F), bf16),
        pltpu.VMEM((D, F), bf16),
        pltpu.VMEM((F, D), bf16),
        pltpu.VMEM((NS, DH2, FH), bf16),
        pltpu.VMEM((NS, DH2, FH), bf16),
        pltpu.VMEM((NS, FH, DH2), bf16),
        pltpu.VMEM((D, 6 * D), bf16),
        pltpu.VMEM((8, 6 * D), f32),
        pltpu.VMEM((D, 128), f32),
        pltpu.VMEM((NG, T0 * TM, 128), f32),
        pltpu.VMEM((KC // 2, 3 * D), u32),
        pltpu.VMEM((TM // 2, KC), u32),
        pltpu.VMEM((TM, D), bf16),
        pltpu.VMEM((NG, TM, 128), f32),
        pltpu.VMEM((NG, HALO + TM, 128), f32),
        pltpu.VMEM((NG, HALO + TM, 128), f32),
        pltpu.VMEM((NG, S - TM, 128), f32),
        pltpu.VMEM((NG, HALO + S - TM, 128), f32),
        pltpu.VMEM((NG, HALO + S - TM, 128), f32),
        pltpu.VMEM((7, TM // 2, DH2), bf16),
        pltpu.VMEM((2, TM, D), bf16),
        pltpu.VMEM((1, D), bf16),
        pltpu.VMEM((8, 128), f32),
        pltpu.SMEM((1,), jnp.int32),
        pltpu.SemaphoreType.DMA((NSEM,)),
    ]


@jax.jit
def pallas_adaLN_cond__sliding_local_dilated__glu_gated_swiglu__prompt_kernel(
    A_x: jax.Array,
    A_wqkv: jax.Array,
    A_wo: jax.Array,
    B_x: jax.Array,
    B_w1: jax.Array,
    B_w3: jax.Array,
    B_w2: jax.Array,
    c: jax.Array,
    w_mod: jax.Array,
):
    del B_x
    x = A_x.reshape(S, D)
    hbm = pl.BlockSpec(memory_space=pl.ANY)
    out = pl.pallas_call(
        _kernel,
        grid=(N1 + NT,),
        in_specs=[hbm] * 8,
        out_specs=hbm,
        out_shape=jax.ShapeDtypeStruct((S, D), A_x.dtype),
        scratch_shapes=_scratch_shapes(),
        compiler_params=pltpu.CompilerParams(
            dimension_semantics=("arbitrary",),
            vmem_limit_bytes=122 * 1024 * 1024,
        ),
        name="adaln_attn_ffn",
    )(x, c, A_wqkv, A_wo, B_w1, B_w3, B_w2, w_mod)
    return out.reshape(1, S, D)
```
